```python
import jax
import jax.numpy as jnp

def _softmax(x, axis=-1):
    return jax.nn.softmax(x, axis=axis)
def _gelu(x):
    return jax.nn.gelu(x, approximate=True)
def _silu(x):
    return jax.nn.silu(x)
def _sigmoid(x):
    return jax.nn.sigmoid(x)
def _layernorm(x, axis=-1, eps=1e-5):
    m = jnp.mean(x, axis=axis, keepdims=True)
    v = jnp.var(x, axis=axis, keepdims=True)
    return (x - m) / jnp.sqrt(v + eps)
def _scatter_add(tgt, idx, src, axis=0):
    return tgt.at[idx].add(src)
def _segment_sum(src, seg, n):
    return jax.ops.segment_sum(src, seg, n)
class _Rng:
    def __init__(self, key):
        self._k = key
    def _next(self):
        self._k, sub = jax.random.split(self._k)
        return sub
    def normal(self, shape):
        return jax.random.normal(self._next(), shape, dtype=jnp.bfloat16)
    def randint(self, lo, hi, shape):
        return jax.random.randint(self._next(), shape, lo, hi, dtype=jnp.int32)
    def uniform(self, shape, lo=0.0, hi=1.0):
        return jax.random.uniform(self._next(), shape, jnp.bfloat16, lo, hi)
    def permutation(self, n):
        return jax.random.permutation(self._next(), n)


kernel_name = 'standalone__batchnorm__sampling'

def setup_inputs():
    _rng = _Rng(jax.random.key(int.from_bytes(__import__("os").urandom(4), "little")))
    _w = (lambda a: (lambda t: t.astype(jnp.bfloat16) if jnp.issubdtype(t.dtype, jnp.floating) else t)(jnp.asarray(a)))
    B, S, C = 1024, 32, 576
    K = 3
    return {
        "x": _w((lambda *s: _rng.normal(s) * 0.05)(B, S, C)),
        "w": _w((lambda *s: _rng.normal(s) * 0.05)(K, C, C) * (1.0 / (K * C) ** 0.5)),
        "mean": _w((lambda *s: _rng.normal(s) * 0.05)(C) * 0.1),
        "var": _w(jnp.abs((lambda *s: _rng.normal(s) * 0.05)(C)) + 0.5),
        "g": _w((lambda *s: _rng.normal(s) * 0.05)(C) + 1.0),
        "b": _w((lambda *s: _rng.normal(s) * 0.05)(C) * 0.1),
    }

def reference(x, w, mean, var, g, b):
    K = 3
    P = K // 2
    S = x.shape[1]
    xp = jnp.pad(x, ((0, 0), (P, P), (0, 0)))
    y = sum(jnp.einsum('bsc,cd->bsd', xp[:, k:k + S, :], w[k]) for k in range(K))
    inv_std = 1.0 / jnp.sqrt(var + 1e-5)
    y = (y - mean) * (g * inv_std) + b
    return _silu(y)
```

```python
import functools
import jax, jax.numpy as jnp
import jax.experimental.pallas as pl
import jax.experimental.pallas.tpu as pltpu

TB = 128
PACK = True
A_ = 2.0 / 3.0
B_ = 1.5
F32 = jnp.float32
BF16 = jnp.bfloat16


def _gcoef():
    a, b = A_, B_
    pts = [0.0, a, -a, b, -b]
    G = []
    for j, p in enumerate(pts):
        f = 1.0
        for k, q in enumerate(pts):
            if k != j:
                f *= (p - q)
        G.append([1.0 / f, p / f, p * p / f])
    G.append([0.0, 0.0, 1.0])
    return G


@jax.jit
def pallas_standalone__batchnorm__sampling_kernel(x, w, mean, var, g, b):
    B, S, C = x.shape
    xt = jnp.transpose(x, (1, 2, 0))
    wt = jnp.transpose(w, (0, 2, 1))
    prm = jnp.stack([mean, var, g, b], axis=1)
    CF = (C // 128) * 128
    CR = C - CF
    KP = C + CR
    a, bb = A_, B_
    a2, b2 = a * a, bb * bb
    G = _gcoef()
    c3p4, c3m4 = a2 / b2, a / bb
    cpk = {0: 1.0 - c3p4, 3: 0.5 * (c3p4 + c3m4), 4: 0.5 * (c3p4 - c3m4), 5: a ** 3 - bb ** 3 * c3m4}

    def kernel(x_ref, w_ref, p_ref, o_ref, a_ref, sh_ref, u_ref):
        @pl.when(pl.program_id(0) == 0)
        def _():
            p = p_ref[...].astype(F32)
            mean_, var_, g_, b_ = p[:, 0:1], p[:, 1:2], p[:, 2:3], p[:, 3:4]
            scale = g_ * jax.lax.rsqrt(var_ + 1e-5)
            sh_ref[...] = jnp.broadcast_to(0.5 * (b_ - mean_ * scale), sh_ref.shape)
            hs = 0.5 * scale
            def rows(r, _):
                r0 = pl.multiple_of(r * 64, 64)
                sl = pl.ds(r0, 64)
                p = p_ref[sl, :].astype(F32)
                hs = 0.5 * p[:, 2:3] * jax.lax.rsqrt(p[:, 1:2] + 1e-5)
                w0 = w_ref[0, sl, :].astype(F32) * hs
                w1 = w_ref[1, sl, :].astype(F32) * hs
                w2 = w_ref[2, sl, :].astype(F32) * hs
                gs = []
                for j in range(6):
                    t = None
                    for cf, wk in zip(G[j], (w0, w1, w2)):
                        if cf != 0.0:
                            term = wk if cf == 1.0 else cf * wk
                            t = term if t is None else t + term
                    gs.append(t)
                for j in range(6):
                    a_ref[j, sl, 0:C] = gs[j].astype(BF16)
                    if PACK and j in cpk:
                        a_ref[j, sl, C:KP] = (cpk[j] * gs[1][:, CF:C]).astype(BF16)
                    else:
                        a_ref[j, sl, C:KP] = jnp.zeros((64, CR), BF16)
                return 0
            jax.lax.fori_loop(0, C // 64, rows, 0)
            if not PACK:
                for j in range(6):
                    u_ref[j, C:KP, :] = jnp.zeros((CR, TB), BF16)
            else:
                u_ref[2, C:KP, :] = jnp.zeros((CR, TB), BF16)

        def quad(q, _):
            s0 = 4 * q
            ld = lambda s: x_ref[s].astype(F32)
            d0 = jnp.where(q > 0, ld(jnp.maximum(s0 - 1, 0)), 0.0)
            d1, d2, d3, d4 = ld(s0), ld(s0 + 1), ld(s0 + 2), ld(s0 + 3)
            d5 = jnp.where(q < S // 4 - 1, ld(jnp.minimum(s0 + 4, S - 1)), 0.0)
            b2d2, a2d2, a2d3, b2d3 = b2 * d2, a2 * d2, a2 * d3, b2 * d3
            e1, e2 = d4 - b2d2, d4 - a2d2
            o1r = d1 - a2d3
            o1, o2 = bb * o1r, a * (d1 - b2d3)
            u = [(d0 + e1) - a2d2, e1 - o1, e1 + o1, e2 - o2, e2 + o2, (d5 + o1r) - b2d3]
            u = [t.astype(BF16) for t in u]
            for j in range(6):
                u_ref[j, 0:C, :] = u[j]
            if PACK:
                for j in cpk:
                    u_ref[j, C:KP, :] = u[1][CF:C, :]
            m = []
            for j in range(6):
                k = CF if (PACK and j == 1) else KP
                m.append(jnp.dot(a_ref[j, :, 0:k], u_ref[j, 0:k, :], preferred_element_type=F32))
            s1, dd1, s2, dd2 = m[1] + m[2], m[1] - m[2], m[3] + m[4], m[3] - m[4]
            sh = sh_ref[...]
            ys = [(m[0] + s1) + (s2 + sh),
                  (a * dd1 + sh) + bb * dd2,
                  (a2 * s1 + sh) + b2 * s2,
                  (a ** 3 * dd1 + sh) + (bb ** 3 * dd2 + m[5])]
            for i in range(4):
                h = ys[i]
                o_ref[s0 + i] = (h * jnp.tanh(h) + h).astype(o_ref.dtype)
            return 0
        jax.lax.fori_loop(0, S // 4, quad, 0)

    out = pl.pallas_call(
        kernel,
        grid=(B // TB,),
        in_specs=[pl.BlockSpec((S, C, TB), lambda i: (0, 0, i)),
                  pl.BlockSpec((3, C, C), lambda i: (0, 0, 0)),
                  pl.BlockSpec((C, 4), lambda i: (0, 0))],
        out_specs=pl.BlockSpec((S, C, TB), lambda i: (0, 0, i)),
        out_shape=jax.ShapeDtypeStruct((S, C, B), x.dtype),
        scratch_shapes=[pltpu.VMEM((6, C, KP), BF16), pltpu.VMEM((C, TB), F32), pltpu.VMEM((6, KP, TB), BF16)],
        compiler_params=pltpu.CompilerParams(dimension_semantics=("arbitrary",), vmem_limit_bytes=100 * 1024 * 1024),
    )(xt, wt, prm)
    return jnp.transpose(out, (2, 0, 1))
```

```python
import os
import jax, jax.numpy as jnp
import jax.experimental.pallas as pl
import jax.experimental.pallas.tpu as pltpu

TB = 128
UPB = int(os.environ.get("UPB", "2"))
RC = int(os.environ.get("RC", "16"))
JORD = [int(c) for c in os.environ.get("JORD", "01234567")]
NEP = int(os.environ.get("NEP", "4"))
F32 = jnp.float32
BF16 = jnp.bfloat16
U32 = jnp.uint32

MO = 6
NP = MO + 2
CH = 8
NPRO = 2
CPK = {0: -2.25, 3: -0.025, 4: 0.075, 5: 0.8, 6: 2.4, 7: 2.25}


@jax.jit
def pallas_standalone__batchnorm__sampling_kernel(x, w, mean, var, g, b):
    B, S, C = x.shape
    xt = jnp.transpose(x, (1, 2, 0))
    NKT = C // 128
    CF = NKT * 128
    CR = C - CF
    SP = S + 1
    NB = B // TB
    NU = NB * SP // MO
    RING = 2 * SP
    UPR = RING // MO
    CPT = S // CH
    NCH = NB * CPT
    NMB = max(2, UPB if UPB % 2 else 2)
    NBODY = (NU - NPRO) // UPB
    assert (NU - NPRO) % UPB == 0
    LEAD = int(os.environ.get("LEAD", "3"))
    NSP = MO * NPRO + 1
    CSP = -(-NSP // CH)

    def chunk_of(p):
        if isinstance(p, int):
            return CPT * (p // SP) + min((p % SP) // CH, CPT - 1)
        return CPT * (p // SP) + jnp.minimum((p % SP) // CH, CPT - 1)

    first = lambda i: NPRO + UPB * i
    xneed = lambda i: chunk_of(MO * first(i + 1) + MO - 1) + 1
    def odone(i):
        p = MO * (first(i + 1) - 1)
        return CPT * (p // SP) + (p % SP) // CH
    def ofree(i):
        p = MO * (first(i + 1) - 1) - 1 - RING
        if isinstance(p, int):
            return 0 if p < 0 else chunk_of(p) + 1
        return jnp.where(p < 0, 0, chunk_of(jnp.maximum(p, 0)) + 1)
    MAXC = (MO * UPB + CH - 1) // CH + (1 if UPB > 2 else 0)
    assert odone(-1) == 0 and odone(NBODY - 1) == NCH - 1
    for i in range(NBODY):
        assert xneed(i + 1) - xneed(i) <= MAXC and odone(i) - odone(i - 1) <= MAXC
        assert ofree(i + 1) - ofree(i) <= MAXC and ofree(i + 1) <= odone(i - 1)
        cmax = min(xneed(i + 1) + LEAD, NCH) - 1 - 2 * CPT
        if cmax >= 0:
            assert SP * (cmax // CPT) + CH * (cmax % CPT) + CH - 1 < MO * first(i + 1) - 1
    assert xneed(0) + LEAD <= 2 * CPT

    XS0, OS0 = 0, 2 * CPT
    WS0 = 4 * CPT
    PS0 = WS0 + NKT + 1
    KS0 = PS0 + 4
    ES0 = KS0 + NKT + 2
    NSEM = ES0 + NEP + 1

    def kernel(x_hbm, w_hbm, mean_hbm, var_hbm, g_hbm, b_hbm, o_hbm,
               a_ref, sh_ref, hs_ref, u0_ref, wbuf, p0, p1, p2, p3, xbuf, obuf, sems, tab, *m_refs):

        def hbm_chunk(ref, c):
            lane0 = (c >> 2) * TB
            if not isinstance(c, int):
                lane0 = pl.multiple_of(lane0, TB)
            return ref.at[pl.ds((c & 3) * CH, CH), :, pl.ds(lane0, TB)]

        def ring_slot(c):
            return ((c >> 2) & 1) * SP + (c & 3) * CH

        def xcopy(c):
            return pltpu.make_async_copy(hbm_chunk(x_hbm, c), xbuf.at[pl.ds(ring_slot(c) + 1, CH)],
                                         sems.at[XS0 + (c & 7)])

        def ocopy(c):
            return pltpu.make_async_copy(obuf.at[pl.ds(ring_slot(c), CH)], hbm_chunk(o_hbm, c),
                                         sems.at[OS0 + (c & 7)])

        def krows(kt):
            if isinstance(kt, int):
                return pl.ds(kt * 128, 128 if kt < NKT else CR)
            return pl.ds(pl.multiple_of(kt * 128, 128), 128)

        def wcopy(kt):
            return pltpu.make_async_copy(w_hbm.at[:, krows(kt), :], wbuf.at[:, krows(kt), :], sems.at[WS0 + kt])

        def kcopy(kt):
            return pltpu.make_async_copy(x_hbm.at[pl.ds(0, NSP), krows(kt), pl.ds(0, TB)],
                                         xbuf.at[pl.ds(1, NSP), krows(kt), :], sems.at[KS0 + kt])
        rcopy = pltpu.make_async_copy(x_hbm.at[pl.ds(NSP, CSP * CH - NSP), :, pl.ds(0, TB)],
                                      xbuf.at[pl.ds(1 + NSP, CSP * CH - NSP)], sems.at[KS0 + NKT + 1])

        pcopies = [pltpu.make_async_copy(s, d, sems.at[PS0 + i])
                   for i, (s, d) in enumerate(zip((mean_hbm, var_hbm, g_hbm, b_hbm), (p0, p1, p2, p3)))]
        for c in pcopies:
            c.start()
        for kt in range(NKT + 1):
            wcopy(kt).start()
            kcopy(kt).start()
        rcopy.start()
        for c in range(CSP, xneed(0) + LEAD):
            xcopy(c).start()

        for i in range(NBODY + 1):
            tab[3 * i], tab[3 * i + 1], tab[3 * i + 2] = odone(i - 1), min(xneed(i), NCH), ofree(i)

        pm = [m_refs[(UPB - NPRO + u) % NMB] for u in range(NPRO)]
        for r in pm:
            r[...] = jnp.zeros(r.shape, F32)
        for s in (0, SP, RING, RING + 1):
            xbuf[s] = jnp.zeros((C, TB), BF16)

        for c in pcopies:
            c.wait()
        mean_, var_, g_, b_ = [r[...].astype(F32).reshape(1, C) for r in (p0, p1, p2, p3)]
        scale = g_ * jax.lax.rsqrt(var_ + 1e-5)
        hs_ref[...] = jnp.broadcast_to(0.5 * scale, (128, C)).T
        sh = 0.5 * (b_ - mean_ * scale)
        sh_hi = sh.astype(BF16).astype(F32)
        sh_mid = (sh - sh_hi).astype(BF16).astype(F32)
        sh_lo = (sh - sh_hi) - sh_mid
        row = jax.lax.broadcasted_iota(jnp.int32, (128, C), 0)
        sh_ref[...] = jnp.where(row == CR, sh_hi, jnp.where(row == CR + 1, sh_mid, jnp.where(row == CR + 2, sh_lo, 0.0))).T

        def prep(kt):
            last = isinstance(kt, int) and kt == NKT
            if last:
                wts = [jnp.concatenate([wbuf[k, CF:C, :], wbuf[k, CF:C, :]], axis=0).T for k in range(3)]
                lo = jax.lax.broadcasted_iota(jnp.int32, (8, 128), 1) < CR
            else:
                wts = [wbuf[k, krows(kt), :].T for k in range(3)]
            wu = [pltpu.bitcast(t, U32) for t in wts]
            for r in range(0, C // 2, 8):
                halves = []
                for h in range(2):
                    hs = hs_ref[pl.ds(2 * r + h, 8, stride=2), :]
                    w0, w1, w2 = [pltpu.unpack_elementwise(t[r:r + 8, :], index=h, packed_dtype=BF16, unpacked_dtype=F32) * hs
                                  for t in wu]
                    e1, o1 = (-2.0 / 9) * (w0 + w2), (-2.0 / 9) * w1
                    e2, o2 = (1.0 / 90) * w0 + (2.0 / 45) * w2, (1.0 / 45) * w1
                    e3, o3 = (32.0 / 45) * w0 + (8.0 / 45) * w2, (16.0 / 45) * w1
                    gs = [w0, e1 + o1, e1 - o1, e2 + o2, e2 - o2, e3 + o3, e3 - o3, w2]
                    if last:
                        ext = dict((j, c * gs[2]) for j, c in CPK.items())
                        ext[1] = sh_ref[pl.ds(2 * r + h, 8, stride=2), :]
                        gs = [jnp.where(lo, gs[j], ext[j]) if j != 2 else None for j in range(NP)]
                    halves.append(gs)
                for j in range(NP):
                    if halves[0][j] is not None:
                        a_ref[j, kt, r:r + 8, :] = pltpu.pack_elementwise([halves[0][j], halves[1][j]], packed_dtype=BF16)

        def tchunk(ld, with_u0=True):
            d1, d2, d3, d4, d5, d6 = [ld(i, 1) for i in range(1, 7)]
            e1, o1 = (d2 + d6) - 4.25 * d4, (d1 + d5) - 4.25 * d3
            d1, d2, d3, d4, d5, d6 = [ld(i, 2) for i in range(1, 7)]
            e2, o2 = (d6 - d4) - 0.25 * (d4 - d2), 2.0 * (d5 - d3) - 0.5 * (d3 - d1)
            d1, d2, d3, d4, d5, d6 = [ld(i, 3) for i in range(1, 7)]
            e3, o3 = (d6 - d4) - 4.0 * (d4 - d2), 0.5 * (d5 - d3) - 2.0 * (d3 - d1)
            d1, d3, d5, d7 = [ld(i, 4) for i in (1, 3, 5, 7)]
            u = [None, e1 + o1, e1 - o1, e2 + o2, e2 - o2, e3 + o3, e3 - o3, (d7 - d1) - 5.25 * (d5 - d3)]
            if with_u0:
                d0, d2, d4, d6 = [ld(i, 0) for i in (0, 2, 4, 6)]
                u[0] = (d0 - d6) + 5.25 * (d4 - d2)
            return u

        def ones_rows():
            return (jax.lax.broadcasted_iota(jnp.int32, (CR, TB), 0) < 3).astype(F32)

        def mm(kt):
            last = isinstance(kt, int) and kt == NKT
            r0 = kt * 128 if isinstance(kt, int) else pl.multiple_of(kt * 128, 128)
            for u in range(NPRO):
                cs = [tchunk(lambda i, gi: xbuf[MO * u + i, pl.ds(r0 + r, RC), :].astype(F32))
                      for r in range(0, CR if last else 128, RC)]
                for j in range(NP):
                    parts = [c[j] for c in cs]
                    if last:
                        if j == 2:
                            continue
                        parts = parts + ([ones_rows()] if j == 1 else [c[2] for c in cs])
                    rhs = jnp.concatenate(parts, axis=0).astype(BF16)
                    pm[u][j] += jnp.dot(pltpu.bitcast(a_ref[j, kt], BF16), rhs, preferred_element_type=F32)

        def carry_u0(t):
            base = (t % UPR) * MO
            for r in range(0, CF, RC):
                d0, d2, d4, d6 = [xbuf[base + i, r:r + RC, :].astype(F32) for i in (0, 2, 4, 6)]
                u0_ref[r:r + RC, :] = ((d0 - d6) + 5.25 * (d4 - d2)).astype(BF16)

        def transform(t, carried, zs):
            base = (t % UPR) * MO
            cs = [tchunk(lambda i, gi: xbuf[base + zs[gi] + i, r:r + RC, :].astype(F32), not (carried and r < CF))
                  for r in range(0, C, RC)]
            tail = [c[2] for c in cs[CF // RC:]]
            out = []
            for j in range(NP):
                parts = [c[j] for c in cs if c[j] is not None]
                if j == 2:
                    parts = parts[:CF // RC]
                else:
                    parts = parts + ([ones_rows()] if j == 1 else tail)
                v = jnp.concatenate(parts, axis=0).astype(BF16)
                if j == 0 and carried:
                    v = jnp.concatenate([u0_ref[...], v], axis=0)
                out.append(v)
            return out

        def dots(us, m_ref, z):
            for j in JORD:
                nk = NKT if j == 2 else NKT + 1
                lhs = pltpu.bitcast(jnp.concatenate([a_ref[j, kt] for kt in range(nk)], axis=1), BF16)
                m_ref[j + z] = jnp.dot(lhs, us[j], preferred_element_type=F32)

        def output(t, m_ref, rlo=0, rhi=C, nout=MO):
            base = (t % UPR) * MO
            for r in range(rlo, rhi, RC):
                m = [m_ref[j, r:r + RC, :] for j in range(NP)]
                s1, s2, s3 = m[1] + m[2], m[3] + m[4], m[5] + m[6]
                d1, d2, d3 = m[1] - m[2], m[3] - m[4], m[5] - m[6]
                ys = [(m[0] + s1) + (s2 + s3),
                      (d1 + 2.0 * d2) + 0.5 * d3,
                      (s1 + 4.0 * s2) + 0.25 * s3,
                      (d1 + 8.0 * d2) + 0.125 * d3,
                      (s1 + 16.0 * s2) + 0.0625 * s3,
                      (d1 + 32.0 * d2) + (0.03125 * d3 + m[7])]
                for i in range(nout):
                    h = ys[i]
                    obuf[base + i, r:r + RC, :] = (h * jnp.tanh(h) + h).astype(BF16)

        wcopy(0).wait()
        prep(0)
        def kblock(kt, _):
            kcopy(kt).wait()
            wcopy(kt + 1).wait()
            prep(kt + 1)
            mm(kt)
            return 0
        jax.lax.fori_loop(0, NKT - 1, kblock, 0)
        kblock(NKT - 1, 0)
        kcopy(NKT).wait()
        mm(NKT)
        for u in range(NPRO - 1):
            output(u, pm[u])
        rcopy.wait()
        for c in range(CSP, xneed(0)):
            xcopy(c).wait()
        carry_u0(NPRO)

        def body(i, _):
            t0 = first(i)
            z = jnp.minimum(i, 0)
            zs = [0] + [jnp.minimum(i + gq, 0) for gq in range(1, 5)]
            for k in range(UPB):
                t = t0 + k
                dots(transform(t, k == 0, zs), m_refs[k % NMB], z)
                output(t - 1, m_refs[(k - 1) % UPB % NMB])
            carry_u0(jnp.minimum(t0 + UPB, NU - 1))
            o0, o1 = tab[3 * i], tab[3 * i + 3]
            for k in range(MAXC):
                @pl.when(o0 + k < o1)
                def _():
                    ocopy(o0 + k).start()
            n0, n1 = tab[3 * i + 1], tab[3 * i + 4]
            for k in range(MAXC):
                @pl.when(jnp.logical_and(n0 + k < n1, n0 + k + LEAD < NCH))
                def _():
                    xcopy(n0 + k + LEAD).start()
            for k in range(MAXC):
                @pl.when(n0 + k < n1)
                def _():
                    xcopy(n0 + k).wait()
            f0, f1 = tab[3 * i + 2], tab[3 * i + 5]
            for k in range(MAXC):
                @pl.when(f0 + k < f1)
                def _():
                    ocopy(f0 + k).wait()
            return 0
        jax.lax.fori_loop(0, NBODY, body, 0)

        plast = MO * (NU - 1)
        s0, sl = S - CH, plast % SP
        slot0 = ring_slot(NCH - 1)
        lanes = pl.ds((NB - 1) * TB, TB)
        ecopies = [pltpu.make_async_copy(obuf.at[pl.ds(slot0, sl - s0)], o_hbm.at[pl.ds(s0, sl - s0), :, lanes],
                                         sems.at[ES0])]
        ecopies[0].start()
        RP = C // NEP
        for e in range(NEP):
            output(NU - 1, m_refs[(UPB - 1) % NMB], e * RP, (e + 1) * RP, S - sl)
            cp = pltpu.make_async_copy(obuf.at[pl.ds(slot0 + sl - s0, S - sl), pl.ds(e * RP, RP), :],
                                       o_hbm.at[pl.ds(sl, S - sl), pl.ds(e * RP, RP), lanes], sems.at[ES0 + 1 + e])
            cp.start()
            ecopies.append(cp)
        for c in range(ofree(NBODY), NCH - 1):
            ocopy(c).wait()
        for cp in ecopies:
            cp.wait()

    any_spec = pl.BlockSpec(memory_space=pl.ANY)
    out = pl.pallas_call(
        kernel,
        in_specs=[any_spec] * 6,
        out_specs=any_spec,
        out_shape=jax.ShapeDtypeStruct((S, C, B), x.dtype),
        scratch_shapes=[pltpu.VMEM((NP, NKT + 1, C // 2, 128), U32),
                        pltpu.VMEM((C, 128), F32), pltpu.VMEM((C, 128), F32),
                        pltpu.VMEM((CF, TB), BF16),
                        pltpu.VMEM((3, C, C), BF16),
                        pltpu.VMEM((C,), BF16), pltpu.VMEM((C,), BF16), pltpu.VMEM((C,), BF16), pltpu.VMEM((C,), BF16),
                        pltpu.VMEM((RING + 2, C, TB), BF16), pltpu.VMEM((RING, C, TB), BF16),
                        pltpu.SemaphoreType.DMA((NSEM,)), pltpu.SMEM((3 * (NBODY + 1),), jnp.int32)]
                       + [pltpu.VMEM((NP, C, TB), F32) for _ in range(NMB)],
        compiler_params=pltpu.CompilerParams(vmem_limit_bytes=100 * 1024 * 1024, disable_bounds_checks=True),
    )(xt, w, mean, var, g, b)
    return jnp.transpose(out, (2, 0, 1))
```

```python
import os
import jax, jax.numpy as jnp
import jax.experimental.pallas as pl
import jax.experimental.pallas.tpu as pltpu

TB = 128
UPB = int(os.environ.get("UPB", "2"))
RC = int(os.environ.get("RC", "16"))
JORD = [int(c) for c in os.environ.get("JORD", "01234567")]
NEP = int(os.environ.get("NEP", "4"))
TIE = int(os.environ.get("TIE", "1"))
KSP = int(os.environ.get("KSP", "0"))
ILV = int(os.environ.get("ILV", "1"))
GRP = [int(c) for c in os.environ.get("GRP", "01222")]
ZO = int(os.environ.get("ZO", "0"))
PTRIG = int(os.environ.get("PTRIG", "99"))
F32 = jnp.float32
BF16 = jnp.bfloat16
U32 = jnp.uint32

MO = 6
NP = MO + 2
CH = 8
NPRO = 2
CPK = {0: -2.25, 3: -0.025, 4: 0.075, 5: 0.8, 6: 2.4, 7: 2.25}


@jax.jit
def pallas_standalone__batchnorm__sampling_kernel(x, w, mean, var, g, b):
    B, S, C = x.shape
    xt = jnp.transpose(x, (1, 2, 0))
    NKT = C // 128
    CF = NKT * 128
    CR = C - CF
    SP = S + 1
    NB = B // TB
    NU = NB * SP // MO
    RING = 2 * SP
    UPR = RING // MO
    CPT = S // CH
    NCH = NB * CPT
    NMB = max(2, UPB if UPB % 2 else 2)
    NBODY = (NU - NPRO) // UPB
    assert (NU - NPRO) % UPB == 0
    LEAD = int(os.environ.get("LEAD", "3"))
    NSP = MO * NPRO + 1
    CSP = -(-NSP // CH)

    def chunk_of(p):
        if isinstance(p, int):
            return CPT * (p // SP) + min((p % SP) // CH, CPT - 1)
        return CPT * (p // SP) + jnp.minimum((p % SP) // CH, CPT - 1)

    first = lambda i: NPRO + UPB * i
    xneed = lambda i: chunk_of(MO * first(i + 1) + MO - 1) + 1
    def odone(i):
        p = MO * (first(i + 1) - 1)
        return CPT * (p // SP) + (p % SP) // CH
    def ofree(i):
        p = MO * (first(i + 1) - 1) - 1 - RING
        if isinstance(p, int):
            return 0 if p < 0 else chunk_of(p) + 1
        return jnp.where(p < 0, 0, chunk_of(jnp.maximum(p, 0)) + 1)
    MAXC = (MO * UPB + CH - 1) // CH + (1 if UPB > 2 else 0)
    assert odone(-1) == 0 and odone(NBODY - 1) == NCH - 1
    for i in range(NBODY):
        assert xneed(i + 1) - xneed(i) <= MAXC and odone(i) - odone(i - 1) <= MAXC
        assert ofree(i + 1) - ofree(i) <= MAXC and ofree(i + 1) <= odone(i - 1)
        cmax = min(xneed(i + 1) + LEAD, NCH) - 1 - 2 * CPT
        if cmax >= 0:
            assert SP * (cmax // CPT) + CH * (cmax % CPT) + CH - 1 < MO * first(i + 1) - 1
    assert xneed(0) + LEAD <= 2 * CPT

    XS0, OS0 = 0, 2 * CPT
    WS0 = 4 * CPT
    PS0 = WS0 + NKT + 1
    KS0 = PS0 + 4
    ES0 = KS0 + NKT + 2
    NSEM = ES0 + NEP + 4

    def kernel(x_hbm, w_hbm, mean_hbm, var_hbm, g_hbm, b_hbm, o_hbm,
               a_ref, sh_ref, hs_ref, u0_ref, wbuf, p0, p1, p2, p3, xbuf, obuf, sems, tab, *m_refs):

        xu = xbuf.bitcast(U32)

        def hbm_chunk(ref, c):
            lane0 = (c >> 2) * TB
            if not isinstance(c, int):
                lane0 = pl.multiple_of(lane0, TB)
            return ref.at[pl.ds((c & 3) * CH, CH), :, pl.ds(lane0, TB)]

        def ring_slot(c):
            return ((c >> 2) & 1) * SP + (c & 3) * CH

        def xcopy(c):
            return pltpu.make_async_copy(hbm_chunk(x_hbm, c), xbuf.at[pl.ds(ring_slot(c) + 1, CH)],
                                         sems.at[XS0 + (c & 7)])

        def ocopy(c):
            return pltpu.make_async_copy(obuf.at[pl.ds(ring_slot(c), CH)], hbm_chunk(o_hbm, c),
                                         sems.at[OS0 + (c & 7)])

        def krows(kt):
            if isinstance(kt, int):
                return pl.ds(kt * 128, 128 if kt < NKT else CR)
            return pl.ds(pl.multiple_of(kt * 128, 128), 128)

        def wcopy(kt):
            return pltpu.make_async_copy(w_hbm.at[:, krows(kt), :], wbuf.at[:, krows(kt), :], sems.at[WS0 + kt])

        def kcopy(kt):
            return pltpu.make_async_copy(x_hbm.at[pl.ds(0, NSP), krows(kt), pl.ds(0, TB)],
                                         xbuf.at[pl.ds(1, NSP), krows(kt), :], sems.at[KS0 + kt])
        rcopy = pltpu.make_async_copy(x_hbm.at[pl.ds(NSP, CSP * CH - NSP), :, pl.ds(0, TB)],
                                      xbuf.at[pl.ds(1 + NSP, CSP * CH - NSP)], sems.at[KS0 + NKT + 1])

        pcopies = [pltpu.make_async_copy(s, d, sems.at[PS0 + i])
                   for i, (s, d) in enumerate(zip((mean_hbm, var_hbm, g_hbm, b_hbm), (p0, p1, p2, p3)))]
        for c in pcopies:
            c.start()
        for kt in range(NKT + 1):
            wcopy(kt).start()
            kcopy(kt).start()
        rcopy.start()
        for c in range(CSP, xneed(0) + LEAD):
            xcopy(c).start()

        for i in range(NBODY + 1):
            tab[3 * i], tab[3 * i + 1], tab[3 * i + 2] = odone(i - 1), min(xneed(i), NCH), ofree(i)

        pm = [m_refs[(UPB - NPRO + u) % NMB] for u in range(NPRO)]
        for r in pm:
            r[...] = jnp.zeros(r.shape, F32)
        for s in (0, SP, RING, RING + 1):
            xbuf[s] = jnp.zeros((C, TB), BF16)

        for c in pcopies:
            c.wait()
        mean_, var_, g_, b_ = [r[...].astype(F32).reshape(1, C) for r in (p0, p1, p2, p3)]
        scale = g_ * jax.lax.rsqrt(var_ + 1e-5)
        hs_ref[...] = jnp.broadcast_to(0.5 * scale, (128, C)).T
        sh = 0.5 * (b_ - mean_ * scale)
        sh_hi = sh.astype(BF16).astype(F32)
        sh_mid = (sh - sh_hi).astype(BF16).astype(F32)
        sh_lo = (sh - sh_hi) - sh_mid
        row = jax.lax.broadcasted_iota(jnp.int32, (128, C), 0)
        sh_ref[...] = jnp.where(row == CR, sh_hi, jnp.where(row == CR + 1, sh_mid, jnp.where(row == CR + 2, sh_lo, 0.0))).T

        def prep(kt):
            last = isinstance(kt, int) and kt == NKT
            lo = jax.lax.broadcasted_iota(jnp.int32, (8, 128), 1) < CR
            for r in range(0, C // 2, 8):
                if r % 64 == 0:
                    cols = slice(2 * r, min(2 * r + 128, C))
                    if last:
                        wts = [jnp.concatenate([wbuf[k, CF:C, cols], wbuf[k, CF:C, cols]], axis=0).T for k in range(3)]
                    else:
                        wts = [wbuf[k, krows(kt), cols].T for k in range(3)]
                    wu = [pltpu.bitcast(t, U32) for t in wts]
                rr = r % 64
                halves = []
                for h in range(2):
                    hs = hs_ref[pl.ds(2 * r + h, 8, stride=2), :]
                    w0, w1, w2 = [pltpu.unpack_elementwise(t[rr:rr + 8, :], index=h, packed_dtype=BF16, unpacked_dtype=F32) * hs
                                  for t in wu]
                    e1, o1 = (-2.0 / 9) * (w0 + w2), (-2.0 / 9) * w1
                    e2, o2 = (1.0 / 90) * w0 + (2.0 / 45) * w2, (1.0 / 45) * w1
                    e3, o3 = (32.0 / 45) * w0 + (8.0 / 45) * w2, (16.0 / 45) * w1
                    gs = [w0, e1 + o1, e1 - o1, e2 + o2, e2 - o2, e3 + o3, e3 - o3, w2]
                    if last:
                        ext = dict((j, c * gs[2]) for j, c in CPK.items())
                        ext[1] = sh_ref[pl.ds(2 * r + h, 8, stride=2), :]
                        gs = [jnp.where(lo, gs[j], ext[j]) if j != 2 else None for j in range(NP)]
                    halves.append(gs)
                for j in range(NP):
                    if halves[0][j] is not None:
                        a_ref[j, kt, r:r + 8, :] = pltpu.pack_elementwise([halves[0][j], halves[1][j]], packed_dtype=BF16)

        def tchunk(ld, with_u0=True):
            d1, d2, d3, d4, d5, d6 = [ld(i, 1) for i in range(1, 7)]
            e1, o1 = (d2 + d6) - 4.25 * d4, (d1 + d5) - 4.25 * d3
            d1, d2, d3, d4, d5, d6 = [ld(i, 2) for i in range(1, 7)]
            e2, o2 = (d6 - d4) - 0.25 * (d4 - d2), 2.0 * (d5 - d3) - 0.5 * (d3 - d1)
            d1, d2, d3, d4, d5, d6 = [ld(i, 3) for i in range(1, 7)]
            e3, o3 = (d6 - d4) - 4.0 * (d4 - d2), 0.5 * (d5 - d3) - 2.0 * (d3 - d1)
            d1, d3, d5, d7 = [ld(i, 4) for i in (1, 3, 5, 7)]
            u = [None, e1 + o1, e1 - o1, e2 + o2, e2 - o2, e3 + o3, e3 - o3, (d7 - d1) - 5.25 * (d5 - d3)]
            if with_u0:
                d0, d2, d4, d6 = [ld(i, 0) for i in (0, 2, 4, 6)]
                u[0] = (d0 - d6) + 5.25 * (d4 - d2)
            return u

        def ones_rows():
            return (jax.lax.broadcasted_iota(jnp.int32, (CR, TB), 0) < 3).astype(F32)

        def mm(kt, z=0):
            last = isinstance(kt, int) and kt == NKT
            r0 = kt * 128 if isinstance(kt, int) else pl.multiple_of(kt * 128, 128)
            for u in range(NPRO):
                cs = [tchunk(lambda i, gi: xbuf[MO * u + i, pl.ds(r0 + r, RC), :].astype(F32))
                      for r in range(0, CR if last else 128, RC)]
                for j in range(NP):
                    parts = [c[j] for c in cs]
                    if last:
                        if j == 2:
                            continue
                        parts = parts + ([ones_rows()] if j == 1 else [c[2] for c in cs])
                    rhs = jnp.concatenate(parts, axis=0).astype(BF16)
                    zz = z if u * NP + j >= PTRIG else 0
                    pm[u][j] += jnp.dot(pltpu.bitcast(a_ref[j + zz, kt], BF16), rhs, preferred_element_type=F32)

        def carry_u0(t):
            base = (t % UPR) * MO
            for r in range(0, CF, RC):
                d0, d2, d4, d6 = [xbuf[base + i, r:r + RC, :].astype(F32) for i in (0, 2, 4, 6)]
                u0_ref[r:r + RC, :] = ((d0 - d6) + 5.25 * (d4 - d2)).astype(BF16)

        def transform(t, carried, zs, never):
            base = (t % UPR) * MO
            if not ILV:
                cs = [tchunk(lambda i, gi: xbuf[base + zs[gi] + i, r:r + RC, :].astype(F32), not (carried and r < CF))
                      for r in range(0, C, RC)]
                tail = [c[2] for c in cs[CF // RC:]]
                out = []
                for j in range(NP):
                    parts = [c[j] for c in cs if c[j] is not None]
                    if j == 2:
                        parts = parts[:CF // RC]
                    else:
                        parts = parts + ([ones_rows()] if j == 1 else tail)
                    v = jnp.concatenate(parts, axis=0).astype(BF16)
                    if j == 0 and carried:
                        v = jnp.concatenate([u0_ref[...], v], axis=0)
                    out.append(v)
                return out
            cs = []
            for r in range(0, C, RC):
                hv = []
                for h in range(2):
                    ld = lambda i, gi: pltpu.unpack_elementwise(
                        xu[base + zs[GRP[gi]] + i, r // 2:(r + RC) // 2, :], index=h, packed_dtype=BF16, unpacked_dtype=F32)
                    hv.append(tchunk(ld, not (carried and r < CF)))
                c = [None if hv[0][j] is None else pltpu.pack_elementwise([hv[0][j], hv[1][j]], packed_dtype=BF16) for j in range(NP)]
                if TIE:
                    gof = [GRP[q] for q in (0, 1, 1, 2, 2, 3, 3, 4)]
                    for gid in sorted(set(GRP)):
                        mem = [j for j in JORD if gof[j] == gid and c[j] is not None]
                        if len(mem) > 1:
                            acc = c[mem[1]]
                            for j in mem[2:]:
                                acc = acc ^ c[j]
                            c[mem[0]] = jnp.where(never, acc, c[mem[0]])
                cs.append(c)
            tail = [c[2] for c in cs[CF // RC:]]
            ones = pltpu.bitcast(ones_rows().astype(BF16), U32)
            out = []
            for j in range(NP):
                parts = [c[j] for c in cs if c[j] is not None]
                if j == 2:
                    parts = parts[:CF // RC]
                else:
                    parts = parts + ([ones] if j == 1 else tail)
                v = pltpu.bitcast(jnp.concatenate(parts, axis=0), BF16)
                if j == 0 and carried:
                    v = jnp.concatenate([u0_ref[...], v], axis=0)
                out.append(v)
            return out

        def dots(us, m_ref, z, rlo=0, rhi=C, skip=()):
            lhs = lambda j, k0, k1: pltpu.bitcast(jnp.concatenate([a_ref[j, kt, rlo // 2:rhi // 2, :] for kt in range(k0, k1)], axis=1), BF16)
            if not KSP:
                for j in JORD:
                    if j in skip:
                        continue
                    nk = NKT if j == 2 else NKT + 1
                    (m_ref[j] if isinstance(m_ref, list) else m_ref)[j + z, rlo:rhi, :] = jnp.dot(lhs(j, 0, nk), us[j], preferred_element_type=F32)
                return
            for grp in ((0,), (1, 2), (3, 4), (5, 6), (7,)):
                acc = {}
                step = KSP if len(grp) > 1 else NKT + 1
                for k0 in range(0, NKT + 1, step):
                    for j in grp:
                        nk = NKT if j == 2 else NKT + 1
                        k1 = min(k0 + step, nk)
                        if k1 <= k0:
                            continue
                        p = jnp.dot(lhs(j, k0, k1), us[j][k0 * 128:k1 * 128], preferred_element_type=F32)
                        acc[j] = p if j not in acc else acc[j] + p
                for j in grp:
                    m_ref[j + z] = acc[j]

        def output(t, m_ref, rlo=0, rhi=C, nout=MO):
            base = (t % UPR) * MO
            for r in range(rlo, rhi, RC):
                m = [(m_ref[j] if isinstance(m_ref, list) else m_ref)[j, r:r + RC, :] if (j < NP - 1 or nout == MO) else 0.0 for j in range(NP)]
                s1, s2, s3 = m[1] + m[2], m[3] + m[4], m[5] + m[6]
                d1, d2, d3 = m[1] - m[2], m[3] - m[4], m[5] - m[6]
                ys = [(m[0] + s1) + (s2 + s3),
                      (d1 + 2.0 * d2) + 0.5 * d3,
                      (s1 + 4.0 * s2) + 0.25 * s3,
                      (d1 + 8.0 * d2) + 0.125 * d3,
                      (s1 + 16.0 * s2) + 0.0625 * s3,
                      (d1 + 32.0 * d2) + (0.03125 * d3 + m[7])]
                for i in range(nout):
                    h = ys[i]
                    obuf[base + i, r:r + RC, :] = (h * jnp.tanh(h) + h).astype(BF16)

        wcopy(0).wait()
        prep(0)
        z = tab[0]
        def kblock(kt, _):
            kcopy(kt).wait()
            wcopy(kt + 1).wait()
            prep(kt + 1)
            mm(kt, z)
            return 0
        jax.lax.fori_loop(0, NKT - 1, kblock, 0)
        jax.lax.fori_loop(0, z + 1, lambda i, c: kblock(NKT - 1, c), 0)
        kcopy(NKT).wait()
        def klast(i, _):
            mm(NKT)
            for u in range(NPRO - 1):
                output(u + z, pm[u])
            return 0
        jax.lax.fori_loop(0, z + 1, klast, 0)
        rcopy.wait()
        for c in range(CSP, xneed(0)):
            xcopy(c).wait()
        carry_u0(NPRO)

        def body(i, _):
            t0 = first(i)
            z = jnp.minimum(i, 0)
            zs = [0] + [jnp.minimum(i + gq, 0) for gq in range(1, 5)]
            for k in range(UPB):
                t = t0 + k
                dots(transform(t, k == 0, zs, i < 0), m_refs[k % NMB], z)
                output(t - 1, m_refs[(k - 1) % UPB % NMB])
            carry_u0(t0 + UPB)
            o0, o1 = tab[3 * i], tab[3 * i + 3]
            for k in range(MAXC):
                @pl.when(o0 + k < o1)
                def _():
                    ocopy(o0 + k).start()
            n0, n1 = tab[3 * i + 1], tab[3 * i + 4]
            for k in range(MAXC):
                @pl.when(jnp.logical_and(n0 + k < n1, n0 + k + LEAD < NCH))
                def _():
                    xcopy(n0 + k + LEAD).start()
            for k in range(MAXC):
                @pl.when(n0 + k < n1)
                def _():
                    xcopy(n0 + k).wait()
            f0, f1 = tab[3 * i + 2], tab[3 * i + 5]
            for k in range(MAXC):
                @pl.when(f0 + k < f1)
                def _():
                    ocopy(f0 + k).wait()
            return z
        z = jax.lax.fori_loop(0, NBODY - 1, body, jnp.int32(0))

        z = tab[0]
        zs = [0] + [jnp.minimum(z + gq, 0) for gq in range(1, 5)]
        never = z < 0
        ta, tb = NU - 2, NU - 1
        tile0 = (NB - 1) * SP
        slot0 = ((NB - 1) % 2) * SP
        lanes = pl.ds((NB - 1) * TB, TB)
        ecopies = []
        def mkecopy(s_lo, s_hi, rlo=0, rhi=C):
            cp = pltpu.make_async_copy(obuf.at[pl.ds(slot0 + s_lo, s_hi - s_lo), pl.ds(rlo, rhi - rlo), :],
                                       o_hbm.at[pl.ds(s_lo, s_hi - s_lo), pl.ds(rlo, rhi - rlo), lanes],
                                       sems.at[ES0 + len(ecopies)])
            ecopies.append(cp)
            return cp
        def ecopy(*args):
            mkecopy(*args).start()
        cdone = odone(NBODY - 2)
        s_a = (cdone - (NB - 1) * CPT) * CH
        s_b, s_c, s_d = MO * (ta - 1) - tile0, MO * ta - tile0, MO * tb - tile0
        pending = list(range(ofree(NBODY - 1), cdone))
        ecopy(s_a, s_b)
        e1 = mkecopy(s_b, s_c)
        e2 = mkecopy(s_c, s_d)
        JS = int(os.environ.get('JS', '4'))
        m42 = [m_refs[0] if j < JS else m_refs[1] for j in range(NP)]
        m43 = [m_refs[2] if j < JS else m_refs[0] for j in range(NP)]
        def last_a(i, _):
            output(ta - 1 + z, m_refs[1])
            dots(transform(ta + z, True, zs, never), m42, z)
            carry_u0(tb + z)
            @pl.when(i >= 0)
            def _():
                e1.start()
            return 0
        jax.lax.fori_loop(0, z + 1, last_a, 0)
        def last_b(i, _):
            output(ta + z, m42)
            dots(transform(tb + z, True, zs, never), m43, z, 0, C, (NP - 1,))
            @pl.when(i >= 0)
            def _():
                e2.start()
            return 0
        jax.lax.fori_loop(0, z + 1, last_b, 0)
        RP = C // NEP
        for e in range(NEP):
            output(tb, m43, e * RP, (e + 1) * RP, S - s_d)
            ecopy(s_d, S, e * RP, (e + 1) * RP)
        for c in pending:
            ocopy(c).wait()
        for cp in ecopies:
            cp.wait()

    any_spec = pl.BlockSpec(memory_space=pl.ANY)
    out = pl.pallas_call(
        kernel,
        in_specs=[any_spec] * 6,
        out_specs=any_spec,
        out_shape=jax.ShapeDtypeStruct((S, C, B), x.dtype),
        scratch_shapes=[pltpu.VMEM((NP, NKT + 1, C // 2, 128), U32),
                        pltpu.VMEM((C, 128), F32), pltpu.VMEM((C, 128), F32),
                        pltpu.VMEM((CF, TB), BF16),
                        pltpu.VMEM((3, C, C), BF16),
                        pltpu.VMEM((C,), BF16), pltpu.VMEM((C,), BF16), pltpu.VMEM((C,), BF16), pltpu.VMEM((C,), BF16),
                        pltpu.VMEM((RING + 2, C, TB), BF16), pltpu.VMEM((RING, C, TB), BF16),
                        pltpu.SemaphoreType.DMA((NSEM,)), pltpu.SMEM((3 * (NBODY + 1),), jnp.int32)]
                       + [pltpu.VMEM((NP, C, TB), F32) for _ in range(NMB + 1)],
        compiler_params=pltpu.CompilerParams(vmem_limit_bytes=100 * 1024 * 1024, disable_bounds_checks=True),
    )(xt, w, mean, var, g, b)
    return jnp.transpose(out, (2, 0, 1))
```

```python
import os
import jax, jax.numpy as jnp
import jax.experimental.pallas as pl
import jax.experimental.pallas.tpu as pltpu

TB = 128
UPB = int(os.environ.get("UPB", "2"))
RC = int(os.environ.get("RC", "16"))
JORD = [int(c) for c in os.environ.get("JORD", "01234567")]
NEP = int(os.environ.get("NEP", "4"))
TIE = int(os.environ.get("TIE", "1"))
KSP = int(os.environ.get("KSP", "0"))
ILV = int(os.environ.get("ILV", "1"))
GRP = [int(c) for c in os.environ.get("GRP", "01222")]
ZO = int(os.environ.get("ZO", "0"))
PTRIG = int(os.environ.get("PTRIG", "99"))
X2Z = int(os.environ.get("X2Z", "0"))
X2O = int(os.environ.get("X2O", "0"))
X2C = int(os.environ.get("X2C", "0"))
X2S = int(os.environ.get("X2S", "1"))
X2J = [int(c) for c in os.environ.get("X2J", "01234567")]
X1K = int(os.environ.get("X1K", "1"))
F32 = jnp.float32
BF16 = jnp.bfloat16
U32 = jnp.uint32

MO = 6
NP = MO + 2
CH = 8
NPRO = 2
CPK = {0: -2.25, 3: -0.025, 4: 0.075, 5: 0.8, 6: 2.4, 7: 2.25}


@jax.jit
def pallas_standalone__batchnorm__sampling_kernel(x, w, mean, var, g, b):
    B, S, C = x.shape
    xt = jnp.transpose(x, (1, 2, 0))
    NKT = C // 128
    CF = NKT * 128
    CR = C - CF
    SP = S + 1
    NB = B // TB
    NU = NB * SP // MO
    RING = 2 * SP
    UPR = RING // MO
    CPT = S // CH
    NCH = NB * CPT
    NMB = max(2, UPB if UPB % 2 else 2)
    NBODY = (NU - NPRO) // UPB
    assert (NU - NPRO) % UPB == 0
    LEAD = int(os.environ.get("LEAD", "3"))
    NSP = MO * NPRO + 1
    CSP = -(-NSP // CH)

    def chunk_of(p):
        if isinstance(p, int):
            return CPT * (p // SP) + min((p % SP) // CH, CPT - 1)
        return CPT * (p // SP) + jnp.minimum((p % SP) // CH, CPT - 1)

    first = lambda i: NPRO + UPB * i
    xneed = lambda i: chunk_of(MO * first(i + 1) + MO - 1) + 1
    def odone(i):
        p = MO * (first(i + 1) - 1)
        return CPT * (p // SP) + (p % SP) // CH
    def ofree(i):
        p = MO * (first(i + 1) - 1) - 1 - RING
        if isinstance(p, int):
            return 0 if p < 0 else chunk_of(p) + 1
        return jnp.where(p < 0, 0, chunk_of(jnp.maximum(p, 0)) + 1)
    MAXC = (MO * UPB + CH - 1) // CH + (1 if UPB > 2 else 0)
    assert odone(-1) == 0 and odone(NBODY - 1) == NCH - 1
    for i in range(NBODY):
        assert xneed(i + 1) - xneed(i) <= MAXC and odone(i) - odone(i - 1) <= MAXC
        assert ofree(i + 1) - ofree(i) <= MAXC and ofree(i + 1) <= odone(i - 1)
        cmax = min(xneed(i + 1) + LEAD, NCH) - 1 - 2 * CPT
        if cmax >= 0:
            assert SP * (cmax // CPT) + CH * (cmax % CPT) + CH - 1 < MO * first(i + 1) - 1
    assert xneed(0) + LEAD <= 2 * CPT

    STEP = MO * UPB

    def sched(q, r, n1, f1, mx=jnp.minimum, sel=jnp.where):
        o2 = CPT * q + (r >> 3)
        rn = r + STEP + 2 * MO - 1
        n2 = sel(rn >= SP, CPT * (q + 1) + mx((rn - SP) >> 3, CPT - 1), CPT * q + mx(rn >> 3, CPT - 1)) + 1
        rf = r + STEP - 1
        f2 = sel(rf >= SP, CPT * (q - 1) + ((rf - SP) >> 3), CPT * (q - 2) + mx(rf >> 3, CPT - 1)) + 1
        return o2, n1, mx(n2, NCH), f1, sel(f2 < 0, 0, f2)

    for i in range(NBODY - 2):
        p = MO * (first(i + 2) - 1)
        got = sched(p // SP, p % SP, min(xneed(i + 1), NCH), ofree(i + 1), min, lambda c, a, b: a if c else b)
        assert got == (odone(i + 1), min(xneed(i + 1), NCH), min(xneed(i + 2), NCH), ofree(i + 1), ofree(i + 2)), (i, got)

    XS0, OS0 = 0, 2 * CPT
    WS0 = 4 * CPT
    PS0 = WS0 + NKT + 1
    KS0 = PS0 + 4
    ES0 = KS0 + NKT + 2
    NSEM = ES0 + NEP + 4

    def kernel(x_hbm, w_hbm, mean_hbm, var_hbm, g_hbm, b_hbm, o_hbm,
               a_ref, sh_ref, hs_ref, u0_ref, wbuf, p0, p1, p2, p3, xbuf, obuf, sems, *m_refs):

        def hbm_chunk(ref, c):
            lane0 = (c >> 2) * TB
            if not isinstance(c, int):
                lane0 = pl.multiple_of(lane0, TB)
            return ref.at[pl.ds((c & 3) * CH, CH), :, pl.ds(lane0, TB)]

        def ring_slot(c):
            return ((c >> 2) & 1) * SP + (c & 3) * CH

        def xcopy(c):
            return pltpu.make_async_copy(hbm_chunk(x_hbm, c), xbuf.at[pl.ds(ring_slot(c) + 1, CH)],
                                         sems.at[XS0 + (c & 7)])

        def ocopy(c):
            return pltpu.make_async_copy(obuf.at[pl.ds(ring_slot(c), CH)], hbm_chunk(o_hbm, c),
                                         sems.at[OS0 + (c & 7)])

        def krows(kt):
            if isinstance(kt, int):
                return pl.ds(kt * 128, 128 if kt < NKT else CR)
            return pl.ds(pl.multiple_of(kt * 128, 128), 128)

        def wcopy(kt):
            return pltpu.make_async_copy(w_hbm.at[:, krows(kt), :], wbuf.at[:, krows(kt), :], sems.at[WS0 + kt])

        def kcopy(kt):
            return pltpu.make_async_copy(x_hbm.at[pl.ds(0, NSP), krows(kt), pl.ds(0, TB)],
                                         xbuf.at[pl.ds(1, NSP), krows(kt), :], sems.at[KS0 + kt])
        rcopy = pltpu.make_async_copy(x_hbm.at[pl.ds(NSP, CSP * CH - NSP), :, pl.ds(0, TB)],
                                      xbuf.at[pl.ds(1 + NSP, CSP * CH - NSP)], sems.at[KS0 + NKT + 1])

        pcopies = [pltpu.make_async_copy(s, d, sems.at[PS0 + i])
                   for i, (s, d) in enumerate(zip((mean_hbm, var_hbm, g_hbm, b_hbm), (p0, p1, p2, p3)))]
        for c in pcopies:
            c.start()
        for kt in range(NKT + 1):
            wcopy(kt).start()
            kcopy(kt).start()
        rcopy.start()
        for c in range(CSP, xneed(0) + LEAD):
            xcopy(c).start()

        pm = [m_refs[(UPB - NPRO + u) % NMB] for u in range(NPRO)]
        for r in pm:
            r[...] = jnp.zeros(r.shape, F32)
        for s in (0, SP, RING, RING + 1):
            xbuf[s] = jnp.zeros((C, TB), BF16)

        for c in pcopies:
            c.wait()
        mean_, var_, g_, b_ = [r[...].astype(F32).reshape(1, C) for r in (p0, p1, p2, p3)]
        scale = g_ * jax.lax.rsqrt(var_ + 1e-5)
        hs_ref[0:C, :] = jnp.broadcast_to(0.5 * scale, (128, C)).T
        sh = 0.5 * (b_ - mean_ * scale)
        sh_hi = sh.astype(BF16).astype(F32)
        sh_mid = (sh - sh_hi).astype(BF16).astype(F32)
        sh_lo = (sh - sh_hi) - sh_mid
        row = jax.lax.broadcasted_iota(jnp.int32, (128, C), 0)
        sh_ref[0:C, :] = jnp.where(row == CR, sh_hi, jnp.where(row == CR + 1, sh_mid, jnp.where(row == CR + 2, sh_lo, 0.0))).T

        def prep(kt):
            last = isinstance(kt, int) and kt == NKT
            lo = jax.lax.broadcasted_iota(jnp.int32, (8, 128), 1) < CR
            for r in range(0, C // 2, 8):
                if r % 64 == 0:
                    cols = slice(2 * r, min(2 * r + 128, C))
                    if last:
                        wts = [jnp.concatenate([wbuf[k, CF:C, cols], wbuf[k, CF:C, cols]], axis=0).T for k in range(3)]
                    else:
                        wts = [wbuf[k, krows(kt), cols].T for k in range(3)]
                    wu = [pltpu.bitcast(t, U32) for t in wts]
                rr = r % 64
                halves = []
                for h in range(2):
                    hs = hs_ref[pl.ds(2 * r + h, 8, stride=2), :]
                    w0, w1, w2 = [pltpu.unpack_elementwise(t[rr:rr + 8, :], index=h, packed_dtype=BF16, unpacked_dtype=F32) * hs
                                  for t in wu]
                    e1, o1 = (-2.0 / 9) * (w0 + w2), (-2.0 / 9) * w1
                    e2, o2 = (1.0 / 90) * w0 + (2.0 / 45) * w2, (1.0 / 45) * w1
                    e3, o3 = (32.0 / 45) * w0 + (8.0 / 45) * w2, (16.0 / 45) * w1
                    gs = [w0, e1 + o1, e1 - o1, e2 + o2, e2 - o2, e3 + o3, e3 - o3, w2]
                    if last:
                        ext = dict((j, c * gs[2]) for j, c in CPK.items())
                        ext[1] = sh_ref[pl.ds(2 * r + h, 8, stride=2), :]
                        gs = [jnp.where(lo, gs[j], ext[j]) if j != 2 else None for j in range(NP)]
                    halves.append(gs)
                for j in range(NP):
                    if halves[0][j] is not None:
                        a_ref[j, kt, r:r + 8, :] = pltpu.pack_elementwise([halves[0][j], halves[1][j]], packed_dtype=BF16)

        def tchunk(ld, with_u0=True):
            d1, d2, d3, d4, d5, d6 = [ld(i, 1) for i in range(1, 7)]
            e1, o1 = (d2 + d6) - 4.25 * d4, (d1 + d5) - 4.25 * d3
            d1, d2, d3, d4, d5, d6 = [ld(i, 2) for i in range(1, 7)]
            e2, o2 = (d6 - d4) - 0.25 * (d4 - d2), 2.0 * (d5 - d3) - 0.5 * (d3 - d1)
            d1, d2, d3, d4, d5, d6 = [ld(i, 3) for i in range(1, 7)]
            e3, o3 = (d6 - d4) - 4.0 * (d4 - d2), 0.5 * (d5 - d3) - 2.0 * (d3 - d1)
            d1, d3, d5, d7 = [ld(i, 4) for i in (1, 3, 5, 7)]
            u = [None, e1 + o1, e1 - o1, e2 + o2, e2 - o2, e3 + o3, e3 - o3, (d7 - d1) - 5.25 * (d5 - d3)]
            if with_u0:
                d0, d2, d4, d6 = [ld(i, 0) for i in (0, 2, 4, 6)]
                u[0] = (d0 - d6) + 5.25 * (d4 - d2)
            return u

        def ones_rows():
            return (jax.lax.broadcasted_iota(jnp.int32, (CR, TB), 0) < 3).astype(F32)

        def mm(kt, z=0):
            last = isinstance(kt, int) and kt == NKT
            r0 = kt * 128 if isinstance(kt, int) else pl.multiple_of(kt * 128, 128)
            for u in range(NPRO):
                cs = [tchunk(lambda i, gi: xbuf[MO * u + i, pl.ds(r0 + r, RC), :].astype(F32))
                      for r in range(0, CR if last else 128, RC)]
                for j in range(NP):
                    parts = [c[j] for c in cs]
                    if last:
                        if j == 2:
                            continue
                        parts = parts + ([ones_rows()] if j == 1 else [c[2] for c in cs])
                    rhs = jnp.concatenate(parts, axis=0).astype(BF16)
                    zz = z if u * NP + j >= PTRIG else 0
                    pm[u][j] += jnp.dot(pltpu.bitcast(a_ref[j + zz, kt], BF16), rhs, preferred_element_type=F32)

        def carry_u0(t):
            base = (t % UPR) * MO
            for r in range(0, CF, RC):
                d0, d2, d4, d6 = [xbuf[base + i, r:r + RC, :].astype(F32) for i in (0, 2, 4, 6)]
                u0_ref[r:r + RC, :] = ((d0 - d6) + 5.25 * (d4 - d2)).astype(BF16)

        def transform(t, carried, zs, never):
            base = (t % UPR) * MO
            if not ILV:
                cs = [tchunk(lambda i, gi: xbuf[base + zs[gi] + i, r:r + RC, :].astype(F32), not (carried and r < CF))
                      for r in range(0, C, RC)]
                tail = [c[2] for c in cs[CF // RC:]]
                out = []
                for j in range(NP):
                    parts = [c[j] for c in cs if c[j] is not None]
                    if j == 2:
                        parts = parts[:CF // RC]
                    else:
                        parts = parts + ([ones_rows()] if j == 1 else tail)
                    v = jnp.concatenate(parts, axis=0).astype(BF16)
                    if j == 0 and carried:
                        v = jnp.concatenate([u0_ref[...], v], axis=0)
                    out.append(v)
                return out
            cs = []
            for r in range(0, C, RC):
                hv = []
                for h in range(2):
                    ld = lambda i, gi: pltpu.unpack_elementwise(
                        pltpu.bitcast(xbuf[base + zs[GRP[gi]] + i, r:r + RC, :], U32), index=h, packed_dtype=BF16, unpacked_dtype=F32)
                    hv.append(tchunk(ld, not (carried and r < CF)))
                c = [None if hv[0][j] is None else pltpu.pack_elementwise([hv[0][j], hv[1][j]], packed_dtype=BF16) for j in range(NP)]
                if TIE:
                    gof = [GRP[q] for q in (0, 1, 1, 2, 2, 3, 3, 4)]
                    for gid in sorted(set(GRP)):
                        mem = [j for j in JORD if gof[j] == gid and c[j] is not None]
                        if len(mem) > 1:
                            acc = c[mem[1]]
                            for j in mem[2:]:
                                acc = acc ^ c[j]
                            c[mem[0]] = jnp.where(never, acc, c[mem[0]])
                cs.append(c)
            tail = [c[2] for c in cs[CF // RC:]]
            ones = pltpu.bitcast(ones_rows().astype(BF16), U32)
            out = []
            for j in range(NP):
                parts = [c[j] for c in cs if c[j] is not None]
                if j == 2:
                    parts = parts[:CF // RC]
                else:
                    parts = parts + ([ones] if j == 1 else tail)
                v = pltpu.bitcast(jnp.concatenate(parts, axis=0), BF16)
                if j == 0 and carried:
                    v = jnp.concatenate([u0_ref[...], v], axis=0)
                out.append(v)
            return out

        def dots(us, m_ref, z, rlo=0, rhi=C, skip=(), jord=JORD):
            lhs = lambda j, k0, k1: pltpu.bitcast(jnp.concatenate([a_ref[j, kt, rlo // 2:rhi // 2, :] for kt in range(k0, k1)], axis=1), BF16)
            if not KSP:
                for j in jord:
                    if j in skip:
                        continue
                    nk = NKT if j == 2 else NKT + 1
                    (m_ref[j] if isinstance(m_ref, list) else m_ref)[j + z, rlo:rhi, :] = jnp.dot(lhs(j, 0, nk), us[j], preferred_element_type=F32)
                return
            for grp in ((0,), (1, 2), (3, 4), (5, 6), (7,)):
                acc = {}
                step = KSP if len(grp) > 1 else NKT + 1
                for k0 in range(0, NKT + 1, step):
                    for j in grp:
                        nk = NKT if j == 2 else NKT + 1
                        k1 = min(k0 + step, nk)
                        if k1 <= k0:
                            continue
                        p = jnp.dot(lhs(j, k0, k1), us[j][k0 * 128:k1 * 128], preferred_element_type=F32)
                        acc[j] = p if j not in acc else acc[j] + p
                for j in grp:
                    m_ref[j + z] = acc[j]

        def output(t, m_ref, rlo=0, rhi=C, nout=MO):
            base = (t % UPR) * MO
            for r in range(rlo, rhi, RC):
                m = [(m_ref[j] if isinstance(m_ref, list) else m_ref)[j, r:r + RC, :] if (j < NP - 1 or nout == MO) else 0.0 for j in range(NP)]
                s1, s2, s3 = m[1] + m[2], m[3] + m[4], m[5] + m[6]
                d1, d2, d3 = m[1] - m[2], m[3] - m[4], m[5] - m[6]
                ys = [(m[0] + s1) + (s2 + s3),
                      (d1 + 2.0 * d2) + 0.5 * d3,
                      (s1 + 4.0 * s2) + 0.25 * s3,
                      (d1 + 8.0 * d2) + 0.125 * d3,
                      (s1 + 16.0 * s2) + 0.0625 * s3,
                      (d1 + 32.0 * d2) + (0.03125 * d3 + m[7])]
                for i in range(nout):
                    h = ys[i]
                    obuf[base + i, r:r + RC, :] = (h * jnp.tanh(h) + h).astype(BF16)

        wcopy(0).wait()
        prep(0)
        def kblock(kt, _):
            kcopy(kt).wait()
            wcopy(kt + 1).wait()
            prep(kt + 1)
            mm(kt)
            return jnp.minimum(kt, 0)
        z = jax.lax.fori_loop(0, NKT - 1, kblock, jnp.int32(0))
        jax.lax.fori_loop(0, z + 1, lambda i, c: kblock(NKT - 1, c), jnp.int32(0))
        kcopy(NKT).wait()
        def klast(i, _):
            mm(NKT)
            for u in range(NPRO - 1):
                output(u + z, pm[u])
            return 0
        jax.lax.fori_loop(0, z + 1, klast, 0)
        rcopy.wait()
        for c in range(CSP, xneed(0)):
            xcopy(c).wait()
        carry_u0(NPRO)

        def body(i, carry):
            o0, o1, n0, n1, f0, f1, q, r = carry
            t0 = first(i)
            z = jnp.minimum(i, 0)
            zs = [0] + [jnp.minimum(i + gq, 0) for gq in range(1, 5)]
            for k in range(UPB):
                t = t0 + k
                dots(transform(t, k == 0, zs, i < 0), m_refs[k % NMB], z)
                output(t - 1, m_refs[(k - 1) % UPB % NMB])
            carry_u0(t0 + UPB)
            for k in range(MAXC):
                @pl.when(o0 + k < o1)
                def _():
                    ocopy(o0 + k).start()
            for k in range(MAXC):
                @pl.when(jnp.logical_and(n0 + k < n1, n0 + k + LEAD < NCH))
                def _():
                    xcopy(n0 + k + LEAD).start()
            for k in range(MAXC):
                @pl.when(n0 + k < n1)
                def _():
                    xcopy(n0 + k).wait()
            for k in range(MAXC):
                @pl.when(f0 + k < f1)
                def _():
                    ocopy(f0 + k).wait()
            wrap = r + STEP >= SP
            return (o1,) + sched(q, r, n1, f1) + (q + wrap.astype(jnp.int32), jnp.where(wrap, r + STEP - SP, r + STEP))
        p1 = MO * (first(2) - 1)
        init = (odone(-1), odone(0), xneed(0), xneed(1), ofree(0), ofree(1), p1 // SP, p1 % SP)
        fin = jax.lax.fori_loop(0, NBODY - 1, body, tuple(jnp.int32(v) for v in init))
        z = jnp.minimum(fin[0], 0)

        zs = [0] + [jnp.minimum(z + gq, 0) for gq in range(1, 5)]
        never = z < 0
        ta, tb = NU - 2, NU - 1
        tile0 = (NB - 1) * SP
        slot0 = ((NB - 1) % 2) * SP
        lanes = pl.ds((NB - 1) * TB, TB)
        ecopies = []
        def mkecopy(s_lo, s_hi, rlo=0, rhi=C):
            cp = pltpu.make_async_copy(obuf.at[pl.ds(slot0 + s_lo, s_hi - s_lo), pl.ds(rlo, rhi - rlo), :],
                                       o_hbm.at[pl.ds(s_lo, s_hi - s_lo), pl.ds(rlo, rhi - rlo), lanes],
                                       sems.at[ES0 + len(ecopies)])
            ecopies.append(cp)
            return cp
        def ecopy(*args):
            mkecopy(*args).start()
        cdone = odone(NBODY - 2)
        s_a = (cdone - (NB - 1) * CPT) * CH
        s_b, s_c, s_d = MO * (ta - 1) - tile0, MO * ta - tile0, MO * tb - tile0
        pending = list(range(ofree(NBODY - 1), cdone))
        ecopy(s_a, s_b)
        e1 = mkecopy(s_b, s_c)
        e2 = mkecopy(s_c, s_d)
        JS = int(os.environ.get('JS', '4'))
        m42 = [m_refs[0] if j < JS else m_refs[1] for j in range(NP)]
        JS2 = int(os.environ.get('JS2', JS))
        m43 = [m_refs[2] if j < JS2 else (m_refs[0] if j >= JS else m_refs[1]) for j in range(NP)]
        def last_a(i, _):
            output(ta - 1 + z, m_refs[1])
            dots(transform(ta + z, True, zs, never), m42, z)
            if X2C or X1K:
                carry_u0(tb + z)
            @pl.when(i >= 0)
            def _():
                e1.start()
            return 0
        jax.lax.fori_loop(0, z + 1, last_a, 0)
        def last_b(i, _):
            zb = jnp.minimum(i, 0) if X2Z else z
            zsb = [0] + [jnp.minimum(zb + gq, 0) for gq in range(1, 5)]
            if X2O == 0:
                output(ta + zb, m42)
            dots(transform(tb + zb, bool(X2C), zsb, zb < 0), m43, zb, 0, C, (NP - 1,) if X2S else (), X2J)
            if X2O == 1:
                output(ta + zb, m42)
            @pl.when(i >= 0)
            def _():
                e2.start()
            return 0
        jax.lax.fori_loop(0, z + 1, last_b, 0)
        RP = C // NEP
        for e in range(NEP):
            output(tb, m43, e * RP, (e + 1) * RP, S - s_d)
            ecopy(s_d, S, e * RP, (e + 1) * RP)
        for c in pending:
            ocopy(c).wait()
        for cp in ecopies:
            cp.wait()

    any_spec = pl.BlockSpec(memory_space=pl.ANY)
    out = pl.pallas_call(
        kernel,
        in_specs=[any_spec] * 6,
        out_specs=any_spec,
        out_shape=jax.ShapeDtypeStruct((S, C, B), x.dtype),
        scratch_shapes=[pltpu.VMEM((NP, NKT + 1, C // 2, 128), U32),
                        pltpu.VMEM((C + 8, 128), F32), pltpu.VMEM((C + 8, 128), F32),
                        pltpu.VMEM((CF, TB), BF16),
                        pltpu.VMEM((3, C, C), BF16),
                        pltpu.VMEM((C,), BF16), pltpu.VMEM((C,), BF16), pltpu.VMEM((C,), BF16), pltpu.VMEM((C,), BF16),
                        pltpu.VMEM((RING + 2, C, TB), BF16), pltpu.VMEM((RING, C, TB), BF16),
                        pltpu.SemaphoreType.DMA((NSEM,))]
                       + [pltpu.VMEM((NP, C, TB), F32) for _ in range(NMB + 1)],
        compiler_params=pltpu.CompilerParams(vmem_limit_bytes=100 * 1024 * 1024, disable_bounds_checks=True),
    )(xt, w, mean, var, g, b)
    return jnp.transpose(out, (2, 0, 1))
```

```python
import jax
import jax.numpy as jnp
import jax.experimental.pallas as pl
import jax.experimental.pallas.tpu as pltpu

F32 = jnp.float32
BF16 = jnp.bfloat16
U32 = jnp.uint32

TB = 128
MO = 6
NP = MO + 2
UPB = 2
NPRO = 2
RC = 16
CH = 8
LEAD = 3
NEP = 4
JS = 4
EPS = 1e-5
CPK = {0: -2.25, 3: -0.025, 4: 0.075, 5: 0.8, 6: 2.4, 7: 2.25}


@jax.jit
def pallas_standalone__batchnorm__sampling_kernel(
    x: jax.Array,
    w: jax.Array,
    mean: jax.Array,
    var: jax.Array,
    g: jax.Array,
    b: jax.Array,
):
    B, S, C = x.shape
    NKT = C // 128
    CF = NKT * 128
    CR = C - CF
    SP = S + 1
    NB = B // TB
    NU = NB * SP // MO
    RING = 2 * SP
    UPR = RING // MO
    CPT = S // CH
    NCH = NB * CPT
    NBODY = (NU - NPRO) // UPB
    STEP = MO * UPB
    NSP = MO * NPRO + 1
    CSP = -(-NSP // CH)
    assert w.shape == (3, C, C) and 2 * CR == 128 and CPT == 4 and CH == 8
    assert NB * TB == B and NU * MO == NB * SP and UPR * MO == RING and NBODY * UPB == NU - NPRO

    chunk_of = lambda p: CPT * (p // SP) + min((p % SP) // CH, CPT - 1)
    first = lambda i: NPRO + UPB * i
    xneed = lambda i: min(chunk_of(MO * first(i + 1) + MO - 1) + 1, NCH)

    def odone(i):
        p = MO * (first(i + 1) - 1)
        return CPT * (p // SP) + (p % SP) // CH

    def ofree(i):
        p = MO * (first(i + 1) - 1) - 1 - RING
        return 0 if p < 0 else chunk_of(p) + 1

    def sched(q, r, mx=jnp.minimum, sel=jnp.where):
        rn = r + STEP + 2 * MO - 1
        n2 = sel(rn >= SP, CPT * (q + 1) + mx((rn - SP) >> 3, CPT - 1), CPT * q + mx(rn >> 3, CPT - 1)) + 1
        rf = r + STEP - 1
        f2 = sel(rf >= SP, CPT * (q - 1) + ((rf - SP) >> 3), CPT * (q - 2) + mx(rf >> 3, CPT - 1)) + 1
        return CPT * q + (r >> 3), mx(n2, NCH), sel(f2 < 0, 0, f2)

    MAXC = 2
    assert odone(-1) == 0 and xneed(0) + LEAD <= 2 * CPT and xneed(NBODY - 1) == NCH
    for i in range(NBODY - 1):
        assert max(xneed(i + 1) - xneed(i), odone(i) - odone(i - 1), ofree(i + 1) - ofree(i)) <= MAXC <= LEAD
        assert ofree(i + 1) <= odone(i - 1)
        old = min(xneed(i + 1) + LEAD, NCH) - 1 - 2 * CPT
        assert old < 0 or SP * (old // CPT) + CH * (old % CPT) + CH - 1 < MO * first(i + 1) - 1
        p = MO * (first(i + 2) - 1)
        assert i == NBODY - 2 or (sched(p // SP, p % SP, min, lambda c, u, v: u if c else v)
                                  == (odone(i + 1), xneed(i + 2), ofree(i + 2)))

    XS0, OS0, WS0 = 0, 2 * CPT, 4 * CPT
    PS0 = WS0 + NKT + 1
    KS0 = PS0 + 4
    ES0 = KS0 + NKT + 3
    NSEM = ES0 + 3 + NEP

    def kernel(x_hbm, w_hbm, mean_hbm, var_hbm, g_hbm, b_hbm, o_hbm,
               a_ref, sh_ref, hs_ref, u0_ref, wbuf, p0, p1, p2, p3, xbuf, obuf, sems,
               ma_ref, mb_ref, mc_ref):

        def hbm_chunk(ref, c):
            lane0 = (c >> 2) * TB
            if not isinstance(c, int):
                lane0 = pl.multiple_of(lane0, TB)
            return ref.at[pl.ds((c & 3) * CH, CH), :, pl.ds(lane0, TB)]

        def ring_slot(c):
            return ((c >> 2) & 1) * SP + (c & 3) * CH

        def xcopy(c):
            return pltpu.make_async_copy(hbm_chunk(x_hbm, c), xbuf.at[pl.ds(ring_slot(c) + 1, CH)],
                                         sems.at[XS0 + (c & 7)])

        def ocopy(c):
            return pltpu.make_async_copy(obuf.at[pl.ds(ring_slot(c), CH)], hbm_chunk(o_hbm, c),
                                         sems.at[OS0 + (c & 7)])

        def krows(kt):
            if isinstance(kt, int):
                return pl.ds(kt * 128, 128 if kt < NKT else CR)
            return pl.ds(pl.multiple_of(kt * 128, 128), 128)

        def wcopy(kt):
            return pltpu.make_async_copy(w_hbm.at[:, krows(kt), :], wbuf.at[:, krows(kt), :],
                                         sems.at[WS0 + kt])

        def kcopy(kt, lo=0, hi=NSP, sem=None):
            return pltpu.make_async_copy(x_hbm.at[pl.ds(lo, hi - lo), krows(kt), pl.ds(0, TB)],
                                         xbuf.at[pl.ds(1 + lo, hi - lo), krows(kt), :],
                                         sems.at[KS0 + kt if sem is None else sem])

        k0a_copy = kcopy(0, 0, MO + 1)
        k0b_copy = kcopy(0, MO + 1, NSP, KS0 + NKT + 1)
        rcopy = pltpu.make_async_copy(x_hbm.at[pl.ds(NSP, CSP * CH - NSP), :, pl.ds(0, TB)],
                                      xbuf.at[pl.ds(1 + NSP, CSP * CH - NSP)], sems.at[KS0 + NKT + 2])
        pcopies = [pltpu.make_async_copy(s, d, sems.at[PS0 + i])
                   for i, (s, d) in enumerate(zip((mean_hbm, var_hbm, g_hbm, b_hbm), (p0, p1, p2, p3)))]
        for c in pcopies:
            c.start()
        wcopy(0).start()
        k0a_copy.start()
        wcopy(1).start()
        k0b_copy.start()
        kcopy(1).start()
        for kt in range(2, NKT + 1):
            wcopy(kt).start()
            kcopy(kt).start()
        rcopy.start()
        for c in range(CSP, xneed(0) + LEAD):
            xcopy(c).start()

        for s in (0, SP, RING, RING + 1):
            xbuf[s] = jnp.zeros((C, TB), BF16)

        for c in pcopies:
            c.wait()
        mean_, var_, g_, b_ = [r[...].astype(F32).reshape(1, C) for r in (p0, p1, p2, p3)]
        scale = g_ * jax.lax.rsqrt(var_ + EPS)
        hs_ref[0:C, :] = jnp.broadcast_to(0.5 * scale, (128, C)).T
        sh = 0.5 * (b_ - mean_ * scale)
        sh_hi = sh.astype(BF16).astype(F32)
        sh_mid = (sh - sh_hi).astype(BF16).astype(F32)
        sh_lo = (sh - sh_hi) - sh_mid
        row = jax.lax.broadcasted_iota(jnp.int32, (128, C), 0)
        sh_ref[0:C, :] = jnp.where(row == CR, sh_hi, jnp.where(
            row == CR + 1, sh_mid, jnp.where(row == CR + 2, sh_lo, 0.0))).T

        def prep(kt):
            last = isinstance(kt, int) and kt == NKT
            lo = jax.lax.broadcasted_iota(jnp.int32, (8, 128), 1) < CR
            for r in range(0, C // 2, 8):
                if r % 64 == 0:
                    cols = slice(2 * r, min(2 * r + 128, C))
                    if last:
                        wts = [jnp.concatenate([wbuf[k, CF:C, cols]] * 2, axis=0).T for k in range(3)]
                    else:
                        wts = [wbuf[k, krows(kt), cols].T for k in range(3)]
                    wu = [pltpu.bitcast(t, U32) for t in wts]
                rr = r % 64
                halves = []
                for h in range(2):
                    hs = hs_ref[pl.ds(2 * r + h, 8, stride=2), :]
                    r0, r1, r2 = [pltpu.unpack_elementwise(t[rr:rr + 8, :], index=h, packed_dtype=BF16,
                                                           unpacked_dtype=F32) for t in wu]
                    w0, w1, w2 = r0 * hs, r1 * hs, r2 * hs
                    e1, o1 = (-2.0 / 9) * (w0 + w2), (-2.0 / 9) * w1
                    e2, o2 = (1.0 / 90) * w0 + (2.0 / 45) * w2, (1.0 / 45) * w1
                    e3, o3 = (32.0 / 45) * w0 + (8.0 / 45) * w2, (16.0 / 45) * w1
                    gs = [r0, e1 + o1, e1 - o1, e2 + o2, e2 - o2, e3 + o3, e3 - o3, r2]
                    if last:
                        ext = dict((j, c * gs[2]) for j, c in CPK.items())
                        raw2 = (r0 + r2) - r1
                        ext[0], ext[7] = (-2.0 / 9 * CPK[0]) * raw2, (-2.0 / 9 * CPK[7]) * raw2
                        ext[1] = sh_ref[pl.ds(2 * r + h, 8, stride=2), :]
                        gs = [jnp.where(lo, gs[j], ext[j]) if j != 2 else None for j in range(NP)]
                    halves.append(gs)
                for j in range(NP):
                    if not last and j in (0, NP - 1):
                        a_ref[j, kt, r:r + 8, :] = wu[0 if j == 0 else 2][rr:rr + 8, :]
                    elif halves[0][j] is not None:
                        a_ref[j, kt, r:r + 8, :] = pltpu.pack_elementwise(
                            [halves[0][j], halves[1][j]], packed_dtype=BF16)

        def tchunk(ld, with_u0=True):
            d1, d2, d3, d4, d5, d6 = [ld(i, 1) for i in range(1, 7)]
            e1, o1 = (d2 + d6) - 4.25 * d4, (d1 + d5) - 4.25 * d3
            d1, d2, d3, d4, d5, d6, d7 = [ld(i, 2) for i in range(1, 8)]
            e2, o2 = (d6 - d4) - 0.25 * (d4 - d2), 2.0 * (d5 - d3) - 0.5 * (d3 - d1)
            e3, o3 = (d6 - d4) - 4.0 * (d4 - d2), 0.5 * (d5 - d3) - 2.0 * (d3 - d1)
            u = [None, e1 + o1, e1 - o1, e2 + o2, e2 - o2, e3 + o3, e3 - o3, (d7 - d1) - 5.25 * (d5 - d3)]
            if with_u0:
                d0, d2, d4, d6 = [ld(i, 0) for i in (0, 2, 4, 6)]
                u[0] = (d0 - d6) + 5.25 * (d4 - d2)
            return u

        def ones_rows():
            return (jax.lax.broadcasted_iota(jnp.int32, (CR, TB), 0) < 3).astype(F32)

        def carry_u0(t):
            base = (t % UPR) * MO
            for r in range(0, CF, RC):
                d0, d2, d4, d6 = [xbuf[base + i, r:r + RC, :].astype(F32) for i in (0, 2, 4, 6)]
                u0_ref[r:r + RC, :] = ((d0 - d6) + 5.25 * (d4 - d2)).astype(BF16)

        def transform(t, carried, zs, never):
            base = (t % UPR) * MO
            cs = []
            for r in range(0, C, RC):
                hv = []
                for h in range(2):
                    ld = lambda i, gi: pltpu.unpack_elementwise(
                        pltpu.bitcast(xbuf[base + zs[gi] + i, r:r + RC, :], U32),
                        index=h, packed_dtype=BF16, unpacked_dtype=F32)
                    hv.append(tchunk(ld, not (carried and r < CF)))
                c = [None if hv[0][j] is None else
                     pltpu.pack_elementwise([hv[0][j], hv[1][j]], packed_dtype=BF16) for j in range(NP)]
                c[1] = jnp.where(never, c[2], c[1])
                c[3] = jnp.where(never, c[4] ^ c[5] ^ c[6] ^ c[7], c[3])
                cs.append(c)
            tail = [c[2] for c in cs[CF // RC:]]
            ones = pltpu.bitcast(ones_rows().astype(BF16), U32)
            us = []
            for j in range(NP):
                parts = [c[j] for c in cs if c[j] is not None]
                if j == 2:
                    parts = parts[:CF // RC]
                else:
                    parts = parts + ([ones] if j == 1 else tail)
                v = pltpu.bitcast(jnp.concatenate(parts, axis=0), BF16)
                if j == 0 and carried:
                    v = jnp.concatenate([u0_ref[...], v], axis=0)
                us.append(v)
            return us

        def dots(us, ms, z, nprod=NP):
            for j in range(nprod):
                nk = NKT if j == 2 else NKT + 1
                lhs = pltpu.bitcast(jnp.concatenate([a_ref[j, kt] for kt in range(nk)], axis=1), BF16)
                ms[j][j + z, 0:C, :] = jnp.dot(lhs, us[j], preferred_element_type=F32)

        def output(t, ms, rlo=0, rhi=C, nout=MO):
            base = (t % UPR) * MO
            for r in range(rlo, rhi, RC):
                m = [ms[j][j, r:r + RC, :] if (j < NP - 1 or nout == MO) else 0.0 for j in range(NP)]
                s1, s2, s3 = m[1] + m[2], m[3] + m[4], m[5] + m[6]
                d1, d2, d3 = m[1] - m[2], m[3] - m[4], m[5] - m[6]
                hs = hs_ref[r:r + RC, :]
                ys = [(hs * m[0] + s1) + (s2 + s3),
                      (d1 + 2.0 * d2) + 0.5 * d3,
                      (s1 + 4.0 * s2) + 0.25 * s3,
                      (d1 + 8.0 * d2) + 0.125 * d3,
                      (s1 + 16.0 * s2) + 0.0625 * s3,
                      (d1 + 32.0 * d2) + (0.03125 * d3 + hs * m[7])]
                for i in range(nout):
                    h = ys[i]
                    obuf[base + i, r:r + RC, :] = (h * jnp.tanh(h) + h).astype(BF16)

        msa, msb = [ma_ref] * NP, [mb_ref] * NP

        def once(z, fn):
            def trip(i, c):
                fn(i)
                return c
            jax.lax.fori_loop(0, z + 1, trip, 0)

        def mm(kt, units=(0, 1)):
            last = isinstance(kt, int) and kt == NKT
            r0 = kt * 128 if isinstance(kt, int) else pl.multiple_of(kt * 128, 128)
            for u in units:
                m_ref = (ma_ref, mb_ref)[u]
                cs = [tchunk(lambda i, gi: xbuf[MO * u + i, pl.ds(r0 + r, RC), :].astype(F32))
                      for r in range(0, CR if last else 128, RC)]
                for j in range(NP):
                    parts = [c[j] for c in cs]
                    if last:
                        if j == 2:
                            continue
                        parts = parts + ([ones_rows()] if j == 1 else [c[2] for c in cs])
                    rhs = jnp.concatenate(parts, axis=0).astype(BF16)
                    p = jnp.dot(pltpu.bitcast(a_ref[j, kt], BF16), rhs, preferred_element_type=F32)
                    m_ref[j] = p if isinstance(kt, int) and kt == 0 else m_ref[j] + p

        def kblock(kt, c):
            kcopy(kt).wait()
            wcopy(kt + 1).wait()
            prep(kt + 1)
            mm(kt)
            return c

        wcopy(0).wait()
        prep(0)
        z = jax.lax.fori_loop(0, 2, lambda i, c: jnp.minimum(i, c), jnp.int32(0))
        k0a_copy.wait()
        once(z, lambda i: mm(0, (0,)))
        wcopy(1).wait()
        k0b_copy.wait()
        once(z, lambda i: (prep(1), mm(0, (1,))))
        jax.lax.fori_loop(1, NKT - 1, kblock, 0)
        once(z, lambda i: kblock(NKT - 1, 0))
        kcopy(NKT).wait()
        once(z, lambda i: (mm(NKT), output(z, msa)))
        rcopy.wait()
        for c in range(CSP, xneed(0)):
            xcopy(c).wait()
        carry_u0(NPRO)

        def body(i, carry):
            o0, o1, n0, n1, f0, f1, q, r = carry
            t0 = first(i)
            z = jnp.minimum(i, 0)
            zs = [0, jnp.minimum(i + 1, 0), jnp.minimum(i + 2, 0)]
            dots(transform(t0, True, zs, i < 0), msa, z)
            output(t0 - 1, msb)
            dots(transform(t0 + 1, False, zs, i < 0), msb, z)
            output(t0, msa)
            carry_u0(t0 + UPB)
            for k in range(MAXC):
                @pl.when(o0 + k < o1)
                def _():
                    ocopy(o0 + k).start()
            for k in range(MAXC):
                @pl.when(jnp.logical_and(n0 + k < n1, n0 + k + LEAD < NCH))
                def _():
                    xcopy(n0 + k + LEAD).start()
            for k in range(MAXC):
                @pl.when(n0 + k < n1)
                def _():
                    xcopy(n0 + k).wait()
            for k in range(MAXC):
                @pl.when(f0 + k < f1)
                def _():
                    ocopy(f0 + k).wait()
            o2, n2, f2 = sched(q, r)
            wrap = r + STEP >= SP
            return (o1, o2, n1, n2, f1, f2, q + wrap.astype(jnp.int32),
                    jnp.where(wrap, r + STEP - SP, r + STEP))

        p1 = MO * (first(2) - 1)
        init = (odone(-1), odone(0), xneed(0), xneed(1), ofree(0), ofree(1), p1 // SP, p1 % SP)
        fin = jax.lax.fori_loop(0, NBODY - 1, body, tuple(jnp.int32(v) for v in init))

        z = jnp.minimum(fin[0], 0)
        zs = [0, jnp.minimum(z + 1, 0), jnp.minimum(z + 2, 0)]
        ta, tb = NU - 2, NU - 1
        tile0 = (NB - 1) * SP
        slot0 = ((NB - 1) % 2) * SP
        lanes = pl.ds((NB - 1) * TB, TB)
        ecopies = []

        def ecopy(s_lo, s_hi, rlo=0, rhi=C):
            cp = pltpu.make_async_copy(
                obuf.at[pl.ds(slot0 + s_lo, s_hi - s_lo), pl.ds(rlo, rhi - rlo), :],
                o_hbm.at[pl.ds(s_lo, s_hi - s_lo), pl.ds(rlo, rhi - rlo), lanes],
                sems.at[ES0 + len(ecopies)])
            ecopies.append(cp)
            return cp

        sent = odone(NBODY - 2)
        s_a = (sent - (NB - 1) * CPT) * CH
        s_b, s_c, s_d = MO * (ta - 1) - tile0, MO * ta - tile0, MO * tb - tile0
        assert 0 <= s_a < s_b and S - s_d == MO - 1
        ecopy(s_a, s_b).start()
        e1, e2 = ecopy(s_b, s_c), ecopy(s_c, s_d)
        mta = [ma_ref if j < JS else mb_ref for j in range(NP)]
        mtb = [mc_ref if j < JS else ma_ref for j in range(NP)]

        def last_a(i):
            output(ta - 1 + z, msb)
            dots(transform(ta + z, True, zs, z < 0), mta, z)
            carry_u0(tb + z)
            pl.when(i >= 0)(e1.start)

        def last_b(i):
            output(ta + z, mta)
            dots(transform(tb + z, False, zs, z < 0), mtb, z, NP - 1)
            pl.when(i >= 0)(e2.start)

        once(z, last_a)
        once(z, last_b)
        RP = C // NEP
        for e in range(NEP):
            output(tb, mtb, e * RP, (e + 1) * RP, MO - 1)
            ecopy(s_d, S, e * RP, (e + 1) * RP).start()
        for c in range(ofree(NBODY - 1), sent):
            ocopy(c).wait()
        for cp in ecopies:
            cp.wait()

    any_spec = pl.BlockSpec(memory_space=pl.ANY)
    out = pl.pallas_call(
        kernel,
        in_specs=[any_spec] * 6,
        out_specs=any_spec,
        out_shape=jax.ShapeDtypeStruct((S, C, B), x.dtype),
        scratch_shapes=[
            pltpu.VMEM((NP, NKT + 1, C // 2, 128), U32),
            pltpu.VMEM((C + 8, 128), F32),
            pltpu.VMEM((C + 8, 128), F32),
            pltpu.VMEM((CF, TB), BF16),
            pltpu.VMEM((3, C, C), BF16),
            pltpu.VMEM((C,), BF16), pltpu.VMEM((C,), BF16),
            pltpu.VMEM((C,), BF16), pltpu.VMEM((C,), BF16),
            pltpu.VMEM((RING + 2, C, TB), BF16),
            pltpu.VMEM((RING, C, TB), BF16),
            pltpu.SemaphoreType.DMA((NSEM,)),
            pltpu.VMEM((NP, C, TB), F32), pltpu.VMEM((NP, C, TB), F32), pltpu.VMEM((NP, C, TB), F32),
        ],
        compiler_params=pltpu.CompilerParams(vmem_limit_bytes=100 * 1024 * 1024,
                                             disable_bounds_checks=True),
    )(jnp.transpose(x, (1, 2, 0)), w, mean, var, g, b)
    return jnp.transpose(out, (2, 0, 1))
```

```python
import jax
import jax.numpy as jnp
import jax.experimental.pallas as pl
import jax.experimental.pallas.tpu as pltpu

F32 = jnp.float32
BF16 = jnp.bfloat16
U32 = jnp.uint32

TB = 128
MO = 6
NP = MO + 2
UPB = 2
NPRO = 2
RC = 16
CH = 8
LEAD = 3
NEP = 4
JS = 4
EPS = 1e-5
PJ = (0, 7, 5, 6, 3, 4, 1, 2)
CPK = {0: -2.25, 3: -0.025, 4: 0.075, 5: 0.8, 6: 2.4, 7: 2.25}


@jax.jit
def pallas_standalone__batchnorm__sampling_kernel(
    x: jax.Array,
    w: jax.Array,
    mean: jax.Array,
    var: jax.Array,
    g: jax.Array,
    b: jax.Array,
):
    B, S, C = x.shape
    NKT = C // 128
    CF = NKT * 128
    CR = C - CF
    SP = S + 1
    NB = B // TB
    NU = NB * SP // MO
    RING = 2 * SP
    UPR = RING // MO
    CPT = S // CH
    NCH = NB * CPT
    NBODY = (NU - NPRO) // UPB
    STEP = MO * UPB
    NSP = MO * NPRO + 1
    CSP = -(-NSP // CH)
    assert w.shape == (3, C, C) and 2 * CR == 128 and CPT == 4 and CH == 8
    assert NB * TB == B and NU * MO == NB * SP and UPR * MO == RING and NBODY * UPB == NU - NPRO

    chunk_of = lambda p: CPT * (p // SP) + min((p % SP) // CH, CPT - 1)
    first = lambda i: NPRO + UPB * i
    xneed = lambda i: min(chunk_of(MO * first(i + 1) + MO - 1) + 1, NCH)

    def odone(i):
        p = MO * (first(i + 1) - 1)
        return CPT * (p // SP) + (p % SP) // CH

    def ofree(i):
        p = MO * (first(i + 1) - 1) - 1 - RING
        return 0 if p < 0 else chunk_of(p) + 1

    def sched(q, r, mx=jnp.minimum, sel=jnp.where):
        rn = r + STEP + 2 * MO - 1
        n2 = sel(rn >= SP, CPT * (q + 1) + mx((rn - SP) >> 3, CPT - 1), CPT * q + mx(rn >> 3, CPT - 1)) + 1
        rf = r + STEP - 1
        f2 = sel(rf >= SP, CPT * (q - 1) + ((rf - SP) >> 3), CPT * (q - 2) + mx(rf >> 3, CPT - 1)) + 1
        return CPT * q + (r >> 3), mx(n2, NCH), sel(f2 < 0, 0, f2)

    MAXC = 2
    assert odone(-1) == 0 and xneed(0) + LEAD <= 2 * CPT and xneed(NBODY - 1) == NCH
    for i in range(NBODY - 1):
        assert max(xneed(i + 1) - xneed(i), odone(i) - odone(i - 1), ofree(i + 1) - ofree(i)) <= MAXC <= LEAD
        assert ofree(i + 1) <= odone(i - 1)
        old = min(xneed(i + 1) + LEAD, NCH) - 1 - 2 * CPT
        assert old < 0 or SP * (old // CPT) + CH * (old % CPT) + CH - 1 < MO * first(i + 1) - 1
        p = MO * (first(i + 2) - 1)
        assert i == NBODY - 2 or (sched(p // SP, p % SP, min, lambda c, u, v: u if c else v)
                                  == (odone(i + 1), xneed(i + 2), ofree(i + 2)))

    XS0, OS0, WS0 = 0, 2 * CPT, 4 * CPT
    PS0 = WS0 + NKT + 1
    KS0 = PS0 + 4
    ES0 = KS0 + NKT + 3
    NSEM = ES0 + 3 + NEP

    def kernel(x_hbm, w_hbm, mean_hbm, var_hbm, g_hbm, b_hbm, o_hbm,
               a_ref, u0_ref, xbuf, obuf, sh_ref, hs_ref, ma_ref, mb_ref, mc_ref, w1_ref, wl_ref, p0, p1, p2, p3, wbuf, sems):

        def hbm_chunk(ref, c):
            lane0 = (c >> 2) * TB
            if not isinstance(c, int):
                lane0 = pl.multiple_of(lane0, TB)
            return ref.at[pl.ds((c & 3) * CH, CH), :, pl.ds(lane0, TB)]

        def ring_slot(c):
            return ((c >> 2) & 1) * SP + (c & 3) * CH

        def xcopy(c):
            return pltpu.make_async_copy(hbm_chunk(x_hbm, c), xbuf.at[pl.ds(ring_slot(c) + 1, CH)],
                                         sems.at[XS0 + (c & 7)])

        def ocopy(c):
            return pltpu.make_async_copy(obuf.at[pl.ds(ring_slot(c), CH)], hbm_chunk(o_hbm, c),
                                         sems.at[OS0 + (c & 7)])

        def krows(kt):
            if isinstance(kt, int):
                return pl.ds(kt * 128, 128 if kt < NKT else CR)
            return pl.ds(pl.multiple_of(kt * 128, 128), 128)

        def wcopy(kt):
            return pltpu.make_async_copy(w_hbm.at[:, krows(kt), :], wbuf.at[:, krows(kt), :],
                                         sems.at[WS0 + kt])

        def kcopy(kt, lo=0, hi=NSP, sem=None):
            return pltpu.make_async_copy(x_hbm.at[pl.ds(lo, hi - lo), krows(kt), pl.ds(0, TB)],
                                         xbuf.at[pl.ds(1 + lo, hi - lo), krows(kt), :],
                                         sems.at[KS0 + kt if sem is None else sem])

        k0a_copy = kcopy(0, 0, MO + 1)
        k0b_copy = kcopy(0, MO + 1, NSP, KS0 + NKT + 1)
        rcopy = pltpu.make_async_copy(x_hbm.at[pl.ds(NSP, CSP * CH - NSP), :, pl.ds(0, TB)],
                                      xbuf.at[pl.ds(1 + NSP, CSP * CH - NSP)], sems.at[KS0 + NKT + 2])
        pcopies = [pltpu.make_async_copy(s, d, sems.at[PS0 + i])
                   for i, (s, d) in enumerate(zip((mean_hbm, var_hbm, g_hbm, b_hbm), (p0, p1, p2, p3)))]
        for c in pcopies:
            c.start()
        wcopy(0).start()
        k0a_copy.start()
        wcopy(1).start()
        k0b_copy.start()
        kcopy(1).start()
        for kt in range(2, NKT + 1):
            wcopy(kt).start()
            kcopy(kt).start()
        rcopy.start()
        for c in range(CSP, xneed(0) + LEAD):
            xcopy(c).start()

        for s in (0, SP, RING, RING + 1):
            xbuf[s] = jnp.zeros((C, TB), BF16)

        for c in pcopies:
            c.wait()
        mean_, var_, g_, b_ = [r[...].astype(F32).reshape(1, C) for r in (p0, p1, p2, p3)]
        scale = g_ * jax.lax.rsqrt(var_ + EPS)
        hs_ref[...] = jnp.broadcast_to(0.5 * scale, (128, C)).T
        sh = 0.5 * (b_ - mean_ * scale)
        sh_hi = sh.astype(BF16).astype(F32)
        sh_mid = (sh - sh_hi).astype(BF16).astype(F32)
        sh_lo = (sh - sh_hi) - sh_mid
        row = jax.lax.broadcasted_iota(jnp.int32, (128, C), 0)
        sh_ref[...] = jnp.where(row == CR, sh_hi, jnp.where(
            row == CR + 1, sh_mid, jnp.where(row == CR + 2, sh_lo, 0.0))).T

        def tchunk(ld, with_u0=True):
            d1, d2, d3, d4, d5, d6 = [ld(i, 1) for i in range(1, 7)]
            e1, o1 = (d2 + d6) - 4.25 * d4, (d1 + d5) - 4.25 * d3
            d1, d2, d3, d4, d5, d6, d7 = [ld(i, 2) for i in range(1, 8)]
            e2, o2 = (d6 - d4) - 0.25 * (d4 - d2), 2.0 * (d5 - d3) - 0.5 * (d3 - d1)
            e3, o3 = (d6 - d4) - 4.0 * (d4 - d2), 0.5 * (d5 - d3) - 2.0 * (d3 - d1)
            u = [None, e1 + o1, e1 - o1, e2 + o2, e2 - o2, e3 + o3, e3 - o3, (d7 - d1) - 5.25 * (d5 - d3)]
            if with_u0:
                d0, d2, d4, d6 = [ld(i, 0) for i in (0, 2, 4, 6)]
                u[0] = (d0 - d6) + 5.25 * (d4 - d2)
            return u

        def ones_rows():
            return (jax.lax.broadcasted_iota(jnp.int32, (CR, TB), 0) < 3).astype(F32)

        def carry_u0(t):
            base = (t % UPR) * MO
            for r in range(0, CF, RC):
                d0, d2, d4, d6 = [xbuf[base + i, r:r + RC, :].astype(F32) for i in (0, 2, 4, 6)]
                u0_ref[r:r + RC, :] = ((d0 - d6) + 5.25 * (d4 - d2)).astype(BF16)

        def transform(t, carried, zs, never):
            base = (t % UPR) * MO
            cs = []
            for r in range(0, C, RC):
                c = tchunk(lambda i, gi: xbuf[base + zs[gi] + i, r:r + RC, :].astype(F32), not (carried and r < CF))
                for j in (2, 4, 5, 6, 7):
                    c[j] = pltpu.bitcast(c[j].astype(BF16), U32)
                for j, dep in ((1, c[2]), (3, c[4] ^ c[5] ^ c[6] ^ c[7])):
                    top = jnp.where(never, jax.lax.bitcast_convert_type(dep, F32), c[j][0:RC // 2])
                    c[j] = jnp.concatenate([top, c[j][RC // 2:]], axis=0)
                cs.append(c)
            tail = pltpu.bitcast(jnp.concatenate([c[2] for c in cs[CF // RC:]], axis=0), BF16)
            us = []
            for j in range(NP):
                parts = [c[j] for c in cs if c[j] is not None]
                if j == 2:
                    parts = parts[:CF // RC]
                if j == 1:
                    parts = parts + [ones_rows()]
                v = jnp.concatenate(parts, axis=0)
                v = v.astype(BF16) if j in (0, 1, 3) else pltpu.bitcast(v, BF16)
                if j not in (1, 2):
                    v = jnp.concatenate([v, tail], axis=0)
                if j == 0 and carried:
                    v = jnp.concatenate([u0_ref[...], v], axis=0)
                us.append(v)
            return us

        def dots(us, ms, z, nprod=NP):
            for j in range(nprod):
                nk = NKT if j == 2 else NKT + 1
                lhs = pltpu.bitcast(jnp.concatenate([a_ref[j, kt] for kt in range(nk)], axis=1), BF16)
                ms[j][j + z, 0:C, :] = jnp.dot(lhs, us[j], preferred_element_type=F32)

        def output(t, ms, rlo=0, rhi=C, nout=MO):
            base = (t % UPR) * MO
            for r in range(rlo, rhi, RC):
                m = [ms[j][j, r:r + RC, :] if (j < NP - 1 or nout == MO) else 0.0 for j in range(NP)]
                s1, s2, s3 = m[1] + m[2], m[3] + m[4], m[5] + m[6]
                d1, d2, d3 = m[1] - m[2], m[3] - m[4], m[5] - m[6]
                hs = hs_ref[r:r + RC, :]
                ys = [(hs * m[0] + s1) + (s2 + s3),
                      (d1 + 2.0 * d2) + 0.5 * d3,
                      (s1 + 4.0 * s2) + 0.25 * s3,
                      (d1 + 8.0 * d2) + 0.125 * d3,
                      (s1 + 16.0 * s2) + 0.0625 * s3,
                      (d1 + 32.0 * d2) + (0.03125 * d3 + hs * m[7])]
                for i in range(nout):
                    h = ys[i]
                    obuf[base + i, r:r + RC, :] = (h * jnp.tanh(h) + h).astype(BF16)

        msa, msb = [ma_ref] * NP, [mb_ref] * NP

        def once(z, fn):
            def trip(i, c):
                fn(i)
                return c
            jax.lax.fori_loop(0, z + 1, trip, 0)

        def xpose(kt):
            last = isinstance(kt, int) and kt == NKT
            for r in range(0, C, 128):
                cols = slice(r, min(r + 128, C))
                rows = slice(r // 2, min(r + 128, C) // 2)
                for k, dst in enumerate((a_ref.at[0], w1_ref, a_ref.at[NP - 1])):
                    if last:
                        t = jnp.concatenate([wbuf[k, CF:C, cols]] * 2, axis=0).T
                        wl_ref[k, rows, :] = pltpu.bitcast(t, U32)
                    else:
                        dst[kt, rows, :] = pltpu.bitcast(wbuf[k, krows(kt), cols].T, U32)

        def combos(kt, zs, never):
            last = isinstance(kt, int) and kt == NKT
            lo = jax.lax.broadcasted_iota(jnp.int32, (RC, 128), 1) < CR
            pack = lambda v: pltpu.bitcast(v.astype(BF16), U32)
            out = dict((j, []) for j in range(NP))
            for r in range(0, C, RC):
                rows = slice(r // 2, (r + RC) // 2)
                def taps(gi):
                    if last:
                        raw = [wl_ref[k + zs[gi], rows, :] for k in range(3)]
                    else:
                        raw = [a_ref[zs[gi], kt, rows, :], w1_ref[kt + zs[gi], rows, :], a_ref[NP - 1 + zs[gi], kt, rows, :]]
                    return [pltpu.bitcast(t, BF16).astype(F32) for t in raw]
                hs = hs_ref[r:r + RC, :]
                for gi, (ce0, ce2, co) in enumerate(((-2.0 / 9, -2.0 / 9, -2.0 / 9), (1.0 / 90, 2.0 / 45, 1.0 / 45),
                                                     (32.0 / 45, 8.0 / 45, 16.0 / 45))):
                    w0, w1, w2 = [t * hs for t in taps(gi)]
                    e = ce0 * (w0 + w2) if gi == 0 else ce0 * w0 + ce2 * w2
                    o = co * w1
                    ja, jb = 2 * gi + 1, 2 * gi + 2
                    ga, gb = e + o, e - o
                    if last:
                        if gi == 0:
                            out[1].append(pack(jnp.where(lo, ga, sh_ref[r:r + RC, :])))
                            continue
                        g2 = (w0 + w2) - w1
                        ga = jnp.where(lo, ga, (-2.0 / 9 * CPK[ja]) * g2)
                        gb = jnp.where(lo, gb, (-2.0 / 9 * CPK[jb]) * g2)
                    pb = pack(gb)
                    out[ja].append(jnp.where(never, pb, pack(ga)))
                    out[jb].append(pb)
                if last:
                    r0, r1, r2 = taps(3)
                    raw2 = (r0 + r2) - r1
                    p7 = pack(jnp.where(lo, r2, (-2.0 / 9 * CPK[7]) * raw2))
                    out[0].append(jnp.where(never, p7, pack(jnp.where(lo, r0, (-2.0 / 9 * CPK[0]) * raw2))))
                    out[7].append(p7)
            res = {}
            for j in range(NP):
                if out[j]:
                    res[j] = jnp.concatenate(out[j], axis=0)
                    a_ref[j, kt] = res[j]
                elif not last:
                    res[j] = a_ref[j, kt]
            return res

        def mm(kt, i, units=(0, 1), fresh=True):
            last = isinstance(kt, int) and kt == NKT
            r0 = kt * 128 if isinstance(kt, int) else pl.multiple_of(kt * 128, 128)
            zs = [jnp.minimum(i + q, 0) for q in range(4)]
            lhs = combos(kt, zs, i < 0) if fresh else dict((j, a_ref[j, kt]) for j in range(NP))
            rhs = []
            for u in units:
                cs = [tchunk(lambda s, gi: xbuf[MO * u + s + zs[gi], pl.ds(r0 + r, RC), :].astype(F32))
                      for r in range(0, CR if last else 128, RC)]
                fin = lambda j: jnp.concatenate([c[j] for c in cs], axis=0).astype(BF16)
                rhs.append(dict(
                    (j, jnp.concatenate([fin(j), ones_rows().astype(BF16) if j == 1 else fin(2)], axis=0)
                     if last else fin(j)) for j in lhs))
            for j in PJ:
                if j in lhs:
                    for u, rh in zip(units, rhs):
                        m_ref = (ma_ref, mb_ref)[u]
                        p = jnp.dot(pltpu.bitcast(lhs[j], BF16), rh[j], preferred_element_type=F32)
                        m_ref[j] = p if isinstance(kt, int) and kt == 0 else m_ref[j] + p

        def kblock(kt, i):
            kcopy(kt).wait()
            wcopy(kt + 1).wait()
            xpose(kt + 1)
            mm(kt, i)
            return 0

        wcopy(0).wait()
        xpose(0)
        z = jax.lax.fori_loop(0, 2, lambda i, c: jnp.minimum(i, c), jnp.int32(0))
        k0a_copy.wait()
        once(z, lambda i: mm(0, i, (0,)))
        wcopy(1).wait()
        k0b_copy.wait()
        once(z, lambda i: (xpose(1), mm(0, i, (1,), False)))
        jax.lax.fori_loop(1, NKT - 1, lambda i, c: kblock(i, i), 0)
        once(z, lambda i: kblock(NKT - 1, i))
        kcopy(NKT).wait()
        once(z, lambda i: (mm(NKT, i), output(z, msa)))
        rcopy.wait()
        for c in range(CSP, xneed(0)):
            xcopy(c).wait()
        carry_u0(NPRO)

        def body(i, carry):
            o0, o1, n0, n1, f0, f1, q, r = carry
            t0 = first(i)
            z = jnp.minimum(i, 0)
            zs = [0, jnp.minimum(i + 1, 0), jnp.minimum(i + 2, 0)]
            dots(transform(t0, True, zs, i < 0), msa, z)
            output(t0 - 1, msb)
            dots(transform(t0 + 1, False, zs, i < 0), msb, z)
            output(t0, msa)
            carry_u0(t0 + UPB)
            for k in range(MAXC):
                @pl.when(o0 + k < o1)
                def _():
                    ocopy(o0 + k).start()
            for k in range(MAXC):
                @pl.when(jnp.logical_and(n0 + k < n1, n0 + k + LEAD < NCH))
                def _():
                    xcopy(n0 + k + LEAD).start()
            for k in range(MAXC):
                @pl.when(n0 + k < n1)
                def _():
                    xcopy(n0 + k).wait()
            for k in range(MAXC):
                @pl.when(f0 + k < f1)
                def _():
                    ocopy(f0 + k).wait()
            o2, n2, f2 = sched(q, r)
            wrap = r + STEP >= SP
            return (o1, o2, n1, n2, f1, f2, q + wrap.astype(jnp.int32),
                    jnp.where(wrap, r + STEP - SP, r + STEP))

        p1 = MO * (first(2) - 1)
        init = (odone(-1), odone(0), xneed(0), xneed(1), ofree(0), ofree(1), p1 // SP, p1 % SP)
        fin = jax.lax.fori_loop(0, NBODY - 1, body, tuple(jnp.int32(v) for v in init))

        z = jnp.minimum(fin[0], 0)
        zs = [0, jnp.minimum(z + 1, 0), jnp.minimum(z + 2, 0)]
        ta, tb = NU - 2, NU - 1
        tile0 = (NB - 1) * SP
        slot0 = ((NB - 1) % 2) * SP
        lanes = pl.ds((NB - 1) * TB, TB)
        ecopies = []

        def ecopy(s_lo, s_hi, rlo=0, rhi=C):
            cp = pltpu.make_async_copy(
                obuf.at[pl.ds(slot0 + s_lo, s_hi - s_lo), pl.ds(rlo, rhi - rlo), :],
                o_hbm.at[pl.ds(s_lo, s_hi - s_lo), pl.ds(rlo, rhi - rlo), lanes],
                sems.at[ES0 + len(ecopies)])
            ecopies.append(cp)
            return cp

        sent = odone(NBODY - 2)
        s_a = (sent - (NB - 1) * CPT) * CH
        s_b, s_c, s_d = MO * (ta - 1) - tile0, MO * ta - tile0, MO * tb - tile0
        assert 0 <= s_a < s_b and S - s_d == MO - 1
        ecopy(s_a, s_b).start()
        e1, e2 = ecopy(s_b, s_c), ecopy(s_c, s_d)
        mta = [ma_ref if j < JS else mb_ref for j in range(NP)]
        mtb = [mc_ref if j < JS else ma_ref for j in range(NP)]

        def last_a(i):
            output(ta - 1 + z, msb)
            dots(transform(ta + z, True, zs, z < 0), mta, z)
            carry_u0(tb + z)
            pl.when(i >= 0)(e1.start)

        def last_b(i):
            output(ta + z, mta)
            dots(transform(tb + z, False, zs, z < 0), mtb, z, NP - 1)
            pl.when(i >= 0)(e2.start)

        once(z, last_a)
        once(z, last_b)
        RP = C // NEP
        for e in range(NEP):
            output(tb, mtb, e * RP, (e + 1) * RP, MO - 1)
            ecopy(s_d, S, e * RP, (e + 1) * RP).start()
        for c in range(ofree(NBODY - 1), sent):
            ocopy(c).wait()
        for cp in ecopies:
            cp.wait()

    any_spec = pl.BlockSpec(memory_space=pl.ANY)
    out = pl.pallas_call(
        kernel,
        in_specs=[any_spec] * 6,
        out_specs=any_spec,
        out_shape=jax.ShapeDtypeStruct((S, C, B), x.dtype),
        scratch_shapes=[
            pltpu.VMEM((NP, NKT + 1, C // 2, 128), U32),
            pltpu.VMEM((CF, TB), BF16),
            pltpu.VMEM((RING + 2, C, TB), BF16),
            pltpu.VMEM((RING, C, TB), BF16),
            pltpu.VMEM((C, 128), F32),
            pltpu.VMEM((C, 128), F32),
            pltpu.VMEM((NP, C, TB), F32),
            pltpu.VMEM((NP, C, TB), F32),
            pltpu.VMEM((NP, C, TB), F32),
            pltpu.VMEM((NKT, C // 2, 128), U32),
            pltpu.VMEM((3, C // 2, 128), U32),
            pltpu.VMEM((C,), BF16), pltpu.VMEM((C,), BF16),
            pltpu.VMEM((C,), BF16), pltpu.VMEM((C,), BF16),
            pltpu.VMEM((3, C + 24, C), BF16),
            pltpu.SemaphoreType.DMA((NSEM,)),
        ],
        compiler_params=pltpu.CompilerParams(vmem_limit_bytes=100 * 1024 * 1024,
                                             disable_bounds_checks=True),
    )(jnp.transpose(x, (1, 2, 0)), w, mean, var, g, b)
    return jnp.transpose(out, (2, 0, 1))
```

```python
import jax
import jax.numpy as jnp
import jax.experimental.pallas as pl
import jax.experimental.pallas.tpu as pltpu

F32 = jnp.float32
BF16 = jnp.bfloat16
U32 = jnp.uint32

TB = 128
MO = 6
NP = MO + 2
UPB = 4
LAG = 2
NPRO = 3
RC = 16
CH = 8
RT = 4
LEAD = 3
NEP = 4
JS = 4
ORDER, GROUPS = (0, 7, 1, 2, 3, 4, 5, 6), (0, 1, 2, 3, 4)
ORDER_END, GROUPS_END = (0, 1, 2, 3, 4, 5, 6, 7), (0, 1, 2, 2, 2)
ORDER_PRO, ORDER_PRO_LAST, GROUPS_PRO = (0, 7, 5, 6, 3, 4, 1, 2), (7, 0, 3, 4, 5, 6, 1), (0, 1, 2, 3, 3)
EPS = 1e-5
CPK = {0: -2.25, 3: -0.025, 4: 0.075, 5: 0.8, 6: 2.4, 7: 2.25}


@jax.jit
def pallas_standalone__batchnorm__sampling_kernel(
    x: jax.Array,
    w: jax.Array,
    mean: jax.Array,
    var: jax.Array,
    g: jax.Array,
    b: jax.Array,
):
    B, S, C = x.shape
    NKT = C // 128
    CF = NKT * 128
    CR = C - CF
    SP = S + 1
    NB = B // TB
    NU = NB * SP // MO
    RING = RT * SP
    UPR = RING // MO
    CPT = S // CH
    NCH = NB * CPT
    NSC = RT * CPT
    U1 = NPRO + 1
    NBODY = (NU - U1 - 4) // UPB
    U2 = U1 + NBODY * UPB
    STEP = MO * UPB
    NSP = MO * NPRO + 1
    CSP = -(-NSP // CH)
    assert w.shape == (3, C, C) and 2 * CR == 128 and CPT == 4 and CH == 8
    assert NB * TB == B and NU * MO == NB * SP and UPR * MO == RING and U2 + 4 == NU and U1 % 4 == 0

    chunk_of = lambda p: CPT * (p // SP) + min((p % SP) // CH, CPT - 1)
    pn = lambda e: MO * e + MO - 1
    po = lambda e: MO * (e - LAG)
    pf = lambda e: po(e) - 1 - RING
    xneed = lambda e: min(chunk_of(pn(e)) + 1, NCH)
    odone = lambda e: CPT * (po(e) // SP) + (po(e) % SP) // CH
    ofree = lambda e: max(chunk_of(pf(e)) + 1, 0)
    ends = [U1] + [U1 + UPB * (i + 1) for i in range(NBODY)] + [U2 + 2, NU]
    MAXC = 3
    assert xneed(U1) + LEAD <= NSC and xneed(U2 + 2) == NCH and ofree(U1) == 0
    for e0, e1 in zip(ends[:-2], ends[1:-1]):
        assert max(xneed(e1) - xneed(e0), ofree(e1) - ofree(e0)) <= MAXC <= LEAD
        assert odone(e1) - odone(e0) <= MAXC and ofree(e1) <= (odone(e0 - UPB) if e0 > U1 else 0)
        old = min(xneed(e1) + LEAD, NCH) - 1 - NSC
        assert old < 0 or SP * (old // CPT) + CH * (old % CPT) + CH - 1 < MO * e0 - 1

    XS0, OS0, WS0 = 0, NSC, 2 * NSC
    PS0 = WS0 + NKT + 1
    KS0 = PS0 + 4
    ES0 = KS0 + NKT + 3
    NSEM = ES0 + 3 + NEP

    def kernel(x_hbm, w_hbm, mean_hbm, var_hbm, g_hbm, b_hbm, o_hbm,
               a_ref, u0_ref, xbuf, obuf, sh_ref, hs_ref, ma_ref, mb_ref, mc_ref, md_ref, w1_ref, wl_ref, p0, p1, p2, p3, wbuf, sems):

        def hbm_chunk(ref, c):
            lane0 = (c >> 2) * TB
            if not isinstance(c, int):
                lane0 = pl.multiple_of(lane0, TB)
            return ref.at[pl.ds((c & 3) * CH, CH), :, pl.ds(lane0, TB)]

        def ring_slot(c):
            return ((c >> 2) & (RT - 1)) * SP + (c & 3) * CH

        def xcopy(c):
            return pltpu.make_async_copy(hbm_chunk(x_hbm, c), xbuf.at[pl.ds(ring_slot(c) + 1, CH)],
                                         sems.at[XS0 + (c & (NSC - 1))])

        def ocopy(c):
            return pltpu.make_async_copy(obuf.at[pl.ds(ring_slot(c), CH)], hbm_chunk(o_hbm, c),
                                         sems.at[OS0 + (c & (NSC - 1))])

        def krows(kt):
            if isinstance(kt, int):
                return pl.ds(kt * 128, 128 if kt < NKT else CR)
            return pl.ds(pl.multiple_of(kt * 128, 128), 128)

        def wcopy(kt):
            return pltpu.make_async_copy(w_hbm.at[:, krows(kt), :], wbuf.at[:, krows(kt), :],
                                         sems.at[WS0 + kt])

        def kcopy(kt, lo=0, hi=NSP, sem=None):
            return pltpu.make_async_copy(x_hbm.at[pl.ds(lo, hi - lo), krows(kt), pl.ds(0, TB)],
                                         xbuf.at[pl.ds(1 + lo, hi - lo), krows(kt), :],
                                         sems.at[KS0 + kt if sem is None else sem])

        k0a_copy = kcopy(0, 0, MO + 1)
        k0b_copy = kcopy(0, MO + 1, NSP, KS0 + NKT + 1)
        rcopy = pltpu.make_async_copy(x_hbm.at[pl.ds(NSP, CSP * CH - NSP), :, pl.ds(0, TB)],
                                      xbuf.at[pl.ds(1 + NSP, CSP * CH - NSP)], sems.at[KS0 + NKT + 2])
        pcopies = [pltpu.make_async_copy(s, d, sems.at[PS0 + i])
                   for i, (s, d) in enumerate(zip((mean_hbm, var_hbm, g_hbm, b_hbm), (p0, p1, p2, p3)))]
        for c in pcopies:
            c.start()
        wcopy(0).start()
        k0a_copy.start()
        wcopy(1).start()
        k0b_copy.start()
        kcopy(1).start()
        for kt in range(2, NKT + 1):
            wcopy(kt).start()
            kcopy(kt).start()
        rcopy.start()
        for c in range(CSP, xneed(U1) + LEAD):
            xcopy(c).start()

        for s in [SP * q for q in range(RT + 1)] + [RING + 1]:
            xbuf[s] = jnp.zeros((C, TB), BF16)

        for c in pcopies:
            c.wait()
        mean_, var_, g_, b_ = [r[...].astype(F32).reshape(1, C) for r in (p0, p1, p2, p3)]
        scale = g_ * jax.lax.rsqrt(var_ + EPS)
        hs_ref[...] = jnp.broadcast_to(0.5 * scale, (128, C)).T
        sh = 0.5 * (b_ - mean_ * scale)
        sh_hi = sh.astype(BF16).astype(F32)
        sh_mid = (sh - sh_hi).astype(BF16).astype(F32)
        sh_lo = (sh - sh_hi) - sh_mid
        row = jax.lax.broadcasted_iota(jnp.int32, (128, C), 0)
        sh_ref[...] = jnp.where(row == CR, sh_hi, jnp.where(
            row == CR + 1, sh_mid, jnp.where(row == CR + 2, sh_lo, 0.0))).T

        def tchunk(ld_, with_u0, grp):
            ld = lambda i, gi: ld_(i, grp[gi])
            d1, d2, d3, d4, d5, d6 = [ld(i, 1) for i in range(1, 7)]
            e1, o1 = (d2 + d6) - 4.25 * d4, (d1 + d5) - 4.25 * d3
            d1, d2, d3, d4, d5, d6 = [ld(i, 2) for i in range(1, 7)]
            e2, o2 = (d6 - d4) - 0.25 * (d4 - d2), 2.0 * (d5 - d3) - 0.5 * (d3 - d1)
            d1, d2, d3, d4, d5, d6 = [ld(i, 3) for i in range(1, 7)]
            e3, o3 = (d6 - d4) - 4.0 * (d4 - d2), 0.5 * (d5 - d3) - 2.0 * (d3 - d1)
            d1, d3, d5, d7 = [ld(i, 4) for i in (1, 3, 5, 7)]
            u = [None, e1 + o1, e1 - o1, e2 + o2, e2 - o2, e3 + o3, e3 - o3, (d7 - d1) - 5.25 * (d5 - d3)]
            if with_u0:
                d0, d2, d4, d6 = [ld(i, 0) for i in (0, 2, 4, 6)]
                u[0] = (d0 - d6) + 5.25 * (d4 - d2)
            return u

        def ones_rows():
            return (jax.lax.broadcasted_iota(jnp.int32, (CR, TB), 0) < 3).astype(F32)

        def carry_u0(t):
            base = (t % UPR) * MO
            for r in range(0, CF, RC):
                d0, d2, d4, d6 = [xbuf[base + i, r:r + RC, :].astype(F32) for i in (0, 2, 4, 6)]
                u0_ref[r:r + RC, :] = ((d0 - d6) + 5.25 * (d4 - d2)).astype(BF16)

        def transform(t, carried, z, grp, order):
            zs = [0] + [jnp.minimum(z + q, 0) for q in range(1, 5)]
            never = z < 0
            base = (t % UPR) * MO
            gof = [grp[q] for q in (0, 1, 1, 2, 2, 3, 3, 4)]
            cs = []
            for r in range(0, C, RC):
                c = tchunk(lambda i, gi: xbuf[base + zs[gi] + i, r:r + RC, :].astype(F32),
                           not (carried and r < CF), grp)
                members = {}
                for j in order:
                    if c[j] is not None:
                        members.setdefault(gof[j], []).append(j)
                for j in set(j for mem in members.values() for j in mem[1:]) | {2}:
                    c[j] = pltpu.bitcast(c[j].astype(BF16), U32)
                for mem in members.values():
                    if len(mem) > 1 and mem[0] != 2:
                        dep = c[mem[1]]
                        for j in mem[2:]:
                            dep = dep ^ c[j]
                        top = jnp.where(never, jax.lax.bitcast_convert_type(dep, F32), c[mem[0]][0:RC // 2])
                        c[mem[0]] = jnp.concatenate([top, c[mem[0]][RC // 2:]], axis=0)
                cs.append(c)
            tail = pltpu.bitcast(jnp.concatenate([c[2] for c in cs[CF // RC:]], axis=0), BF16)
            us = {}
            for j in order:
                parts = [c[j] for c in cs if c[j] is not None]
                if j == 2:
                    parts = parts[:CF // RC]
                if j == 1:
                    parts = parts + [ones_rows()]
                v = jnp.concatenate(parts, axis=0)
                v = v.astype(BF16) if v.dtype == F32 else pltpu.bitcast(v, BF16)
                if j not in (1, 2):
                    v = jnp.concatenate([v, tail], axis=0)
                if j == 0 and carried:
                    v = jnp.concatenate([u0_ref[...], v], axis=0)
                us[j] = v
            return us

        def unit(t, carried, ms, i, grp, order):
            us = transform(t, carried, i, grp, order)
            z = jnp.minimum(i, 0)
            for j in order:
                nk = NKT if j == 2 else NKT + 1
                lhs = pltpu.bitcast(jnp.concatenate([a_ref[j, kt] for kt in range(nk)], axis=1), BF16)
                ms[j][j + z, 0:C, :] = jnp.dot(lhs, us[j], preferred_element_type=F32)

        def output(t, ms, rlo=0, rhi=C, nout=MO):
            base = (t % UPR) * MO
            for r in range(rlo, rhi, RC):
                m = [ms[j][j, r:r + RC, :] if (j < NP - 1 or nout == MO) else 0.0 for j in range(NP)]
                s1, s2, s3 = m[1] + m[2], m[3] + m[4], m[5] + m[6]
                d1, d2, d3 = m[1] - m[2], m[3] - m[4], m[5] - m[6]
                hs = hs_ref[r:r + RC, :]
                ys = [(hs * m[0] + s1) + (s2 + s3),
                      (d1 + 2.0 * d2) + 0.5 * d3,
                      (s1 + 4.0 * s2) + 0.25 * s3,
                      (d1 + 8.0 * d2) + 0.125 * d3,
                      (s1 + 16.0 * s2) + 0.0625 * s3,
                      (d1 + 32.0 * d2) + (0.03125 * d3 + hs * m[7])]
                for i in range(nout):
                    h = ys[i]
                    obuf[base + i, r:r + RC, :] = (h * jnp.tanh(h) + h).astype(BF16)

        mbuf = [[r] * NP for r in (ma_ref, mb_ref, mc_ref, md_ref)]

        def once(z, fn):
            def trip(i, c):
                fn(i)
                return c
            jax.lax.fori_loop(0, z + 1, trip, 0)

        def xpose(kt):
            last = isinstance(kt, int) and kt == NKT
            for r in range(0, C, 128):
                cols = slice(r, min(r + 128, C))
                rows = slice(r // 2, min(r + 128, C) // 2)
                for k, dst in enumerate((a_ref.at[0], w1_ref, a_ref.at[NP - 1])):
                    if last:
                        t = jnp.concatenate([wbuf[k, CF:C, cols]] * 2, axis=0).T
                        wl_ref[k, rows, :] = pltpu.bitcast(t, U32)
                    else:
                        dst[kt, rows, :] = pltpu.bitcast(wbuf[k, krows(kt), cols].T, U32)

        def combos(kt, zs, never):
            last = isinstance(kt, int) and kt == NKT
            lo = jax.lax.broadcasted_iota(jnp.int32, (RC, 128), 1) < CR
            pack = lambda v: pltpu.bitcast(v.astype(BF16), U32)
            out = dict((j, []) for j in range(NP))
            for r in range(0, C, RC):
                rows = slice(r // 2, (r + RC) // 2)
                def taps(gi):
                    if last:
                        raw = [wl_ref[k + zs[gi], rows, :] for k in range(3)]
                    else:
                        raw = [a_ref[zs[gi], kt, rows, :], w1_ref[kt + zs[gi], rows, :], a_ref[NP - 1 + zs[gi], kt, rows, :]]
                    return [pltpu.bitcast(t, BF16).astype(F32) for t in raw]
                hs = hs_ref[r:r + RC, :]
                for gi, (ce0, ce2, co) in enumerate(((-2.0 / 9, -2.0 / 9, -2.0 / 9), (1.0 / 90, 2.0 / 45, 1.0 / 45),
                                                     (32.0 / 45, 8.0 / 45, 16.0 / 45))):
                    w0, w1, w2 = [t * hs for t in taps(gi)]
                    e = ce0 * (w0 + w2) if gi == 0 else ce0 * w0 + ce2 * w2
                    o = co * w1
                    ja, jb = 2 * gi + 1, 2 * gi + 2
                    ga, gb = e + o, e - o
                    if last:
                        if gi == 0:
                            out[1].append(pack(jnp.where(lo, ga, sh_ref[r:r + RC, :])))
                            continue
                        g2 = (w0 + w2) - w1
                        ga = jnp.where(lo, ga, (-2.0 / 9 * CPK[ja]) * g2)
                        gb = jnp.where(lo, gb, (-2.0 / 9 * CPK[jb]) * g2)
                    pb = pack(gb)
                    out[ja].append(jnp.where(never, pb, pack(ga)))
                    out[jb].append(pb)
                if last:
                    r0, r1, r2 = taps(3)
                    raw2 = (r0 + r2) - r1
                    p7 = pack(jnp.where(lo, r2, (-2.0 / 9 * CPK[7]) * raw2))
                    out[0].append(jnp.where(never, p7, pack(jnp.where(lo, r0, (-2.0 / 9 * CPK[0]) * raw2))))
                    out[7].append(p7)
            res = {}
            for j in range(NP):
                if out[j]:
                    res[j] = jnp.concatenate(out[j], axis=0)
                    a_ref[j, kt] = res[j]
                elif not last:
                    res[j] = a_ref[j, kt]
            return res

        def mm(kt, i, units=(0, 1, 2), fresh=True):
            last = isinstance(kt, int) and kt == NKT
            r0 = kt * 128 if isinstance(kt, int) else pl.multiple_of(kt * 128, 128)
            zs = [jnp.minimum(i + q, 0) for q in range(5)]
            lhs = combos(kt, zs, i < 0) if fresh else dict((j, a_ref[j, kt]) for j in range(NP))
            rhs = []
            for u in units:
                cs = [tchunk(lambda s, gi: xbuf[MO * u + s + zs[gi], pl.ds(r0 + r, RC), :].astype(F32), True, GROUPS_PRO)
                      for r in range(0, CR if last else 128, RC)]
                fin = lambda j: jnp.concatenate([c[j] for c in cs], axis=0).astype(BF16)
                rhs.append(dict(
                    (j, jnp.concatenate([fin(j), ones_rows().astype(BF16) if j == 1 else fin(2)], axis=0)
                     if last else fin(j)) for j in lhs))
            for j in (ORDER_PRO_LAST if last else ORDER_PRO):
                for u, rh in zip(units, rhs):
                    m_ref = mbuf[u][j]
                    p = jnp.dot(pltpu.bitcast(lhs[j], BF16), rh[j], preferred_element_type=F32)
                    m_ref[j] = p if isinstance(kt, int) and kt == 0 else m_ref[j] + p

        def kblock(kt, i):
            kcopy(kt).wait()
            wcopy(kt + 1).wait()
            xpose(kt + 1)
            mm(kt, i)
            return 0

        wcopy(0).wait()
        xpose(0)
        z = jax.lax.fori_loop(0, 2, lambda i, c: jnp.minimum(i, c), jnp.int32(0))
        k0a_copy.wait()
        once(z, lambda i: mm(0, i, (0,)))
        wcopy(1).wait()
        k0b_copy.wait()
        once(z, lambda i: (xpose(1), mm(0, i, (1, 2), False)))
        jax.lax.fori_loop(1, NKT - 1, lambda i, c: kblock(i, i), 0)
        once(z, lambda i: kblock(NKT - 1, i))
        kcopy(NKT).wait()
        once(z, lambda i: mm(NKT, i))
        rcopy.wait()
        for c in range(CSP, xneed(U1)):
            xcopy(c).wait()
        carry_u0(NPRO)

        def units(t0, n, i):
            for k in range(n):
                unit(t0 + k, k == 0, mbuf[k], i, GROUPS, ORDER)
                output(t0 + k - LAG, mbuf[(k - LAG) % 4])
            carry_u0(t0 + n)

        def copies(o0, o1, n0, n1, f0, f1):
            for k in range(MAXC):
                pl.when(o0 + k < o1)(lambda: ocopy(o0 + k).start())
            for k in range(MAXC):
                pl.when(jnp.logical_and(n0 + k < n1, n0 + k + LEAD < NCH))(lambda: xcopy(n0 + k + LEAD).start())
            for k in range(MAXC):
                pl.when(n0 + k < n1)(lambda: xcopy(n0 + k).wait())
            for k in range(MAXC):
                pl.when(f0 + k < f1)(lambda: ocopy(f0 + k).wait())

        def first1(i):
            output(z, mbuf[0])
            output(z + 1, mbuf[1])
            unit(NPRO + z, True, mbuf[NPRO], i, GROUPS, ORDER)
            carry_u0(U1 + z)
            copies(z, z + odone(U1), z + xneed(U1), z + xneed(U1 + UPB), z, z + ofree(U1 + UPB))

        once(z, first1)

        def advance(q, r):
            wrap = r + STEP >= SP
            return q + wrap.astype(jnp.int32), jnp.where(wrap, r + STEP - SP, r + STEP)

        def body(i, carry):
            o0, o1, n0, n1, f0, f1, qo, ro, qn, rn, qf, rf = carry
            units(U1 + UPB * i, UPB, i)
            copies(o0, o1, n0, n1, f0, f1)
            o2 = CPT * qo + (ro >> 3)
            n2 = jnp.minimum(CPT * qn + jnp.minimum(rn >> 3, CPT - 1) + 1, NCH)
            f2 = jnp.maximum(CPT * qf + jnp.minimum(rf >> 3, CPT - 1) + 1, 0)
            return (o1, o2, n1, n2, f1, f2) + advance(qo, ro) + advance(qn, rn) + advance(qf, rf)

        e1, e2, e3 = U1 + UPB, U1 + 2 * UPB, U1 + 3 * UPB
        init = (odone(U1), odone(e1), xneed(e1), xneed(e2), ofree(e1), ofree(e2),
                po(e2) // SP, po(e2) % SP, pn(e3) // SP, pn(e3) % SP, pf(e3) // SP, pf(e3) % SP)
        fin = jax.lax.fori_loop(0, NBODY, body, tuple(jnp.int32(v) for v in init))
        waited = ofree(NU + LAG)
        assert xneed(U2 + UPB) == NCH and ofree(U2 + UPB) <= waited <= odone(U2 - UPB)
        for c in range(ofree(U2 + UPB), waited):
            ocopy(c).wait()

        z = jnp.minimum(fin[0], 0)
        tile0 = (NB - 1) * SP
        slot0 = ((NB - 1) % RT) * SP
        lanes = pl.ds((NB - 1) * TB, TB)
        ecopies = []

        def ecopy(s_lo, s_hi, rlo=0, rhi=C):
            cp = pltpu.make_async_copy(
                obuf.at[pl.ds(slot0 + s_lo, s_hi - s_lo), pl.ds(rlo, rhi - rlo), :],
                o_hbm.at[pl.ds(s_lo, s_hi - s_lo), pl.ds(rlo, rhi - rlo), lanes],
                sems.at[ES0 + len(ecopies)])
            ecopies.append(cp)
            return cp

        ta, tb = NU - 2, NU - 1
        s_a, s_c, s_d = MO * U2 - tile0, MO * ta - tile0, MO * tb - tile0
        sent0, sent = odone(U2), (NB - 1) * CPT
        assert sent0 <= sent <= sent0 + MAXC and 0 < s_a and S - s_d == MO - 1
        ea, eb, ec = ecopy(0, s_a), ecopy(s_a, s_c), ecopy(s_c, s_d)

        def last2(i):
            units(U2 + z, 2, i)
            pl.when(i >= 0)(ea.start)
            copies(z + sent0, z + sent, z + NCH, z + NCH, z + waited, z + waited + MAXC)

        mta = [mc_ref if j < JS else ma_ref for j in range(NP)]
        mtb = [md_ref if j < JS else mc_ref for j in range(NP)]

        def last_a(i):
            output(U2 + z, mbuf[0])
            output(U2 + 1 + z, mbuf[1])
            unit(ta + z, True, mta, i, GROUPS_END, ORDER_END)
            carry_u0(tb + z)
            pl.when(i >= 0)(eb.start)

        def last_b(i):
            output(ta + z, mta)
            unit(tb + z, True, mtb, i, GROUPS_END, ORDER_END[:-1])
            pl.when(i >= 0)(ec.start)

        once(z, last2)
        once(z, last_a)
        once(z, last_b)
        RP = C // NEP
        for e in range(NEP):
            output(tb, mtb, e * RP, (e + 1) * RP, MO - 1)
            ecopy(s_d, S, e * RP, (e + 1) * RP).start()
        for c in range(waited + MAXC, sent):
            ocopy(c).wait()
        for cp in ecopies:
            cp.wait()

    any_spec = pl.BlockSpec(memory_space=pl.ANY)
    out = pl.pallas_call(
        kernel,
        in_specs=[any_spec] * 6,
        out_specs=any_spec,
        out_shape=jax.ShapeDtypeStruct((S, C, B), x.dtype),
        scratch_shapes=[
            pltpu.VMEM((NP, NKT + 1, C // 2, 128), U32),
            pltpu.VMEM((CF, TB), BF16),
            pltpu.VMEM((RING + 2, C, TB), BF16),
            pltpu.VMEM((RING, C, TB), BF16),
            pltpu.VMEM((C, 128), F32),
            pltpu.VMEM((C, 128), F32),
            pltpu.VMEM((NP, C, TB), F32),
            pltpu.VMEM((NP, C, TB), F32),
            pltpu.VMEM((NP, C, TB), F32),
            pltpu.VMEM((NP, C, TB), F32),
            pltpu.VMEM((NKT, C // 2, 128), U32),
            pltpu.VMEM((3, C // 2, 128), U32),
            pltpu.VMEM((C,), BF16), pltpu.VMEM((C,), BF16),
            pltpu.VMEM((C,), BF16), pltpu.VMEM((C,), BF16),
            pltpu.VMEM((3, C + 24, C), BF16),
            pltpu.SemaphoreType.DMA((NSEM,)),
        ],
        compiler_params=pltpu.CompilerParams(vmem_limit_bytes=100 * 1024 * 1024,
                                             disable_bounds_checks=True),
    )(jnp.transpose(x, (1, 2, 0)), w, mean, var, g, b)
    return jnp.transpose(out, (2, 0, 1))
```

```python
import jax
import jax.numpy as jnp
import jax.experimental.pallas as pl
import jax.experimental.pallas.tpu as pltpu

F32 = jnp.float32
BF16 = jnp.bfloat16
U32 = jnp.uint32

TB = 128
MO = 6
NP = MO + 2
UPB = 4
LAG = 2
NPRO = 3
RC = 16
CH = 8
RT = 4
LEAD = 3
NEP = 4
JS = 4
ORDER, GROUPS = (0, 7, 1, 2, 3, 4, 5, 6), (0, 1, 2, 3, 4)
ORDER_END, GROUPS_END = (0, 1, 2, 3, 4, 5, 6, 7), (0, 1, 2, 2, 2)
ORDER_PRO, ORDER_HALF, GROUPS_PRO = (0, 7, 5, 6, 3, 4, 1, 2), (1, 0, 7, 3, 4, 5, 6), (0, 1, 2, 3, 3)
EPS = 1e-5
CPK = {0: -2.25, 3: -0.025, 4: 0.075, 5: 0.8, 6: 2.4, 7: 2.25}


@jax.jit
def pallas_standalone__batchnorm__sampling_kernel(
    x: jax.Array,
    w: jax.Array,
    mean: jax.Array,
    var: jax.Array,
    g: jax.Array,
    b: jax.Array,
):
    B, S, C = x.shape
    NKT = C // 128
    CF = NKT * 128
    CR = C - CF
    SP = S + 1
    NB = B // TB
    NU = NB * SP // MO
    RING = RT * SP
    UPR = RING // MO
    CPT = S // CH
    NCH = NB * CPT
    NSC = RT * CPT
    U1 = NPRO + 1
    NBODY = (NU - U1 - 4) // UPB
    U2 = U1 + NBODY * UPB
    STEP = MO * UPB
    NSP = MO * NPRO + 1
    CSP = -(-NSP // CH)
    assert w.shape == (3, C, C) and 2 * CR == 128 and CPT == 4 and CH == 8
    assert NB * TB == B and NU * MO == NB * SP and UPR * MO == RING and U2 + 4 == NU and U1 % 4 == 0

    chunk_of = lambda p: CPT * (p // SP) + min((p % SP) // CH, CPT - 1)
    pn = lambda e: MO * e + MO - 1
    po = lambda e: MO * (e - LAG)
    pf = lambda e: po(e) - 1 - RING
    xneed = lambda e: min(chunk_of(pn(e)) + 1, NCH)
    odone = lambda e: CPT * (po(e) // SP) + (po(e) % SP) // CH
    ofree = lambda e: max(chunk_of(pf(e)) + 1, 0)
    ends = [U1] + [U1 + UPB * (i + 1) for i in range(NBODY)] + [U2 + 2, NU]
    MAXC = 3
    assert xneed(U1) + LEAD <= NSC and xneed(U2 + 2) == NCH and ofree(U1) == 0
    for e0, e1 in zip(ends[:-2], ends[1:-1]):
        assert max(xneed(e1) - xneed(e0), ofree(e1) - ofree(e0)) <= MAXC <= LEAD
        assert odone(e1) - odone(e0) <= MAXC and ofree(e1) <= (odone(e0 - UPB) if e0 > U1 else 0)
        old = min(xneed(e1) + LEAD, NCH) - 1 - NSC
        assert old < 0 or SP * (old // CPT) + CH * (old % CPT) + CH - 1 < MO * e0 - 1

    XS0, OS0, WS0 = 0, NSC, 2 * NSC
    PS0 = WS0 + NKT + 1
    KS0 = PS0 + 4
    ES0 = KS0 + NKT + 3
    NSEM = ES0 + 3 + NEP

    def kernel(x_hbm, w_hbm, mean_hbm, var_hbm, g_hbm, b_hbm, o_hbm,
               a_ref, u0_ref, xbuf, obuf, sh_ref, hs_ref, ma_ref, mb_ref, mc_ref, md_ref, w1_ref, wl_ref, p0, p1, p2, p3, wbuf, sems):

        def hbm_chunk(ref, c):
            lane0 = (c >> 2) * TB
            if not isinstance(c, int):
                lane0 = pl.multiple_of(lane0, TB)
            return ref.at[pl.ds((c & 3) * CH, CH), :, pl.ds(lane0, TB)]

        def ring_slot(c):
            return ((c >> 2) & (RT - 1)) * SP + (c & 3) * CH

        def xcopy(c):
            return pltpu.make_async_copy(hbm_chunk(x_hbm, c), xbuf.at[pl.ds(ring_slot(c) + 1, CH)],
                                         sems.at[XS0 + (c & (NSC - 1))])

        def ocopy(c):
            return pltpu.make_async_copy(obuf.at[pl.ds(ring_slot(c), CH)], hbm_chunk(o_hbm, c),
                                         sems.at[OS0 + (c & (NSC - 1))])

        def krows(kt):
            if isinstance(kt, int):
                return pl.ds(kt * 128, 128 if kt < NKT else CR)
            return pl.ds(pl.multiple_of(kt * 128, 128), 128)

        def wcopy(kt):
            return pltpu.make_async_copy(w_hbm.at[:, krows(kt), :], wbuf.at[:, krows(kt), :],
                                         sems.at[WS0 + kt])

        def kcopy(kt, lo=0, hi=NSP, sem=None):
            return pltpu.make_async_copy(x_hbm.at[pl.ds(lo, hi - lo), krows(kt), pl.ds(0, TB)],
                                         xbuf.at[pl.ds(1 + lo, hi - lo), krows(kt), :],
                                         sems.at[KS0 + kt if sem is None else sem])

        k0a_copy = kcopy(0, 0, MO + 1)
        k0b_copy = kcopy(0, MO + 1, NSP, KS0 + NKT + 1)
        rcopy = pltpu.make_async_copy(x_hbm.at[pl.ds(NSP, CSP * CH - NSP), :, pl.ds(0, TB)],
                                      xbuf.at[pl.ds(1 + NSP, CSP * CH - NSP)], sems.at[KS0 + NKT + 2])
        pcopies = [pltpu.make_async_copy(s, d, sems.at[PS0 + i])
                   for i, (s, d) in enumerate(zip((mean_hbm, var_hbm, g_hbm, b_hbm), (p0, p1, p2, p3)))]
        for c in pcopies:
            c.start()
        wcopy(0).start()
        k0a_copy.start()
        wcopy(1).start()
        k0b_copy.start()
        kcopy(1).start()
        for kt in range(2, NKT + 1):
            wcopy(kt).start()
            kcopy(kt).start()
        rcopy.start()
        for c in range(CSP, xneed(U1) + LEAD):
            xcopy(c).start()

        for s in [SP * q for q in range(RT + 1)] + [RING + 1]:
            xbuf[s] = jnp.zeros((C, TB), BF16)

        for c in pcopies:
            c.wait()
        mean_, var_, g_, b_ = [r[...].astype(F32).reshape(1, C) for r in (p0, p1, p2, p3)]
        scale = g_ * jax.lax.rsqrt(var_ + EPS)
        hs_ref[...] = jnp.broadcast_to(0.5 * scale, (128, C)).T
        sh = 0.5 * (b_ - mean_ * scale)
        sh_hi = sh.astype(BF16).astype(F32)
        sh_mid = (sh - sh_hi).astype(BF16).astype(F32)
        sh_lo = (sh - sh_hi) - sh_mid
        row = jax.lax.broadcasted_iota(jnp.int32, (128, C), 0)
        sh_ref[...] = jnp.where(row == CR, sh_hi, jnp.where(
            row == CR + 1, sh_mid, jnp.where(row == CR + 2, sh_lo, 0.0))).T

        def tchunk(ld_, with_u0, grp):
            ld = lambda i, gi: ld_(i, grp[gi])
            d1, d2, d3, d4, d5, d6 = [ld(i, 1) for i in range(1, 7)]
            e1, o1 = (d2 + d6) - 4.25 * d4, (d1 + d5) - 4.25 * d3
            d1, d2, d3, d4, d5, d6 = [ld(i, 2) for i in range(1, 7)]
            e2, o2 = (d6 - d4) - 0.25 * (d4 - d2), 2.0 * (d5 - d3) - 0.5 * (d3 - d1)
            d1, d2, d3, d4, d5, d6 = [ld(i, 3) for i in range(1, 7)]
            e3, o3 = (d6 - d4) - 4.0 * (d4 - d2), 0.5 * (d5 - d3) - 2.0 * (d3 - d1)
            d1, d3, d5, d7 = [ld(i, 4) for i in (1, 3, 5, 7)]
            u = [None, e1 + o1, e1 - o1, e2 + o2, e2 - o2, e3 + o3, e3 - o3, (d7 - d1) - 5.25 * (d5 - d3)]
            if with_u0:
                d0, d2, d4, d6 = [ld(i, 0) for i in (0, 2, 4, 6)]
                u[0] = (d0 - d6) + 5.25 * (d4 - d2)
            return u

        def ones_rows():
            return (jax.lax.broadcasted_iota(jnp.int32, (CR, TB), 0) < 3).astype(F32)

        def carry_u0(t):
            base = (t % UPR) * MO
            for r in range(0, CF, RC):
                d0, d2, d4, d6 = [xbuf[base + i, r:r + RC, :].astype(F32) for i in (0, 2, 4, 6)]
                u0_ref[r:r + RC, :] = ((d0 - d6) + 5.25 * (d4 - d2)).astype(BF16)

        def transform(t, carried, z, grp, order):
            zs = [0] + [jnp.minimum(z + q, 0) for q in range(1, 5)]
            never = z < 0
            base = (t % UPR) * MO
            gof = [grp[q] for q in (0, 1, 1, 2, 2, 3, 3, 4)]
            cs = []
            for r in range(0, C, RC):
                c = tchunk(lambda i, gi: xbuf[base + zs[gi] + i, r:r + RC, :].astype(F32),
                           not (carried and r < CF), grp)
                members = {}
                for j in order:
                    if c[j] is not None:
                        members.setdefault(gof[j], []).append(j)
                for j in set(j for mem in members.values() for j in mem[1:]) | {2}:
                    c[j] = pltpu.bitcast(c[j].astype(BF16), U32)
                for mem in members.values():
                    if len(mem) > 1 and mem[0] != 2:
                        dep = c[mem[1]]
                        for j in mem[2:]:
                            dep = dep ^ c[j]
                        top = jnp.where(never, jax.lax.bitcast_convert_type(dep, F32), c[mem[0]][0:RC // 2])
                        c[mem[0]] = jnp.concatenate([top, c[mem[0]][RC // 2:]], axis=0)
                cs.append(c)
            tail = pltpu.bitcast(jnp.concatenate([c[2] for c in cs[CF // RC:]], axis=0), BF16)
            us = {}
            for j in order:
                parts = [c[j] for c in cs if c[j] is not None]
                if j == 2:
                    parts = parts[:CF // RC]
                if j == 1:
                    parts = parts + [ones_rows()]
                v = jnp.concatenate(parts, axis=0)
                v = v.astype(BF16) if v.dtype == F32 else pltpu.bitcast(v, BF16)
                if j not in (1, 2):
                    v = jnp.concatenate([v, tail], axis=0)
                if j == 0 and carried:
                    v = jnp.concatenate([u0_ref[...], v], axis=0)
                us[j] = v
            return us

        def unit(t, carried, ms, i, grp, order):
            us = transform(t, carried, i, grp, order)
            z = jnp.minimum(i, 0)
            for j in order:
                nk = NKT if j == 2 else NKT + 1
                lhs = pltpu.bitcast(jnp.concatenate([a_ref[j, kt] for kt in range(nk)], axis=1), BF16)
                ms[j][j + z, 0:C, :] = jnp.dot(lhs, us[j], preferred_element_type=F32)

        def output(t, ms, rlo=0, rhi=C, nout=MO):
            base = (t % UPR) * MO
            for r in range(rlo, rhi, RC):
                m = [ms[j][j, r:r + RC, :] if (j < NP - 1 or nout == MO) else 0.0 for j in range(NP)]
                s1, s2, s3 = m[1] + m[2], m[3] + m[4], m[5] + m[6]
                d1, d2, d3 = m[1] - m[2], m[3] - m[4], m[5] - m[6]
                hs = hs_ref[r:r + RC, :]
                ys = [(hs * m[0] + s1) + (s2 + s3),
                      (d1 + 2.0 * d2) + 0.5 * d3,
                      (s1 + 4.0 * s2) + 0.25 * s3,
                      (d1 + 8.0 * d2) + 0.125 * d3,
                      (s1 + 16.0 * s2) + 0.0625 * s3,
                      (d1 + 32.0 * d2) + (0.03125 * d3 + hs * m[7])]
                for i in range(nout):
                    h = ys[i]
                    obuf[base + i, r:r + RC, :] = (h * jnp.tanh(h) + h).astype(BF16)

        mbuf = [[r] * NP for r in (ma_ref, mb_ref, mc_ref, md_ref)]

        def once(z, fn):
            def trip(i, c):
                fn(i)
                return c
            jax.lax.fori_loop(0, z + 1, trip, 0)

        def xpose(kt):
            last = isinstance(kt, int) and kt == NKT
            for r in range(0, C, 128):
                cols = slice(r, min(r + 128, C))
                rows = slice(r // 2, min(r + 128, C) // 2)
                for k, dst in enumerate((a_ref.at[0], w1_ref, a_ref.at[NP - 1])):
                    if last:
                        t = jnp.concatenate([wbuf[k, CF:C, cols]] * 2, axis=0).T
                        wl_ref[k, rows, :] = pltpu.bitcast(t, U32)
                    else:
                        dst[kt, rows, :] = pltpu.bitcast(wbuf[k, krows(kt), cols].T, U32)

        def combos(kt, zs, never):
            last = isinstance(kt, int) and kt == NKT
            lo = jax.lax.broadcasted_iota(jnp.int32, (RC, 128), 1) < CR
            pack = lambda v: pltpu.bitcast(v.astype(BF16), U32)
            out = dict((j, []) for j in range(NP))
            for r in range(0, C, RC):
                rows = slice(r // 2, (r + RC) // 2)
                def taps(gi):
                    if last:
                        raw = [wl_ref[k + zs[gi], rows, :] for k in range(3)]
                    else:
                        raw = [a_ref[zs[gi], kt, rows, :], w1_ref[kt + zs[gi], rows, :], a_ref[NP - 1 + zs[gi], kt, rows, :]]
                    return [pltpu.bitcast(t, BF16).astype(F32) for t in raw]
                hs = hs_ref[r:r + RC, :]
                for gi, (ce0, ce2, co) in enumerate(((-2.0 / 9, -2.0 / 9, -2.0 / 9), (1.0 / 90, 2.0 / 45, 1.0 / 45),
                                                     (32.0 / 45, 8.0 / 45, 16.0 / 45))):
                    w0, w1, w2 = [t * hs for t in taps(gi)]
                    e = ce0 * (w0 + w2) if gi == 0 else ce0 * w0 + ce2 * w2
                    o = co * w1
                    ja, jb = 2 * gi + 1, 2 * gi + 2
                    ga, gb = e + o, e - o
                    if last:
                        if gi == 0:
                            out[1].append(pack(jnp.where(lo, ga, sh_ref[r:r + RC, :])))
                            continue
                        g2 = (w0 + w2) - w1
                        ga = jnp.where(lo, ga, (-2.0 / 9 * CPK[ja]) * g2)
                        gb = jnp.where(lo, gb, (-2.0 / 9 * CPK[jb]) * g2)
                    pb = pack(gb)
                    out[ja].append(jnp.where(never, pb, pack(ga)))
                    out[jb].append(pb)
                if last:
                    r0, r1, r2 = taps(3)
                    raw2 = (r0 + r2) - r1
                    p7 = pack(jnp.where(lo, r2, (-2.0 / 9 * CPK[7]) * raw2))
                    out[0].append(jnp.where(never, p7, pack(jnp.where(lo, r0, (-2.0 / 9 * CPK[0]) * raw2))))
                    out[7].append(p7)
            res = {}
            for j in range(NP):
                if out[j]:
                    res[j] = jnp.concatenate(out[j], axis=0)
                    a_ref[j, kt] = res[j]
                elif not last:
                    res[j] = a_ref[j, kt]
            return res

        def mm(kt, i, order, units=(0, 1, 2), fresh=True):
            last = isinstance(kt, int) and kt == NKT
            r0 = kt * 128 if isinstance(kt, int) else pl.multiple_of(kt * 128, 128)
            zs = [jnp.minimum(i + q, 0) for q in range(5)]
            lhs = combos(kt, zs, i < 0) if fresh else dict((j, a_ref[j, kt]) for j in range(NP))
            rhs = []
            for u in units:
                cs = [tchunk(lambda s, gi: xbuf[MO * u + s + zs[gi], pl.ds(r0 + r, RC), :].astype(F32),
                             True, GROUPS_PRO) for r in range(0, CR if last else 128, RC)]
                fin = lambda j: jnp.concatenate([c[j] for c in cs], axis=0).astype(BF16)
                rhs.append(dict(
                    (j, jnp.concatenate([fin(j), ones_rows().astype(BF16) if j == 1 else fin(2)], axis=0)
                     if last else fin(j)) for j in lhs))

            def products():
                for j in order:
                    for u, rh in zip(units, rhs):
                        m_ref = mbuf[u][j]
                        p = jnp.dot(pltpu.bitcast(lhs[j], BF16), rh[j], preferred_element_type=F32)
                        m_ref[j] = p if isinstance(kt, int) and kt == 0 else m_ref[j] + p
            return products

        def kblock(kt, i):
            kcopy(kt).wait()
            wcopy(kt + 1).wait()
            xpose(kt + 1)
            mm(kt, i, ORDER_PRO)()
            return 0

        wcopy(0).wait()
        xpose(0)
        z = jax.lax.fori_loop(0, 2, lambda i, c: jnp.minimum(i, c), jnp.int32(0))
        k0a_copy.wait()
        once(z, lambda i: mm(0, i, ORDER_PRO, (0,))())
        wcopy(1).wait()
        k0b_copy.wait()
        once(z, lambda i: (xpose(1), mm(0, i, ORDER_PRO, (1, 2), False)()))
        jax.lax.fori_loop(1, NKT - 1, lambda i, c: kblock(i, i), 0)
        wcopy(NKT).wait()
        kcopy(NKT - 1).wait()
        kcopy(NKT).wait()

        def klast(i):
            xpose(NKT)
            for products in [mm(NKT - 1, i, ORDER), mm(NKT, i, ORDER_HALF)]:
                products()

        once(z, klast)
        rcopy.wait()
        for c in range(CSP, xneed(U1)):
            xcopy(c).wait()
        carry_u0(NPRO)

        def units(t0, n, i):
            for k in range(n):
                unit(t0 + k, k == 0, mbuf[k], i, GROUPS, ORDER)
                output(t0 + k - LAG, mbuf[(k - LAG) % 4])
            carry_u0(t0 + n)

        def copies(o0, o1, n0, n1, f0, f1):
            for k in range(MAXC):
                pl.when(o0 + k < o1)(lambda: ocopy(o0 + k).start())
            for k in range(MAXC):
                pl.when(jnp.logical_and(n0 + k < n1, n0 + k + LEAD < NCH))(lambda: xcopy(n0 + k + LEAD).start())
            for k in range(MAXC):
                pl.when(n0 + k < n1)(lambda: xcopy(n0 + k).wait())
            for k in range(MAXC):
                pl.when(f0 + k < f1)(lambda: ocopy(f0 + k).wait())

        def first1(i):
            output(z, mbuf[0])
            output(z + 1, mbuf[1])
            unit(NPRO + z, True, mbuf[NPRO], i, GROUPS, ORDER)
            carry_u0(U1 + z)
            copies(z, z + odone(U1), z + xneed(U1), z + xneed(U1 + UPB), z, z + ofree(U1 + UPB))

        once(z, first1)

        def advance(q, r):
            wrap = r + STEP >= SP
            return q + wrap.astype(jnp.int32), jnp.where(wrap, r + STEP - SP, r + STEP)

        def body(i, carry):
            o0, o1, n0, n1, f0, f1, qo, ro, qn, rn, qf, rf = carry
            units(U1 + UPB * i, UPB, i)
            copies(o0, o1, n0, n1, f0, f1)
            o2 = CPT * qo + (ro >> 3)
            n2 = jnp.minimum(CPT * qn + jnp.minimum(rn >> 3, CPT - 1) + 1, NCH)
            f2 = jnp.maximum(CPT * qf + jnp.minimum(rf >> 3, CPT - 1) + 1, 0)
            return (o1, o2, n1, n2, f1, f2) + advance(qo, ro) + advance(qn, rn) + advance(qf, rf)

        e1, e2, e3 = U1 + UPB, U1 + 2 * UPB, U1 + 3 * UPB
        init = (odone(U1), odone(e1), xneed(e1), xneed(e2), ofree(e1), ofree(e2),
                po(e2) // SP, po(e2) % SP, pn(e3) // SP, pn(e3) % SP, pf(e3) // SP, pf(e3) % SP)
        fin = jax.lax.fori_loop(0, NBODY, body, tuple(jnp.int32(v) for v in init))
        waited = ofree(NU + LAG)
        assert xneed(U2 + UPB) == NCH and ofree(U2 + UPB) <= waited <= odone(U2 - UPB)
        for c in range(ofree(U2 + UPB), waited):
            ocopy(c).wait()

        z = jnp.minimum(fin[0], 0)
        tile0 = (NB - 1) * SP
        slot0 = ((NB - 1) % RT) * SP
        lanes = pl.ds((NB - 1) * TB, TB)
        ecopies = []

        def ecopy(s_lo, s_hi, rlo=0, rhi=C):
            cp = pltpu.make_async_copy(
                obuf.at[pl.ds(slot0 + s_lo, s_hi - s_lo), pl.ds(rlo, rhi - rlo), :],
                o_hbm.at[pl.ds(s_lo, s_hi - s_lo), pl.ds(rlo, rhi - rlo), lanes],
                sems.at[ES0 + len(ecopies)])
            ecopies.append(cp)
            return cp

        ta, tb = NU - 2, NU - 1
        s_a, s_c, s_d = MO * U2 - tile0, MO * ta - tile0, MO * tb - tile0
        sent0, sent = odone(U2), (NB - 1) * CPT
        assert sent0 <= sent <= sent0 + MAXC and 0 < s_a and S - s_d == MO - 1
        ea, eb, ec = ecopy(0, s_a), ecopy(s_a, s_c), ecopy(s_c, s_d)

        def last2(i):
            units(U2 + z, 2, i)
            pl.when(i >= 0)(ea.start)
            copies(z + sent0, z + sent, z + NCH, z + NCH, z + waited, z + waited + MAXC)

        mta = [mc_ref if j < JS else ma_ref for j in range(NP)]
        mtb = [md_ref if j < JS else mc_ref for j in range(NP)]

        def last_a(i):
            output(U2 + z, mbuf[0])
            output(U2 + 1 + z, mbuf[1])
            unit(ta + z, True, mta, i, GROUPS_END, ORDER_END)
            carry_u0(tb + z)
            pl.when(i >= 0)(eb.start)

        def last_b(i):
            output(ta + z, mta)
            unit(tb + z, True, mtb, i, GROUPS_END, ORDER_END[:-1])
            pl.when(i >= 0)(ec.start)

        once(z, last2)
        once(z, last_a)
        once(z, last_b)
        RP = C // NEP
        for e in range(NEP):
            output(tb, mtb, e * RP, (e + 1) * RP, MO - 1)
            ecopy(s_d, S, e * RP, (e + 1) * RP).start()
        for c in range(waited + MAXC, sent):
            ocopy(c).wait()
        for cp in ecopies:
            cp.wait()

    any_spec = pl.BlockSpec(memory_space=pl.ANY)
    out = pl.pallas_call(
        kernel,
        in_specs=[any_spec] * 6,
        out_specs=any_spec,
        out_shape=jax.ShapeDtypeStruct((S, C, B), x.dtype),
        scratch_shapes=[
            pltpu.VMEM((NP, NKT + 1, C // 2, 128), U32),
            pltpu.VMEM((CF, TB), BF16),
            pltpu.VMEM((RING + 2, C, TB), BF16),
            pltpu.VMEM((RING, C, TB), BF16),
            pltpu.VMEM((C, 128), F32),
            pltpu.VMEM((C, 128), F32),
            pltpu.VMEM((NP, C, TB), F32),
            pltpu.VMEM((NP, C, TB), F32),
            pltpu.VMEM((NP, C, TB), F32),
            pltpu.VMEM((NP, C, TB), F32),
            pltpu.VMEM((NKT, C // 2, 128), U32),
            pltpu.VMEM((3, C // 2, 128), U32),
            pltpu.VMEM((C,), BF16), pltpu.VMEM((C,), BF16),
            pltpu.VMEM((C,), BF16), pltpu.VMEM((C,), BF16),
            pltpu.VMEM((3, C + 24, C), BF16),
            pltpu.SemaphoreType.DMA((NSEM,)),
        ],
        compiler_params=pltpu.CompilerParams(vmem_limit_bytes=100 * 1024 * 1024,
                                             disable_bounds_checks=True),
    )(jnp.transpose(x, (1, 2, 0)), w, mean, var, g, b)
    return jnp.transpose(out, (2, 0, 1))
```

```python
import jax
import jax.numpy as jnp
import jax.experimental.pallas as pl
import jax.experimental.pallas.tpu as pltpu

F32 = jnp.float32
BF16 = jnp.bfloat16
U32 = jnp.uint32

TB = 128
MO = 6
NP = MO + 2
UPB = 4
LAG = 2
NPRO = 3
RC = 16
CH = 8
RT = 4
LEAD = 3
NEP = 4
JS = 4
ORDER, GROUPS = (0, 7, 1, 2, 3, 4, 5, 6), (0, 1, 2, 3, 4)
ORDER_END, GROUPS_END = (0, 1, 2, 3, 4, 5, 6, 7), (0, 1, 2, 2, 2)
ORDER_PRO, ORDER_HALF, GROUPS_PRO = (0, 7, 5, 6, 3, 4, 1, 2), (1, 0, 7, 3, 4, 5, 6), (0, 1, 2, 3, 3)
EPS = 1e-5
CPK = {0: -2.25, 3: -0.025, 4: 0.075, 5: 0.8, 6: 2.4, 7: 2.25}


@jax.jit
def pallas_standalone__batchnorm__sampling_kernel(
    x: jax.Array,
    w: jax.Array,
    mean: jax.Array,
    var: jax.Array,
    g: jax.Array,
    b: jax.Array,
):
    B, S, C = x.shape
    NKT = C // 128
    CF = NKT * 128
    CR = C - CF
    SP = S + 1
    NB = B // TB
    NU = NB * SP // MO
    RING = RT * SP
    UPR = RING // MO
    CPT = S // CH
    NCH = NB * CPT
    NSC = RT * CPT
    U1 = NPRO + 1
    NBODY = (NU - U1 - 4) // UPB
    U2 = U1 + NBODY * UPB
    STEP = MO * UPB
    NSP = MO * NPRO + 1
    CSP = -(-NSP // CH)
    assert w.shape == (3, C, C) and 2 * CR == 128 and CPT == 4 and CH == 8
    assert NB * TB == B and NU * MO == NB * SP and UPR * MO == RING and U2 + 4 == NU and U1 % 4 == 0

    chunk_of = lambda p: CPT * (p // SP) + min((p % SP) // CH, CPT - 1)
    pn = lambda e: MO * e + MO - 1
    po = lambda e: MO * (e - LAG)
    xneed = lambda e: min(chunk_of(pn(e)) + 1, NCH)
    odone = lambda e: CPT * (po(e) // SP) + (po(e) % SP) // CH
    ends = [U1] + [U1 + UPB * (i + 1) for i in range(NBODY)] + [U2 + 2, NU]
    MAXC = 3
    assert xneed(U1) + LEAD <= NSC and xneed(U2 + 2) == NCH
    for e0, e1 in zip(ends[:-2], ends[1:-1]):
        assert max(xneed(e1) - xneed(e0), odone(e1) - odone(e0)) <= MAXC <= LEAD
        old = min(xneed(e1) + LEAD, NCH) - 1 - NSC
        assert old < 0 or SP * (old // CPT) + CH * (old % CPT) + CH - 1 < MO * e0 - 1

    XS0, OS0, WS0 = 0, NSC, NSC + NCH
    PS0 = WS0 + NKT + 1
    KS0 = PS0 + 4
    ES0 = KS0 + NKT + 3
    NSEM = ES0 + 3 + NEP

    def kernel(x_hbm, w_hbm, mean_hbm, var_hbm, g_hbm, b_hbm, o_hbm,
               a_ref, u0_ref, xbuf, obuf, sh_ref, hs_ref, ma_ref, mb_ref, mc_ref, md_ref,
               w1_ref, wl_ref, p0, p1, p2, p3, wbuf, sems):

        def hbm_chunk(ref, c):
            lane0 = (c >> 2) * TB
            if not isinstance(c, int):
                lane0 = pl.multiple_of(lane0, TB)
            return ref.at[pl.ds((c & 3) * CH, CH), :, pl.ds(lane0, TB)]

        def ring_slot(c):
            return ((c >> 2) & (RT - 1)) * SP + (c & 3) * CH

        def xcopy(c):
            return pltpu.make_async_copy(hbm_chunk(x_hbm, c), xbuf.at[pl.ds(ring_slot(c) + 1, CH)],
                                         sems.at[XS0 + (c & (NSC - 1))])

        def ocopy(c):
            return pltpu.make_async_copy(obuf.at[pl.ds((c >> 2) * SP + (c & 3) * CH, CH)], hbm_chunk(o_hbm, c),
                                         sems.at[OS0 + c])

        def krows(kt):
            if isinstance(kt, int):
                return pl.ds(kt * 128, 128 if kt < NKT else CR)
            return pl.ds(pl.multiple_of(kt * 128, 128), 128)

        def wcopy(kt):
            return pltpu.make_async_copy(w_hbm.at[:, krows(kt), :], wbuf.at[:, krows(kt), :],
                                         sems.at[WS0 + kt])

        def kcopy(kt, lo=0, hi=NSP, sem=None):
            return pltpu.make_async_copy(x_hbm.at[pl.ds(lo, hi - lo), krows(kt), pl.ds(0, TB)],
                                         xbuf.at[pl.ds(1 + lo, hi - lo), krows(kt), :],
                                         sems.at[KS0 + kt if sem is None else sem])

        k0a_copy = kcopy(0, 0, MO + 1)
        k0b_copy = kcopy(0, MO + 1, NSP, KS0 + NKT + 1)
        rcopy = pltpu.make_async_copy(x_hbm.at[pl.ds(NSP, CSP * CH - NSP), :, pl.ds(0, TB)],
                                      xbuf.at[pl.ds(1 + NSP, CSP * CH - NSP)], sems.at[KS0 + NKT + 2])
        pcopies = [pltpu.make_async_copy(s, d, sems.at[PS0 + i])
                   for i, (s, d) in enumerate(zip((mean_hbm, var_hbm, g_hbm, b_hbm), (p0, p1, p2, p3)))]
        for c in pcopies:
            c.start()
        wcopy(0).start()
        k0a_copy.start()
        wcopy(1).start()
        k0b_copy.start()
        kcopy(1).start()
        for kt in range(2, NKT + 1):
            wcopy(kt).start()
            kcopy(kt).start()
        rcopy.start()
        for c in range(CSP, xneed(U1) + LEAD):
            xcopy(c).start()

        for s in [SP * q for q in range(RT + 1)] + [RING + 1]:
            xbuf[s] = jnp.zeros((C, TB), BF16)

        for c in pcopies:
            c.wait()
        mean_, var_, g_, b_ = [r[...].astype(F32).reshape(1, C) for r in (p0, p1, p2, p3)]
        scale = g_ * jax.lax.rsqrt(var_ + EPS)
        hs_ref[...] = jnp.broadcast_to(0.5 * scale, (128, C)).T
        sh = 0.5 * (b_ - mean_ * scale)
        sh_hi = sh.astype(BF16).astype(F32)
        sh_mid = (sh - sh_hi).astype(BF16).astype(F32)
        sh_lo = (sh - sh_hi) - sh_mid
        row = jax.lax.broadcasted_iota(jnp.int32, (128, C), 0)
        sh_ref[...] = jnp.where(row == CR, sh_hi, jnp.where(
            row == CR + 1, sh_mid, jnp.where(row == CR + 2, sh_lo, 0.0))).T

        def tchunk(ld_, with_u0, grp):
            ld = lambda i, gi: ld_(i, grp[gi])
            d1, d2, d3, d4, d5, d6 = [ld(i, 1) for i in range(1, 7)]
            e1, o1 = (d2 + d6) - 4.25 * d4, (d1 + d5) - 4.25 * d3
            d1, d2, d3, d4, d5, d6 = [ld(i, 2) for i in range(1, 7)]
            e2, o2 = (d6 - d4) - 0.25 * (d4 - d2), 2.0 * (d5 - d3) - 0.5 * (d3 - d1)
            d1, d2, d3, d4, d5, d6 = [ld(i, 3) for i in range(1, 7)]
            e3, o3 = (d6 - d4) - 4.0 * (d4 - d2), 0.5 * (d5 - d3) - 2.0 * (d3 - d1)
            d1, d3, d5, d7 = [ld(i, 4) for i in (1, 3, 5, 7)]
            u = [None, e1 + o1, e1 - o1, e2 + o2, e2 - o2, e3 + o3, e3 - o3, (d7 - d1) - 5.25 * (d5 - d3)]
            if with_u0:
                d0, d2, d4, d6 = [ld(i, 0) for i in (0, 2, 4, 6)]
                u[0] = (d0 - d6) + 5.25 * (d4 - d2)
            return u

        def ones_rows():
            return (jax.lax.broadcasted_iota(jnp.int32, (CR, TB), 0) < 3).astype(F32)

        def carry_u0(t):
            base = (t % UPR) * MO
            for r in range(0, CF, RC):
                d0, d2, d4, d6 = [xbuf[base + i, r:r + RC, :].astype(F32) for i in (0, 2, 4, 6)]
                u0_ref[r:r + RC, :] = ((d0 - d6) + 5.25 * (d4 - d2)).astype(BF16)

        def transform(t, carried, z, grp, order):
            zs = [0] + [jnp.minimum(z + q, 0) for q in range(1, 5)]
            never = z < 0
            base = (t % UPR) * MO
            gof = [grp[q] for q in (0, 1, 1, 2, 2, 3, 3, 4)]
            cs = []
            for r in range(0, C, RC):
                c = tchunk(lambda i, gi: xbuf[base + zs[gi] + i, r:r + RC, :].astype(F32),
                           not (carried and r < CF), grp)
                members = {}
                for j in order:
                    if c[j] is not None:
                        members.setdefault(gof[j], []).append(j)
                for j in set(j for mem in members.values() for j in mem[1:]) | {2}:
                    c[j] = pltpu.bitcast(c[j].astype(BF16), U32)
                for mem in members.values():
                    if len(mem) > 1 and mem[0] != 2:
                        dep = c[mem[1]]
                        for j in mem[2:]:
                            dep = dep ^ c[j]
                        top = jnp.where(never, jax.lax.bitcast_convert_type(dep, F32), c[mem[0]][0:RC // 2])
                        c[mem[0]] = jnp.concatenate([top, c[mem[0]][RC // 2:]], axis=0)
                cs.append(c)
            tail = pltpu.bitcast(jnp.concatenate([c[2] for c in cs[CF // RC:]], axis=0), BF16)
            us = {}
            for j in order:
                parts = [c[j] for c in cs if c[j] is not None]
                if j == 2:
                    parts = parts[:CF // RC]
                if j == 1:
                    parts = parts + [ones_rows()]
                v = jnp.concatenate(parts, axis=0)
                v = v.astype(BF16) if v.dtype == F32 else pltpu.bitcast(v, BF16)
                if j not in (1, 2):
                    v = jnp.concatenate([v, tail], axis=0)
                if j == 0 and carried:
                    v = jnp.concatenate([u0_ref[...], v], axis=0)
                us[j] = v
            return us

        def unit(t, carried, ms, i, grp, order):
            us = transform(t, carried, i, grp, order)
            z = jnp.minimum(i, 0)
            for j in order:
                nk = NKT if j == 2 else NKT + 1
                lhs = pltpu.bitcast(jnp.concatenate([a_ref[j, kt] for kt in range(nk)], axis=1), BF16)
                ms[j][j + z, 0:C, :] = jnp.dot(lhs, us[j], preferred_element_type=F32)

        def output(t, ms, rlo=0, rhi=C, nout=MO):
            base = (t % UPR) * MO + (t // UPR) * RING
            for r in range(rlo, rhi, RC):
                m = [ms[j][j, r:r + RC, :] if (j < NP - 1 or nout == MO) else 0.0 for j in range(NP)]
                s1, s2, s3 = m[1] + m[2], m[3] + m[4], m[5] + m[6]
                d1, d2, d3 = m[1] - m[2], m[3] - m[4], m[5] - m[6]
                hs = hs_ref[r:r + RC, :]
                ys = [(hs * m[0] + s1) + (s2 + s3),
                      (d1 + 2.0 * d2) + 0.5 * d3,
                      (s1 + 4.0 * s2) + 0.25 * s3,
                      (d1 + 8.0 * d2) + 0.125 * d3,
                      (s1 + 16.0 * s2) + 0.0625 * s3,
                      (d1 + 32.0 * d2) + (0.03125 * d3 + hs * m[7])]
                for i in range(nout):
                    h = ys[i]
                    obuf[base + i, r:r + RC, :] = (h * jnp.tanh(h) + h).astype(BF16)

        mbuf = [[r] * NP for r in (ma_ref, mb_ref, mc_ref, md_ref)]

        def once(z, fn):
            def trip(i, c):
                fn(i)
                return c
            jax.lax.fori_loop(0, z + 1, trip, 0)

        def xpose(kt):
            last = isinstance(kt, int) and kt == NKT
            for r in range(0, C, 128):
                cols = slice(r, min(r + 128, C))
                rows = slice(r // 2, min(r + 128, C) // 2)
                for k, dst in enumerate((a_ref.at[0], w1_ref, a_ref.at[NP - 1])):
                    if last:
                        t = jnp.concatenate([wbuf[k, CF:C, cols]] * 2, axis=0).T
                        wl_ref[k, rows, :] = pltpu.bitcast(t, U32)
                    else:
                        dst[kt, rows, :] = pltpu.bitcast(wbuf[k, krows(kt), cols].T, U32)

        def combos(kt, zs, never):
            last = isinstance(kt, int) and kt == NKT
            lo = jax.lax.broadcasted_iota(jnp.int32, (RC, 128), 1) < CR
            pack = lambda v: pltpu.bitcast(v.astype(BF16), U32)
            out = dict((j, []) for j in range(NP))
            for r in range(0, C, RC):
                rows = slice(r // 2, (r + RC) // 2)
                def taps(gi):
                    if last:
                        raw = [wl_ref[k + zs[gi], rows, :] for k in range(3)]
                    else:
                        raw = [a_ref[zs[gi], kt, rows, :], w1_ref[kt + zs[gi], rows, :], a_ref[NP - 1 + zs[gi], kt, rows, :]]
                    return [pltpu.bitcast(t, BF16).astype(F32) for t in raw]
                hs = hs_ref[r:r + RC, :]
                for gi, (ce0, ce2, co) in enumerate(((-2.0 / 9, -2.0 / 9, -2.0 / 9), (1.0 / 90, 2.0 / 45, 1.0 / 45),
                                                     (32.0 / 45, 8.0 / 45, 16.0 / 45))):
                    w0, w1, w2 = [t * hs for t in taps(gi)]
                    e = ce0 * (w0 + w2) if gi == 0 else ce0 * w0 + ce2 * w2
                    o = co * w1
                    ja, jb = 2 * gi + 1, 2 * gi + 2
                    ga, gb = e + o, e - o
                    if last:
                        if gi == 0:
                            out[1].append(pack(jnp.where(lo, ga, sh_ref[r:r + RC, :])))
                            continue
                        g2 = (w0 + w2) - w1
                        ga = jnp.where(lo, ga, (-2.0 / 9 * CPK[ja]) * g2)
                        gb = jnp.where(lo, gb, (-2.0 / 9 * CPK[jb]) * g2)
                    pb = pack(gb)
                    out[ja].append(jnp.where(never, pb, pack(ga)))
                    out[jb].append(pb)
                if last:
                    r0, r1, r2 = taps(3)
                    raw2 = (r0 + r2) - r1
                    p7 = pack(jnp.where(lo, r2, (-2.0 / 9 * CPK[7]) * raw2))
                    out[0].append(jnp.where(never, p7, pack(jnp.where(lo, r0, (-2.0 / 9 * CPK[0]) * raw2))))
                    out[7].append(p7)
            res = {}
            for j in range(NP):
                if out[j]:
                    res[j] = jnp.concatenate(out[j], axis=0)
                    a_ref[j, kt] = res[j]
                elif not last:
                    res[j] = a_ref[j, kt]
            return res

        def mm(kt, i, order, units=(0, 1, 2), fresh=True):
            last = isinstance(kt, int) and kt == NKT
            r0 = kt * 128 if isinstance(kt, int) else pl.multiple_of(kt * 128, 128)
            zs = [jnp.minimum(i + q, 0) for q in range(5)]
            lhs = combos(kt, zs, i < 0) if fresh else dict((j, a_ref[j, kt]) for j in range(NP))
            rhs = []
            for u in units:
                cs = [tchunk(lambda s, gi: xbuf[MO * u + s + zs[gi], pl.ds(r0 + r, RC), :].astype(F32),
                             True, GROUPS_PRO) for r in range(0, CR if last else 128, RC)]
                fin = lambda j: jnp.concatenate([c[j] for c in cs], axis=0).astype(BF16)
                rhs.append(dict(
                    (j, jnp.concatenate([fin(j), ones_rows().astype(BF16) if j == 1 else fin(2)], axis=0)
                     if last else fin(j)) for j in lhs))

            def products():
                for j in order:
                    for u, rh in zip(units, rhs):
                        m_ref = mbuf[u][j]
                        p = jnp.dot(pltpu.bitcast(lhs[j], BF16), rh[j], preferred_element_type=F32)
                        m_ref[j] = p if isinstance(kt, int) and kt == 0 else m_ref[j] + p
            return products

        def kblock(kt, i):
            kcopy(kt).wait()
            wcopy(kt + 1).wait()
            xpose(kt + 1)
            mm(kt, i, ORDER_PRO)()
            return 0

        wcopy(0).wait()
        xpose(0)
        z = jax.lax.fori_loop(0, 2, lambda i, c: jnp.minimum(i, c), jnp.int32(0))
        k0a_copy.wait()
        once(z, lambda i: mm(0, i, ORDER_PRO, (0,))())
        wcopy(1).wait()
        k0b_copy.wait()
        once(z, lambda i: (xpose(1), mm(0, i, ORDER_PRO, (1, 2), False)()))
        jax.lax.fori_loop(1, NKT - 1, lambda i, c: kblock(i, i), 0)
        wcopy(NKT).wait()
        kcopy(NKT - 1).wait()
        kcopy(NKT).wait()

        def klast(i):
            xpose(NKT)
            for products in [mm(NKT - 1, i, ORDER), mm(NKT, i, ORDER_HALF)]:
                products()

        once(z, klast)
        rcopy.wait()
        for c in range(CSP, xneed(U1)):
            xcopy(c).wait()
        carry_u0(NPRO)

        def units(t0, n, i):
            for k in range(n):
                unit(t0 + k, k == 0, mbuf[k], i, GROUPS, ORDER)
                output(t0 + k - LAG, mbuf[(k - LAG) % 4])
            carry_u0(t0 + n)

        def copies(o0, o1, n0, n1):
            for k in range(MAXC):
                pl.when(o0 + k < o1)(lambda: ocopy(o0 + k).start())
            for k in range(MAXC):
                pl.when(jnp.logical_and(n0 + k < n1, n0 + k + LEAD < NCH))(lambda: xcopy(n0 + k + LEAD).start())
            for k in range(MAXC):
                pl.when(n0 + k < n1)(lambda: xcopy(n0 + k).wait())

        def first1(i):
            output(z, mbuf[0])
            output(z + 1, mbuf[1])
            unit(NPRO + z, True, mbuf[NPRO], i, GROUPS, ORDER)
            carry_u0(U1 + z)
            copies(z, z + odone(U1), z + xneed(U1), z + xneed(U1 + UPB))

        once(z, first1)

        def advance(q, r):
            wrap = r + STEP >= SP
            return q + wrap.astype(jnp.int32), jnp.where(wrap, r + STEP - SP, r + STEP)

        def body(i, carry):
            o0, o1, n0, n1, qo, ro, qn, rn = carry
            units(U1 + UPB * i, UPB, i)
            copies(o0, o1, n0, n1)
            o2 = CPT * qo + (ro >> 3)
            n2 = jnp.minimum(CPT * qn + jnp.minimum(rn >> 3, CPT - 1) + 1, NCH)
            return (o1, o2, n1, n2) + advance(qo, ro) + advance(qn, rn)

        e1, e2, e3 = U1 + UPB, U1 + 2 * UPB, U1 + 3 * UPB
        init = (odone(U1), odone(e1), xneed(e1), xneed(e2), po(e2) // SP, po(e2) % SP, pn(e3) // SP, pn(e3) % SP)
        fin = jax.lax.fori_loop(0, NBODY, body, tuple(jnp.int32(v) for v in init))
        assert xneed(U2 + UPB) == NCH

        z = jnp.minimum(fin[0], 0)
        tile0 = (NB - 1) * SP
        lanes = pl.ds((NB - 1) * TB, TB)
        ecopies = []

        def ecopy(s_lo, s_hi, rlo=0, rhi=C):
            cp = pltpu.make_async_copy(
                obuf.at[pl.ds(tile0 + s_lo, s_hi - s_lo), pl.ds(rlo, rhi - rlo), :],
                o_hbm.at[pl.ds(s_lo, s_hi - s_lo), pl.ds(rlo, rhi - rlo), lanes],
                sems.at[ES0 + len(ecopies)])
            ecopies.append(cp)
            return cp

        ta, tb = NU - 2, NU - 1
        s_a, s_c, s_d = MO * U2 - tile0, MO * ta - tile0, MO * tb - tile0
        sent0, sent = odone(U2), (NB - 1) * CPT
        assert sent0 <= sent <= sent0 + MAXC and 0 < s_a and S - s_d == MO - 1
        ea, eb, ec = ecopy(0, s_a), ecopy(s_a, s_c), ecopy(s_c, s_d)

        def last2(i):
            units(U2 + z, 2, i)
            pl.when(i >= 0)(ea.start)
            copies(z + sent0, z + sent, z + NCH, z + NCH)
            pl.when(i >= 0)(ocopy(z).wait)

        mta = [mc_ref if j < JS else ma_ref for j in range(NP)]
        mtb = [md_ref if j < JS else mc_ref for j in range(NP)]

        def last_a(i):
            output(U2 + z, mbuf[0])
            output(U2 + 1 + z, mbuf[1])
            unit(ta + z, True, mta, i, GROUPS_END, ORDER_END)
            carry_u0(tb + z)
            pl.when(i >= 0)(eb.start)

        def last_b(i):
            output(ta + z, mta)
            unit(tb + z, True, mtb, i, GROUPS_END, ORDER_END[:-1])
            pl.when(i >= 0)(ec.start)

        once(z, last2)
        once(z, last_a)
        once(z, last_b)
        RP = C // NEP
        for e in range(NEP):
            output(tb, mtb, e * RP, (e + 1) * RP, MO - 1)
            ecopy(s_d, S, e * RP, (e + 1) * RP).start()
        for c in range(1, sent):
            ocopy(c).wait()
        for cp in ecopies:
            cp.wait()

    any_spec = pl.BlockSpec(memory_space=pl.ANY)
    out = pl.pallas_call(
        kernel,
        in_specs=[any_spec] * 6,
        out_specs=any_spec,
        out_shape=jax.ShapeDtypeStruct((S, C, B), x.dtype),
        scratch_shapes=[
            pltpu.VMEM((NP, NKT + 1, C // 2, 128), U32),
            pltpu.VMEM((CF, TB), BF16),
            pltpu.VMEM((RING + 2, C, TB), BF16),
            pltpu.VMEM((NU * MO, C, TB), BF16),
            pltpu.VMEM((C, 128), F32),
            pltpu.VMEM((C, 128), F32),
            pltpu.VMEM((NP, C, TB), F32),
            pltpu.VMEM((NP, C, TB), F32),
            pltpu.VMEM((NP, C, TB), F32),
            pltpu.VMEM((NP, C, TB), F32),
            pltpu.VMEM((NKT, C // 2, 128), U32),
            pltpu.VMEM((3, C // 2, 128), U32),
            pltpu.VMEM((C,), BF16), pltpu.VMEM((C,), BF16),
            pltpu.VMEM((C,), BF16), pltpu.VMEM((C,), BF16),
            pltpu.VMEM((3, C + 24, C), BF16),
            pltpu.SemaphoreType.DMA((NSEM,)),
        ],
        compiler_params=pltpu.CompilerParams(vmem_limit_bytes=100 * 1024 * 1024,
                                             disable_bounds_checks=True),
    )(jnp.transpose(x, (1, 2, 0)), w, mean, var, g, b)
    return jnp.transpose(out, (2, 0, 1))
```

```python
import jax
import jax.numpy as jnp
import jax.experimental.pallas as pl
import jax.experimental.pallas.tpu as pltpu

F32 = jnp.float32
BF16 = jnp.bfloat16
U32 = jnp.uint32

TB = 128
MO = 6
NP = MO + 2
UPB = 4
LAG = 2
NPRO = 3
RC = 16
CH = 8
RT = 4
LEAD = 3
NEP = 4
JS = 4
ORDER, GROUPS = (0, 7, 1, 2, 3, 4, 5, 6), (0, 1, 2, 3, 4)
ORDER_END, GROUPS_END = (0, 1, 2, 3, 4, 5, 6, 7), (0, 1, 2, 2, 2)
ORDER_PRO, ORDER_HALF, GROUPS_PRO = (0, 7, 5, 6, 3, 4, 1, 2), (1, 0, 7, 3, 4, 5, 6), (0, 1, 2, 3, 3)
EPS = 1e-5
CPK = {0: -2.25, 3: -0.025, 4: 0.075, 5: 0.8, 6: 2.4, 7: 2.25}


@jax.jit
def pallas_standalone__batchnorm__sampling_kernel(
    x: jax.Array,
    w: jax.Array,
    mean: jax.Array,
    var: jax.Array,
    g: jax.Array,
    b: jax.Array,
):
    B, S, C = x.shape
    NKT = C // 128
    CF = NKT * 128
    CR = C - CF
    SP = S + 1
    NB = B // TB
    NU = NB * SP // MO
    RING = RT * SP
    UPR = RING // MO
    CPT = S // CH
    NCH = NB * CPT
    NSC = RT * CPT
    U1 = NPRO + 1
    NBODY = (NU - U1 - 4) // UPB
    U2 = U1 + NBODY * UPB
    STEP = MO * UPB
    NSP = MO * NPRO + 1
    CSP = -(-NSP // CH)
    assert w.shape == (3, C, C) and 2 * CR == 128 and CPT == 4 and CH == 8
    assert NB * TB == B and NU * MO == NB * SP and UPR * MO == RING and U2 + 4 == NU and U1 % 4 == 0

    chunk_of = lambda p: CPT * (p // SP) + min((p % SP) // CH, CPT - 1)
    pn = lambda e: MO * e + MO - 1
    po = lambda e: MO * (e - LAG)
    xneed = lambda e: min(chunk_of(pn(e)) + 1, NCH)
    odone = lambda e: CPT * (po(e) // SP) + (po(e) % SP) // CH
    ends = [U1] + [U1 + UPB * (i + 1) for i in range(NBODY)] + [U2 + 2, NU]
    MAXC = 3
    assert xneed(U1) + LEAD <= NSC and xneed(U2 + 2) == NCH
    for e0, e1 in zip(ends[:-2], ends[1:-1]):
        assert max(xneed(e1) - xneed(e0), odone(e1) - odone(e0)) <= MAXC <= LEAD
        old = min(xneed(e1) + LEAD, NCH) - 1 - NSC
        assert old < 0 or SP * (old // CPT) + CH * (old % CPT) + CH - 1 < MO * e0 - 1

    XS0, OS0, WS0 = 0, NSC, NSC + NCH
    PS0 = WS0 + NKT + 1
    KS0 = PS0 + 4
    ES0 = KS0 + NKT + 3
    NSEM = ES0 + 3 + NEP

    def kernel(x_hbm, w_hbm, mean_hbm, var_hbm, g_hbm, b_hbm, o_hbm,
               a_ref, u0_ref, xbuf, obuf, sh_ref, hs_ref, ma_ref, mb_ref, mc_ref, md_ref,
               w1_ref, wl_ref, p0, p1, p2, p3, wbuf, sems):

        def hbm_chunk(ref, c):
            lane0 = (c >> 2) * TB
            if not isinstance(c, int):
                lane0 = pl.multiple_of(lane0, TB)
            return ref.at[pl.ds((c & 3) * CH, CH), :, pl.ds(lane0, TB)]

        def ring_slot(c):
            return ((c >> 2) & (RT - 1)) * SP + (c & 3) * CH

        def xcopy(c):
            return pltpu.make_async_copy(hbm_chunk(x_hbm, c), xbuf.at[pl.ds(ring_slot(c) + 1, CH)],
                                         sems.at[XS0 + (c & (NSC - 1))])

        def ocopy(c):
            return pltpu.make_async_copy(obuf.at[pl.ds((c >> 2) * SP + (c & 3) * CH, CH)], hbm_chunk(o_hbm, c),
                                         sems.at[OS0 + c])

        def krows(kt):
            if isinstance(kt, int):
                return pl.ds(kt * 128, 128 if kt < NKT else CR)
            return pl.ds(pl.multiple_of(kt * 128, 128), 128)

        def wcopy(kt):
            return pltpu.make_async_copy(w_hbm.at[:, krows(kt), :], wbuf.at[:, krows(kt), :],
                                         sems.at[WS0 + kt])

        def kcopy(kt, lo=0, hi=NSP, sem=None):
            return pltpu.make_async_copy(x_hbm.at[pl.ds(lo, hi - lo), krows(kt), pl.ds(0, TB)],
                                         xbuf.at[pl.ds(1 + lo, hi - lo), krows(kt), :],
                                         sems.at[KS0 + kt if sem is None else sem])

        k0a_copy = kcopy(0, 0, MO + 1)
        k0b_copy = kcopy(0, MO + 1, NSP, KS0 + NKT + 1)
        rcopy = pltpu.make_async_copy(x_hbm.at[pl.ds(NSP, CSP * CH - NSP), :, pl.ds(0, TB)],
                                      xbuf.at[pl.ds(1 + NSP, CSP * CH - NSP)], sems.at[KS0 + NKT + 2])
        pcopies = [pltpu.make_async_copy(s, d, sems.at[PS0 + i])
                   for i, (s, d) in enumerate(zip((mean_hbm, var_hbm, g_hbm, b_hbm), (p0, p1, p2, p3)))]
        for c in pcopies:
            c.start()
        wcopy(0).start()
        k0a_copy.start()
        wcopy(1).start()
        k0b_copy.start()
        kcopy(1).start()
        for kt in range(2, NKT + 1):
            wcopy(kt).start()
            kcopy(kt).start()
        rcopy.start()
        for c in range(CSP, xneed(U1) + LEAD):
            xcopy(c).start()

        for s in [SP * q for q in range(RT + 1)] + [RING + 1]:
            xbuf[s] = jnp.zeros((C, TB), BF16)

        for c in pcopies:
            c.wait()
        mean_, var_, g_, b_ = [r[...].astype(F32).reshape(1, C) for r in (p0, p1, p2, p3)]
        scale = g_ * jax.lax.rsqrt(var_ + EPS)
        hs_ref[...] = jnp.broadcast_to(0.5 * scale, (128, C)).T
        sh = 0.5 * (b_ - mean_ * scale)
        sh_hi = sh.astype(BF16).astype(F32)
        sh_mid = (sh - sh_hi).astype(BF16).astype(F32)
        sh_lo = (sh - sh_hi) - sh_mid
        row = jax.lax.broadcasted_iota(jnp.int32, (128, C), 0)
        sh_ref[...] = jnp.where(row == CR, sh_hi, jnp.where(
            row == CR + 1, sh_mid, jnp.where(row == CR + 2, sh_lo, 0.0))).T

        def tchunk(ld_, with_u0, grp):
            ld = lambda i, gi: ld_(i, grp[gi])
            d1, d2, d3, d4, d5, d6 = [ld(i, 1) for i in range(1, 7)]
            e1, o1 = (d2 + d6) - 4.25 * d4, (d1 + d5) - 4.25 * d3
            d1, d2, d3, d4, d5, d6 = [ld(i, 2) for i in range(1, 7)]
            e2, o2 = (d6 - d4) - 0.25 * (d4 - d2), 2.0 * (d5 - d3) - 0.5 * (d3 - d1)
            d1, d2, d3, d4, d5, d6 = [ld(i, 3) for i in range(1, 7)]
            e3, o3 = (d6 - d4) - 4.0 * (d4 - d2), 0.5 * (d5 - d3) - 2.0 * (d3 - d1)
            d1, d3, d5, d7 = [ld(i, 4) for i in (1, 3, 5, 7)]
            u = [None, e1 + o1, e1 - o1, e2 + o2, e2 - o2, e3 + o3, e3 - o3, (d7 - d1) - 5.25 * (d5 - d3)]
            if with_u0:
                d0, d2, d4, d6 = [ld(i, 0) for i in (0, 2, 4, 6)]
                u[0] = (d0 - d6) + 5.25 * (d4 - d2)
            return u

        def ones_rows():
            return (jax.lax.broadcasted_iota(jnp.int32, (CR, TB), 0) < 3).astype(F32)

        def carry_u0(t):
            base = (t % UPR) * MO
            slabs = [base + i for i in (0, 2, 4, 6)]
            for r in range(0, CF, RC):
                d0, d2, d4, d6 = [xbuf[s, r:r + RC, :].astype(F32) for s in slabs]
                u0_ref[r:r + RC, :] = ((d0 - d6) + 5.25 * (d4 - d2)).astype(BF16)

        def transform(t, carried, z, grp, order):
            zs = [0] + [jnp.minimum(z + q, 0) for q in range(1, 5)]
            never = z < 0
            base = (t % UPR) * MO
            gof = [grp[q] for q in (0, 1, 1, 2, 2, 3, 3, 4)]
            slab = dict(((i, gi), base + zs[gi] + i) for gi in set(grp) for i in range(NP))
            cs = []
            for r in range(0, C, RC):
                c = tchunk(lambda i, gi: xbuf[slab[i, gi], r:r + RC, :].astype(F32),
                           not (carried and r < CF), grp)
                members = {}
                for j in order:
                    if c[j] is not None:
                        members.setdefault(gof[j], []).append(j)
                for j in set(j for mem in members.values() for j in mem[1:]) | {2}:
                    c[j] = pltpu.bitcast(c[j].astype(BF16), U32)
                for mem in members.values():
                    if len(mem) > 1 and mem[0] != 2:
                        dep = c[mem[1]]
                        for j in mem[2:]:
                            dep = dep ^ c[j]
                        top = jax.lax.select(never, jax.lax.bitcast_convert_type(dep, F32), c[mem[0]][0:RC // 2])
                        c[mem[0]] = jnp.concatenate([top, c[mem[0]][RC // 2:]], axis=0)
                cs.append(c)
            tail = pltpu.bitcast(jnp.concatenate([c[2] for c in cs[CF // RC:]], axis=0), BF16)
            us = {}
            for j in order:
                parts = [c[j] for c in cs if c[j] is not None]
                if j == 2:
                    parts = parts[:CF // RC]
                if j == 1:
                    parts = parts + [ones_rows()]
                v = jnp.concatenate(parts, axis=0)
                v = v.astype(BF16) if v.dtype == F32 else pltpu.bitcast(v, BF16)
                if j not in (1, 2):
                    v = jnp.concatenate([v, tail], axis=0)
                if j == 0 and carried:
                    v = jnp.concatenate([u0_ref[...], v], axis=0)
                us[j] = v
            return us

        def unit(t, carried, ms, i, grp, order):
            us = transform(t, carried, i, grp, order)
            z = jnp.minimum(i, 0)
            for j in order:
                nk = NKT if j == 2 else NKT + 1
                lhs = pltpu.bitcast(jnp.concatenate([a_ref[j, kt] for kt in range(nk)], axis=1), BF16)
                ms[j][j + z, 0:C, :] = jnp.dot(lhs, us[j], preferred_element_type=F32)

        def output(t, ms, rlo=0, rhi=C, nout=MO):
            base = (t % UPR) * MO + (t // UPR) * RING
            slabs = [base + i for i in range(nout)]
            for r in range(rlo, rhi, RC):
                m = [ms[j][j, r:r + RC, :] if (j < NP - 1 or nout == MO) else 0.0 for j in range(NP)]
                s1, s2, s3 = m[1] + m[2], m[3] + m[4], m[5] + m[6]
                d1, d2, d3 = m[1] - m[2], m[3] - m[4], m[5] - m[6]
                hs = hs_ref[r:r + RC, :]
                ys = [(hs * m[0] + s1) + (s2 + s3),
                      (d1 + 2.0 * d2) + 0.5 * d3,
                      (s1 + 4.0 * s2) + 0.25 * s3,
                      (d1 + 8.0 * d2) + 0.125 * d3,
                      (s1 + 16.0 * s2) + 0.0625 * s3,
                      (d1 + 32.0 * d2) + (0.03125 * d3 + hs * m[7])]
                for i in range(nout):
                    h = ys[i]
                    obuf[slabs[i], r:r + RC, :] = (h * jnp.tanh(h) + h).astype(BF16)

        mbuf = [[r] * NP for r in (ma_ref, mb_ref, mc_ref, md_ref)]

        def once(z, fn):
            def trip(i, c):
                fn(i)
                return c
            jax.lax.fori_loop(0, z + 1, trip, 0)

        def xpose(kt):
            last = isinstance(kt, int) and kt == NKT
            for r in range(0, C, 128):
                cols = slice(r, min(r + 128, C))
                rows = slice(r // 2, min(r + 128, C) // 2)
                for k, dst in enumerate((a_ref.at[0], w1_ref, a_ref.at[NP - 1])):
                    if last:
                        t = jnp.concatenate([wbuf[k, CF:C, cols]] * 2, axis=0).T
                        wl_ref[k, rows, :] = pltpu.bitcast(t, U32)
                    else:
                        dst[kt, rows, :] = pltpu.bitcast(wbuf[k, krows(kt), cols].T, U32)

        def combos(kt, zs, never):
            last = isinstance(kt, int) and kt == NKT
            lo = jax.lax.broadcasted_iota(jnp.int32, (RC, 128), 1) < CR
            pack = lambda v: pltpu.bitcast(v.astype(BF16), U32)
            out = dict((j, []) for j in range(NP))
            idx = [[z + 1, z + 2] if last else [z + kt, z + NP - 1] for z in zs[:4]]
            for r in range(0, C, RC):
                rows = slice(r // 2, (r + RC) // 2)
                def taps(gi):
                    if last:
                        raw = [wl_ref[k, rows, :] for k in [zs[gi]] + idx[gi]]
                    else:
                        raw = [a_ref[zs[gi], kt, rows, :], w1_ref[idx[gi][0], rows, :], a_ref[idx[gi][1], kt, rows, :]]
                    return [pltpu.bitcast(t, BF16).astype(F32) for t in raw]
                hs = hs_ref[r:r + RC, :]
                for gi, (ce0, ce2, co) in enumerate(((-2.0 / 9, -2.0 / 9, -2.0 / 9), (1.0 / 90, 2.0 / 45, 1.0 / 45),
                                                     (32.0 / 45, 8.0 / 45, 16.0 / 45))):
                    w0, w1, w2 = [t * hs for t in taps(gi)]
                    e = ce0 * (w0 + w2) if gi == 0 else ce0 * w0 + ce2 * w2
                    o = co * w1
                    ja, jb = 2 * gi + 1, 2 * gi + 2
                    ga, gb = e + o, e - o
                    if last:
                        if gi == 0:
                            out[1].append(pack(jnp.where(lo, ga, sh_ref[r:r + RC, :])))
                            continue
                        g2 = (w0 + w2) - w1
                        ga = jnp.where(lo, ga, (-2.0 / 9 * CPK[ja]) * g2)
                        gb = jnp.where(lo, gb, (-2.0 / 9 * CPK[jb]) * g2)
                    pb = pack(gb)
                    out[ja].append(jax.lax.select(never, pb, pack(ga)))
                    out[jb].append(pb)
                if last:
                    r0, r1, r2 = taps(3)
                    raw2 = (r0 + r2) - r1
                    p7 = pack(jnp.where(lo, r2, (-2.0 / 9 * CPK[7]) * raw2))
                    out[0].append(jax.lax.select(never, p7, pack(jnp.where(lo, r0, (-2.0 / 9 * CPK[0]) * raw2))))
                    out[7].append(p7)
            res = {}
            for j in range(NP):
                if out[j]:
                    res[j] = jnp.concatenate(out[j], axis=0)
                    a_ref[j, kt] = res[j]
                elif not last:
                    res[j] = a_ref[j, kt]
            return res

        def mm(kt, i, order, units=(0, 1, 2), fresh=True):
            last = isinstance(kt, int) and kt == NKT
            r0 = kt * 128 if isinstance(kt, int) else pl.multiple_of(kt * 128, 128)
            zs = [jnp.minimum(i + q, 0) for q in range(5)]
            lhs = combos(kt, zs, i < 0) if fresh else dict((j, a_ref[j, kt]) for j in range(NP))
            rhs = []
            rows = [pl.ds(r0 + r, RC) for r in range(0, CR if last else 128, RC)]
            for u in units:
                slab = dict(((s, gi), MO * u + s + zs[gi]) for gi in set(GROUPS_PRO) for s in range(NP))
                cs = [tchunk(lambda s, gi: xbuf[slab[s, gi], rw, :].astype(F32), True, GROUPS_PRO) for rw in rows]
                fin = lambda j: jnp.concatenate([c[j] for c in cs], axis=0).astype(BF16)
                rhs.append(dict(
                    (j, jnp.concatenate([fin(j), ones_rows().astype(BF16) if j == 1 else fin(2)], axis=0)
                     if last else fin(j)) for j in lhs))

            def products():
                for j in order:
                    for u, rh in zip(units, rhs):
                        m_ref = mbuf[u][j]
                        p = jnp.dot(pltpu.bitcast(lhs[j], BF16), rh[j], preferred_element_type=F32)
                        m_ref[j] = p if isinstance(kt, int) and kt == 0 else m_ref[j] + p
            return products

        def kblock(kt, i):
            kcopy(kt).wait()
            wcopy(kt + 1).wait()
            xpose(kt + 1)
            mm(kt, i, ORDER_PRO)()
            return 0

        wcopy(0).wait()
        xpose(0)
        z = jax.lax.fori_loop(0, 2, lambda i, c: jnp.minimum(i, c), jnp.int32(0))
        k0a_copy.wait()
        once(z, lambda i: mm(0, i, ORDER_PRO, (0,))())
        wcopy(1).wait()
        k0b_copy.wait()
        once(z, lambda i: (xpose(1), mm(0, i, ORDER_PRO, (1, 2), False)()))
        jax.lax.fori_loop(1, NKT - 1, lambda i, c: kblock(i, i), 0)
        wcopy(NKT).wait()
        kcopy(NKT - 1).wait()
        kcopy(NKT).wait()

        def klast(i):
            xpose(NKT)
            for products in [mm(NKT - 1, i, ORDER), mm(NKT, i, ORDER_HALF)]:
                products()

        once(z, klast)
        rcopy.wait()
        for c in range(CSP, xneed(U1)):
            xcopy(c).wait()
        carry_u0(NPRO)

        def units(t0, n, i):
            for k in range(n):
                unit(t0 + k, k == 0, mbuf[k], i, GROUPS, ORDER)
                output(t0 + k - LAG, mbuf[(k - LAG) % 4])
            carry_u0(t0 + n)

        def copies(o0, o1, n0, n1):
            for k in range(MAXC):
                pl.when(o0 + k < o1)(lambda: ocopy(o0 + k).start())
            for k in range(MAXC):
                pl.when(jnp.logical_and(n0 + k < n1, n0 + k + LEAD < NCH))(lambda: xcopy(n0 + k + LEAD).start())
            for k in range(MAXC):
                pl.when(n0 + k < n1)(lambda: xcopy(n0 + k).wait())

        def first1(i):
            output(z, mbuf[0])
            output(z + 1, mbuf[1])
            unit(NPRO + z, True, mbuf[NPRO], i, GROUPS, ORDER)
            carry_u0(U1 + z)
            copies(z, z + odone(U1), z + xneed(U1), z + xneed(U1 + UPB))

        once(z, first1)

        def advance(q, r):
            wrap = r + STEP >= SP
            return q + wrap.astype(jnp.int32), jnp.where(wrap, r + STEP - SP, r + STEP)

        def body(i, carry):
            o0, o1, n0, n1, qo, ro, qn, rn = carry
            units(U1 + UPB * i, UPB, i)
            copies(o0, o1, n0, n1)
            o2 = CPT * qo + (ro >> 3)
            n2 = jnp.minimum(CPT * qn + jnp.minimum(rn >> 3, CPT - 1) + 1, NCH)
            return (o1, o2, n1, n2) + advance(qo, ro) + advance(qn, rn)

        e1, e2, e3 = U1 + UPB, U1 + 2 * UPB, U1 + 3 * UPB
        init = (odone(U1), odone(e1), xneed(e1), xneed(e2), po(e2) // SP, po(e2) % SP, pn(e3) // SP, pn(e3) % SP)
        fin = jax.lax.fori_loop(0, NBODY, body, tuple(jnp.int32(v) for v in init))
        assert xneed(U2 + UPB) == NCH

        z = jnp.minimum(fin[0], 0)
        tile0 = (NB - 1) * SP
        lanes = pl.ds((NB - 1) * TB, TB)
        ecopies = []

        def ecopy(s_lo, s_hi, rlo=0, rhi=C):
            cp = pltpu.make_async_copy(
                obuf.at[pl.ds(tile0 + s_lo, s_hi - s_lo), pl.ds(rlo, rhi - rlo), :],
                o_hbm.at[pl.ds(s_lo, s_hi - s_lo), pl.ds(rlo, rhi - rlo), lanes],
                sems.at[ES0 + len(ecopies)])
            ecopies.append(cp)
            return cp

        ta, tb = NU - 2, NU - 1
        s_a, s_c, s_d = MO * U2 - tile0, MO * ta - tile0, MO * tb - tile0
        sent0, sent = odone(U2), (NB - 1) * CPT
        assert sent0 <= sent <= sent0 + MAXC and 0 < s_a and S - s_d == MO - 1
        ea, eb, ec = ecopy(0, s_a), ecopy(s_a, s_c), ecopy(s_c, s_d)

        def last2(i):
            units(U2 + z, 2, i)
            pl.when(i >= 0)(ea.start)
            copies(z + sent0, z + sent, z + NCH, z + NCH)
            pl.when(i >= 0)(ocopy(z).wait)

        mta = [mc_ref if j < JS else ma_ref for j in range(NP)]
        mtb = [md_ref if j < JS else mc_ref for j in range(NP)]

        def last_a(i):
            output(U2 + z, mbuf[0])
            output(U2 + 1 + z, mbuf[1])
            unit(ta + z, True, mta, i, GROUPS_END, ORDER_END)
            carry_u0(tb + z)
            pl.when(i >= 0)(eb.start)

        def last_b(i):
            output(ta + z, mta)
            unit(tb + z, True, mtb, i, GROUPS_END, ORDER_END[:-1])
            pl.when(i >= 0)(ec.start)

        once(z, last2)
        once(z, last_a)
        once(z, last_b)
        RP = C // NEP
        for e in range(NEP):
            output(tb, mtb, e * RP, (e + 1) * RP, MO - 1)
            ecopy(s_d, S, e * RP, (e + 1) * RP).start()
        for c in range(1, sent):
            ocopy(c).wait()
        for cp in ecopies:
            cp.wait()

    any_spec = pl.BlockSpec(memory_space=pl.ANY)
    out = pl.pallas_call(
        kernel,
        in_specs=[any_spec] * 6,
        out_specs=any_spec,
        out_shape=jax.ShapeDtypeStruct((S, C, B), x.dtype),
        scratch_shapes=[
            pltpu.VMEM((NP, NKT + 1, C // 2, 128), U32),
            pltpu.VMEM((CF, TB), BF16),
            pltpu.VMEM((RING + 2, C, TB), BF16),
            pltpu.VMEM((NU * MO, C, TB), BF16),
            pltpu.VMEM((C, 128), F32),
            pltpu.VMEM((C, 128), F32),
            pltpu.VMEM((NP, C, TB), F32),
            pltpu.VMEM((NP, C, TB), F32),
            pltpu.VMEM((NP, C, TB), F32),
            pltpu.VMEM((NP, C, TB), F32),
            pltpu.VMEM((NKT, C // 2, 128), U32),
            pltpu.VMEM((3, C // 2, 128), U32),
            pltpu.VMEM((C,), BF16), pltpu.VMEM((C,), BF16),
            pltpu.VMEM((C,), BF16), pltpu.VMEM((C,), BF16),
            pltpu.VMEM((3, C + 24, C), BF16),
            pltpu.SemaphoreType.DMA((NSEM,)),
        ],
        compiler_params=pltpu.CompilerParams(vmem_limit_bytes=100 * 1024 * 1024,
                                             disable_bounds_checks=True),
    )(jnp.transpose(x, (1, 2, 0)), w, mean, var, g, b)
    return jnp.transpose(out, (2, 0, 1))
```

```python
import jax
import jax.numpy as jnp
import jax.experimental.pallas as pl
import jax.experimental.pallas.tpu as pltpu

F32 = jnp.float32
BF16 = jnp.bfloat16
U32 = jnp.uint32

TB = 128
MO = 6
NP = MO + 2
UPB = 4
LAG = 2
NPRO = 3
RC = 16
CH = 8
RT = 4
LEAD = 3
PIECES = (0, 32, 96, 208, 368, 576)
JS = 4
ORDER, GROUPS = (0, 7, 1, 2, 3, 4, 5, 6), (0, 1, 2, 3, 4)
ORDER_END, GROUPS_END = (0, 1, 2, 3, 4, 5, 6, 7), (0, 1, 2, 2, 2)
ORDER_PRO, ORDER_HALF, GROUPS_PRO = (0, 7, 5, 6, 3, 4, 1, 2), (1, 0, 7, 3, 4, 5, 6), (0, 1, 2, 3, 3)
EPS = 1e-5
CPK = {0: -2.25, 3: -0.025, 4: 0.075, 5: 0.8, 6: 2.4, 7: 2.25}


@jax.jit
def pallas_standalone__batchnorm__sampling_kernel(
    x: jax.Array,
    w: jax.Array,
    mean: jax.Array,
    var: jax.Array,
    g: jax.Array,
    b: jax.Array,
):
    B, S, C = x.shape
    NKT = C // 128
    CF = NKT * 128
    CR = C - CF
    SP = S + 1
    NB = B // TB
    NU = NB * SP // MO
    RING = RT * SP
    UPR = RING // MO
    CPT = S // CH
    NCH = NB * CPT
    NSC = RT * CPT
    U1 = NPRO + 1
    NBODY = (NU - U1 - 4) // UPB
    U2 = U1 + NBODY * UPB
    STEP = MO * UPB
    NSP = MO * NPRO + 1
    CSP = -(-NSP // CH)
    assert w.shape == (3, C, C) and 2 * CR == 128 and CPT == 4 and CH == 8 and PIECES[-1] == C
    assert NB * TB == B and NU * MO == NB * SP and UPR * MO == RING and U2 + 4 == NU and U1 % 4 == 0

    chunk_of = lambda p: CPT * (p // SP) + min((p % SP) // CH, CPT - 1)
    pn = lambda e: MO * e + MO - 1
    po = lambda e: MO * (e - LAG)
    xneed = lambda e: min(chunk_of(pn(e)) + 1, NCH)
    odone = lambda e: CPT * (po(e) // SP) + (po(e) % SP) // CH
    ends = [U1] + [U1 + UPB * (i + 1) for i in range(NBODY)] + [U2 + 2, NU]
    MAXC = 3
    assert xneed(U1) + LEAD <= NSC and xneed(U2 + 2) == NCH
    for e0, e1 in zip(ends[:-2], ends[1:-1]):
        assert max(xneed(e1) - xneed(e0), odone(e1) - odone(e0)) <= MAXC <= LEAD
        old = min(xneed(e1) + LEAD, NCH) - 1 - NSC
        assert old < 0 or SP * (old // CPT) + CH * (old % CPT) + CH - 1 < MO * e0 - 1

    XS0, OS0, WS0 = 0, NSC, NSC + NCH
    PS0 = WS0 + NKT + 1
    KS0 = PS0 + 4
    ES0 = KS0 + NKT + 3
    NSEM = ES0 + 2 + len(PIECES)

    def kernel(x_hbm, w_hbm, mean_hbm, var_hbm, g_hbm, b_hbm, o_hbm,
               a_ref, u0_ref, xbuf, obuf, sh_ref, hs_ref, ma_ref, mb_ref, mc_ref, md_ref,
               w1_ref, wl_ref, p0, p1, p2, p3, wbuf, sems):

        def hbm_chunk(ref, c):
            lane0 = (c >> 2) * TB
            if not isinstance(c, int):
                lane0 = pl.multiple_of(lane0, TB)
            return ref.at[pl.ds((c & 3) * CH, CH), :, pl.ds(lane0, TB)]

        def ring_slot(c):
            return ((c >> 2) & (RT - 1)) * SP + (c & 3) * CH

        def xcopy(c):
            return pltpu.make_async_copy(hbm_chunk(x_hbm, c), xbuf.at[pl.ds(ring_slot(c) + 1, CH)],
                                         sems.at[XS0 + (c & (NSC - 1))])

        def ocopy(c):
            return pltpu.make_async_copy(obuf.at[pl.ds((c >> 2) * SP + (c & 3) * CH, CH)], hbm_chunk(o_hbm, c),
                                         sems.at[OS0 + c])

        def krows(kt):
            if isinstance(kt, int):
                return pl.ds(kt * 128, 128 if kt < NKT else CR)
            return pl.ds(pl.multiple_of(kt * 128, 128), 128)

        def wcopy(kt):
            return pltpu.make_async_copy(w_hbm.at[:, krows(kt), :], wbuf.at[:, krows(kt), :],
                                         sems.at[WS0 + kt])

        def kcopy(kt, lo=0, hi=NSP, sem=None):
            return pltpu.make_async_copy(x_hbm.at[pl.ds(lo, hi - lo), krows(kt), pl.ds(0, TB)],
                                         xbuf.at[pl.ds(1 + lo, hi - lo), krows(kt), :],
                                         sems.at[KS0 + kt if sem is None else sem])

        k0a_copy = kcopy(0, 0, MO + 1)
        k0b_copy = kcopy(0, MO + 1, NSP, KS0 + NKT + 1)
        rcopy = pltpu.make_async_copy(x_hbm.at[pl.ds(NSP, CSP * CH - NSP), :, pl.ds(0, TB)],
                                      xbuf.at[pl.ds(1 + NSP, CSP * CH - NSP)], sems.at[KS0 + NKT + 2])
        pcopies = [pltpu.make_async_copy(s, d, sems.at[PS0 + i])
                   for i, (s, d) in enumerate(zip((mean_hbm, var_hbm, g_hbm, b_hbm), (p0, p1, p2, p3)))]
        for c in pcopies:
            c.start()
        wcopy(0).start()
        k0a_copy.start()
        wcopy(1).start()
        k0b_copy.start()
        kcopy(1).start()
        for kt in range(2, NKT + 1):
            wcopy(kt).start()
            kcopy(kt).start()
        rcopy.start()
        for c in range(CSP, xneed(U1) + LEAD):
            xcopy(c).start()

        for s in [SP * q for q in range(RT + 1)] + [RING + 1]:
            xbuf[s] = jnp.zeros((C, TB), BF16)

        for c in pcopies:
            c.wait()
        mean_, var_, g_, b_ = [r[...].astype(F32).reshape(1, C) for r in (p0, p1, p2, p3)]
        scale = g_ * jax.lax.rsqrt(var_ + EPS)
        hs_ref[...] = jnp.broadcast_to(0.5 * scale, (128, C)).T
        sh = 0.5 * (b_ - mean_ * scale)
        sh_hi = sh.astype(BF16).astype(F32)
        sh_mid = (sh - sh_hi).astype(BF16).astype(F32)
        sh_lo = (sh - sh_hi) - sh_mid
        row = jax.lax.broadcasted_iota(jnp.int32, (128, C), 0)
        sh_ref[...] = jnp.where(row == CR, sh_hi, jnp.where(
            row == CR + 1, sh_mid, jnp.where(row == CR + 2, sh_lo, 0.0))).T

        def tchunk(ld_, with_u0, grp):
            ld = lambda i, gi: ld_(i, grp[gi])
            d1, d2, d3, d4, d5, d6 = [ld(i, 1) for i in range(1, 7)]
            e1, o1 = (d2 + d6) - 4.25 * d4, (d1 + d5) - 4.25 * d3
            d1, d2, d3, d4, d5, d6 = [ld(i, 2) for i in range(1, 7)]
            e2, o2 = (d6 - d4) - 0.25 * (d4 - d2), 2.0 * (d5 - d3) - 0.5 * (d3 - d1)
            d1, d2, d3, d4, d5, d6 = [ld(i, 3) for i in range(1, 7)]
            e3, o3 = (d6 - d4) - 4.0 * (d4 - d2), 0.5 * (d5 - d3) - 2.0 * (d3 - d1)
            d1, d3, d5, d7 = [ld(i, 4) for i in (1, 3, 5, 7)]
            u = [None, e1 + o1, e1 - o1, e2 + o2, e2 - o2, e3 + o3, e3 - o3, (d7 - d1) - 5.25 * (d5 - d3)]
            if with_u0:
                d0, d2, d4, d6 = [ld(i, 0) for i in (0, 2, 4, 6)]
                u[0] = (d0 - d6) + 5.25 * (d4 - d2)
            return u

        def ones_rows():
            return (jax.lax.broadcasted_iota(jnp.int32, (CR, TB), 0) < 3).astype(F32)

        def carry_u0(t):
            base = (t % UPR) * MO
            slabs = [base + i for i in (0, 2, 4, 6)]
            for r in range(0, CF, RC):
                d0, d2, d4, d6 = [xbuf[s, r:r + RC, :].astype(F32) for s in slabs]
                u0_ref[r:r + RC, :] = ((d0 - d6) + 5.25 * (d4 - d2)).astype(BF16)

        def transform(t, carried, z, grp, order):
            zs = [0] + [jnp.minimum(z + q, 0) for q in range(1, 5)]
            never = z < 0
            base = (t % UPR) * MO
            gof = [grp[q] for q in (0, 1, 1, 2, 2, 3, 3, 4)]
            slab = dict(((i, gi), base + zs[gi] + i) for gi in set(grp) for i in range(NP))
            cs = []
            for r in range(0, C, RC):
                c = tchunk(lambda i, gi: xbuf[slab[i, gi], r:r + RC, :].astype(F32),
                           not (carried and r < CF), grp)
                members = {}
                for j in order:
                    if c[j] is not None:
                        members.setdefault(gof[j], []).append(j)
                for j in set(j for mem in members.values() for j in mem[1:]) | {2}:
                    c[j] = pltpu.bitcast(c[j].astype(BF16), U32)
                for mem in members.values():
                    if len(mem) > 1 and mem[0] != 2:
                        dep = c[mem[1]]
                        for j in mem[2:]:
                            dep = dep ^ c[j]
                        top = jax.lax.select(never, jax.lax.bitcast_convert_type(dep, F32), c[mem[0]][0:RC // 2])
                        c[mem[0]] = jnp.concatenate([top, c[mem[0]][RC // 2:]], axis=0)
                cs.append(c)
            tail = pltpu.bitcast(jnp.concatenate([c[2] for c in cs[CF // RC:]], axis=0), BF16)
            us = {}
            for j in order:
                parts = [c[j] for c in cs if c[j] is not None]
                if j == 2:
                    parts = parts[:CF // RC]
                if j == 1:
                    parts = parts + [ones_rows()]
                v = jnp.concatenate(parts, axis=0)
                v = v.astype(BF16) if v.dtype == F32 else pltpu.bitcast(v, BF16)
                if j not in (1, 2):
                    v = jnp.concatenate([v, tail], axis=0)
                if j == 0 and carried:
                    v = jnp.concatenate([u0_ref[...], v], axis=0)
                us[j] = v
            return us

        def unit(t, carried, ms, i, grp, order):
            us = transform(t, carried, i, grp, order)
            z = jnp.minimum(i, 0)
            for j in order:
                nk = NKT if j == 2 else NKT + 1
                lhs = pltpu.bitcast(jnp.concatenate([a_ref[j, kt] for kt in range(nk)], axis=1), BF16)
                ms[j][j + z, 0:C, :] = jnp.dot(lhs, us[j], preferred_element_type=F32)

        def output(t, ms, rlo=0, rhi=C, nout=MO):
            base = (t % UPR) * MO + (t // UPR) * RING
            slabs = [base + i for i in range(nout)]
            for r in range(rlo, rhi, RC):
                m = [ms[j][j, r:r + RC, :] if (j < NP - 1 or nout == MO) else 0.0 for j in range(NP)]
                s1, s2, s3 = m[1] + m[2], m[3] + m[4], m[5] + m[6]
                d1, d2, d3 = m[1] - m[2], m[3] - m[4], m[5] - m[6]
                hs = hs_ref[r:r + RC, :]
                ys = [(hs * m[0] + s1) + (s2 + s3),
                      (d1 + 2.0 * d2) + 0.5 * d3,
                      (s1 + 4.0 * s2) + 0.25 * s3,
                      (d1 + 8.0 * d2) + 0.125 * d3,
                      (s1 + 16.0 * s2) + 0.0625 * s3,
                      (d1 + 32.0 * d2) + (0.03125 * d3 + hs * m[7])]
                for i in range(nout):
                    h = ys[i]
                    obuf[slabs[i], r:r + RC, :] = (h * jnp.tanh(h) + h).astype(BF16)

        mbuf = [[r] * NP for r in (ma_ref, mb_ref, mc_ref, md_ref)]

        def once(z, fn):
            def trip(i, c):
                fn(i)
                return c
            jax.lax.fori_loop(0, z + 1, trip, 0)

        def xpose(kt):
            last = isinstance(kt, int) and kt == NKT
            for r in range(0, C, 128):
                cols = slice(r, min(r + 128, C))
                rows = slice(r // 2, min(r + 128, C) // 2)
                for k, dst in enumerate((a_ref.at[0], w1_ref, a_ref.at[NP - 1])):
                    if last:
                        t = jnp.concatenate([wbuf[k, CF:C, cols]] * 2, axis=0).T
                        wl_ref[k, rows, :] = pltpu.bitcast(t, U32)
                    else:
                        dst[kt, rows, :] = pltpu.bitcast(wbuf[k, krows(kt), cols].T, U32)

        def combos(kt, zs, never):
            last = isinstance(kt, int) and kt == NKT
            lo = jax.lax.broadcasted_iota(jnp.int32, (RC, 128), 1) < CR
            pack = lambda v: pltpu.bitcast(v.astype(BF16), U32)
            out = dict((j, []) for j in range(NP))
            idx = [[z + 1, z + 2] if last else [z + kt, z + NP - 1] for z in zs[:4]]
            for r in range(0, C, RC):
                rows = slice(r // 2, (r + RC) // 2)
                def taps(gi):
                    if last:
                        raw = [wl_ref[k, rows, :] for k in [zs[gi]] + idx[gi]]
                    else:
                        raw = [a_ref[zs[gi], kt, rows, :], w1_ref[idx[gi][0], rows, :], a_ref[idx[gi][1], kt, rows, :]]
                    return [pltpu.bitcast(t, BF16).astype(F32) for t in raw]
                hs = hs_ref[r:r + RC, :]
                for gi, (ce0, ce2, co) in enumerate(((-2.0 / 9, -2.0 / 9, -2.0 / 9), (1.0 / 90, 2.0 / 45, 1.0 / 45),
                                                     (32.0 / 45, 8.0 / 45, 16.0 / 45))):
                    w0, w1, w2 = [t * hs for t in taps(gi)]
                    e = ce0 * (w0 + w2) if gi == 0 else ce0 * w0 + ce2 * w2
                    o = co * w1
                    ja, jb = 2 * gi + 1, 2 * gi + 2
                    ga, gb = e + o, e - o
                    if last:
                        if gi == 0:
                            out[1].append(pack(jnp.where(lo, ga, sh_ref[r:r + RC, :])))
                            continue
                        g2 = (w0 + w2) - w1
                        ga = jnp.where(lo, ga, (-2.0 / 9 * CPK[ja]) * g2)
                        gb = jnp.where(lo, gb, (-2.0 / 9 * CPK[jb]) * g2)
                    pb = pack(gb)
                    out[ja].append(jax.lax.select(never, pb, pack(ga)))
                    out[jb].append(pb)
                if last:
                    r0, r1, r2 = taps(3)
                    raw2 = (r0 + r2) - r1
                    p7 = pack(jnp.where(lo, r2, (-2.0 / 9 * CPK[7]) * raw2))
                    out[0].append(jax.lax.select(never, p7, pack(jnp.where(lo, r0, (-2.0 / 9 * CPK[0]) * raw2))))
                    out[7].append(p7)
            res = {}
            for j in range(NP):
                if out[j]:
                    res[j] = jnp.concatenate(out[j], axis=0)
                    a_ref[j, kt] = res[j]
                elif not last:
                    res[j] = a_ref[j, kt]
            return res

        def mm(kt, i, order, units=(0, 1, 2), fresh=True):
            last = isinstance(kt, int) and kt == NKT
            r0 = kt * 128 if isinstance(kt, int) else pl.multiple_of(kt * 128, 128)
            zs = [jnp.minimum(i + q, 0) for q in range(5)]
            lhs = combos(kt, zs, i < 0) if fresh else dict((j, a_ref[j, kt]) for j in range(NP))
            rhs = []
            rows = [pl.ds(r0 + r, RC) for r in range(0, CR if last else 128, RC)]
            for u in units:
                slab = dict(((s, gi), MO * u + s + zs[gi]) for gi in set(GROUPS_PRO) for s in range(NP))
                cs = [tchunk(lambda s, gi: xbuf[slab[s, gi], rw, :].astype(F32), True, GROUPS_PRO) for rw in rows]
                fin = lambda j: jnp.concatenate([c[j] for c in cs], axis=0).astype(BF16)
                rhs.append(dict(
                    (j, jnp.concatenate([fin(j), ones_rows().astype(BF16) if j == 1 else fin(2)], axis=0)
                     if last else fin(j)) for j in lhs))

            def products():
                for j in order:
                    for u, rh in zip(units, rhs):
                        m_ref = mbuf[u][j]
                        p = jnp.dot(pltpu.bitcast(lhs[j], BF16), rh[j], preferred_element_type=F32)
                        m_ref[j] = p if isinstance(kt, int) and kt == 0 else m_ref[j] + p
            return products

        def kblock(kt, i):
            kcopy(kt).wait()
            wcopy(kt + 1).wait()
            xpose(kt + 1)
            mm(kt, i, ORDER_PRO)()
            return 0

        wcopy(0).wait()
        xpose(0)
        z = jax.lax.fori_loop(0, 2, lambda i, c: jnp.minimum(i, c), jnp.int32(0))
        k0a_copy.wait()
        once(z, lambda i: mm(0, i, ORDER_PRO, (0,))())
        wcopy(1).wait()
        k0b_copy.wait()
        once(z, lambda i: (xpose(1), mm(0, i, ORDER_PRO, (1, 2), False)()))
        jax.lax.fori_loop(1, NKT - 1, lambda i, c: kblock(i, i), 0)
        wcopy(NKT).wait()
        kcopy(NKT - 1).wait()
        kcopy(NKT).wait()

        def klast(i):
            xpose(NKT)
            for products in [mm(NKT - 1, i, ORDER), mm(NKT, i, ORDER_HALF)]:
                products()

        once(z, klast)
        rcopy.wait()
        for c in range(CSP, xneed(U1)):
            xcopy(c).wait()
        carry_u0(NPRO)

        def units(t0, n, i):
            for k in range(n):
                unit(t0 + k, k == 0, mbuf[k], i, GROUPS, ORDER)
                output(t0 + k - LAG, mbuf[(k - LAG) % 4])
            carry_u0(t0 + n)

        def copies(o0, o1, n0, n1):
            for k in range(MAXC):
                pl.when(o0 + k < o1)(lambda: ocopy(o0 + k).start())
            for k in range(MAXC):
                pl.when(jnp.logical_and(n0 + k < n1, n0 + k + LEAD < NCH))(lambda: xcopy(n0 + k + LEAD).start())
            for k in range(MAXC):
                pl.when(n0 + k < n1)(lambda: xcopy(n0 + k).wait())

        def first1(i):
            output(z, mbuf[0])
            output(z + 1, mbuf[1])
            unit(NPRO + z, True, mbuf[NPRO], i, GROUPS, ORDER)
            carry_u0(U1 + z)
            copies(z, z + odone(U1), z + xneed(U1), z + xneed(U1 + UPB))

        once(z, first1)

        def advance(q, r):
            wrap = r + STEP >= SP
            return q + wrap.astype(jnp.int32), jnp.where(wrap, r + STEP - SP, r + STEP)

        def body(i, carry):
            o0, o1, n0, n1, qo, ro, qn, rn = carry
            units(U1 + UPB * i, UPB, i)
            copies(o0, o1, n0, n1)
            o2 = CPT * qo + (ro >> 3)
            n2 = jnp.minimum(CPT * qn + jnp.minimum(rn >> 3, CPT - 1) + 1, NCH)
            return (o1, o2, n1, n2) + advance(qo, ro) + advance(qn, rn)

        e1, e2, e3 = U1 + UPB, U1 + 2 * UPB, U1 + 3 * UPB
        init = (odone(U1), odone(e1), xneed(e1), xneed(e2), po(e2) // SP, po(e2) % SP, pn(e3) // SP, pn(e3) % SP)
        fin = jax.lax.fori_loop(0, NBODY, body, tuple(jnp.int32(v) for v in init))
        assert xneed(U2 + UPB) == NCH

        z = jnp.minimum(fin[0], 0)
        tile0 = (NB - 1) * SP
        lanes = pl.ds((NB - 1) * TB, TB)
        ecopies = []

        def ecopy(s_lo, s_hi, rlo=0, rhi=C):
            cp = pltpu.make_async_copy(
                obuf.at[pl.ds(tile0 + s_lo, s_hi - s_lo), pl.ds(rlo, rhi - rlo), :],
                o_hbm.at[pl.ds(s_lo, s_hi - s_lo), pl.ds(rlo, rhi - rlo), lanes],
                sems.at[ES0 + len(ecopies)])
            ecopies.append(cp)
            return cp

        ta, tb = NU - 2, NU - 1
        s_a, s_c, s_d = MO * U2 - tile0, MO * ta - tile0, MO * tb - tile0
        sent0, sent = odone(U2), (NB - 1) * CPT
        assert sent0 <= sent <= sent0 + MAXC and 0 < s_a and S - s_d == MO - 1
        ea, eb, ec = ecopy(0, s_a), ecopy(s_a, s_c), ecopy(s_c, s_d)

        def last2(i):
            units(U2 + z, 2, i)
            pl.when(i >= 0)(ea.start)
            copies(z + sent0, z + sent, z + NCH, z + NCH)
            pl.when(i >= 0)(ocopy(z).wait)

        mta = [mc_ref if j < JS else ma_ref for j in range(NP)]
        mtb = [md_ref if j < JS else mc_ref for j in range(NP)]

        def last_a(i):
            output(U2 + z, mbuf[0])
            output(U2 + 1 + z, mbuf[1])
            unit(ta + z, True, mta, i, GROUPS_END, ORDER_END)
            carry_u0(tb + z)
            pl.when(i >= 0)(eb.start)

        def last_b(i):
            output(ta + z, mta)
            unit(tb + z, True, mtb, i, GROUPS_END, ORDER_END[:-1])
            pl.when(i >= 0)(ec.start)

        once(z, last2)
        once(z, last_a)
        once(z, last_b)
        for rlo, rhi in zip(PIECES[:-1], PIECES[1:]):
            output(tb, mtb, rlo, rhi, MO - 1)
            ecopy(s_d, S, rlo, rhi).start()
        for c in range(1, sent):
            ocopy(c).wait()
        for cp in ecopies:
            cp.wait()

    any_spec = pl.BlockSpec(memory_space=pl.ANY)
    out = pl.pallas_call(
        kernel,
        in_specs=[any_spec] * 6,
        out_specs=any_spec,
        out_shape=jax.ShapeDtypeStruct((S, C, B), x.dtype),
        scratch_shapes=[
            pltpu.VMEM((NP, NKT + 1, C // 2, 128), U32),
            pltpu.VMEM((CF, TB), BF16),
            pltpu.VMEM((RING + 2, C, TB), BF16),
            pltpu.VMEM((NU * MO, C, TB), BF16),
            pltpu.VMEM((C, 128), F32),
            pltpu.VMEM((C, 128), F32),
            pltpu.VMEM((NP, C, TB), F32),
            pltpu.VMEM((NP, C, TB), F32),
            pltpu.VMEM((NP, C, TB), F32),
            pltpu.VMEM((NP, C, TB), F32),
            pltpu.VMEM((NKT, C // 2, 128), U32),
            pltpu.VMEM((3, C // 2, 128), U32),
            pltpu.VMEM((C,), BF16), pltpu.VMEM((C,), BF16),
            pltpu.VMEM((C,), BF16), pltpu.VMEM((C,), BF16),
            pltpu.VMEM((3, C + 24, C), BF16),
            pltpu.SemaphoreType.DMA((NSEM,)),
        ],
        compiler_params=pltpu.CompilerParams(vmem_limit_bytes=100 * 1024 * 1024,
                                             disable_bounds_checks=True, disable_semaphore_checks=True),
    )(jnp.transpose(x, (1, 2, 0)), w, mean, var, g, b)
    return jnp.transpose(out, (2, 0, 1))
```
